```python
import jax
import jax.numpy as jnp

def _softmax(x, axis=-1):
    return jax.nn.softmax(x, axis=axis)
def _gelu(x):
    return jax.nn.gelu(x, approximate=True)
def _silu(x):
    return jax.nn.silu(x)
def _sigmoid(x):
    return jax.nn.sigmoid(x)
def _layernorm(x, axis=-1, eps=1e-5):
    m = jnp.mean(x, axis=axis, keepdims=True)
    v = jnp.var(x, axis=axis, keepdims=True)
    return (x - m) / jnp.sqrt(v + eps)
def _scatter_add(tgt, idx, src, axis=0):
    return tgt.at[idx].add(src)
def _segment_sum(src, seg, n):
    return jax.ops.segment_sum(src, seg, n)
class _Rng:
    def __init__(self, key):
        self._k = key
    def _next(self):
        self._k, sub = jax.random.split(self._k)
        return sub
    def normal(self, shape):
        return jax.random.normal(self._next(), shape, dtype=jnp.bfloat16)
    def randint(self, lo, hi, shape):
        return jax.random.randint(self._next(), shape, lo, hi, dtype=jnp.int32)
    def uniform(self, shape, lo=0.0, hi=1.0):
        return jax.random.uniform(self._next(), shape, jnp.bfloat16, lo, hi)
    def permutation(self, n):
        return jax.random.permutation(self._next(), n)


kernel_name = 'concat_heads__ssm_conv_h3__compressed_kv_cla__prompt'

def setup_inputs():
    _rng = _Rng(jax.random.key(int.from_bytes(__import__("os").urandom(4), "little")))
    _w = (lambda a: (lambda t: t.astype(jnp.bfloat16) if jnp.issubdtype(t.dtype, jnp.floating) else t)(jnp.asarray(a)))
    def _A_setup():
        B, S, D = 1, 2048, 448
        ks = 4
        return {
            "q": _w((lambda *s: _rng.normal(s) * 0.05)(B, S, D)),
            "k": _w((lambda *s: _rng.normal(s) * 0.05)(B, S, D)),
            "v": _w((lambda *s: _rng.normal(s) * 0.05)(B, S, D)),
            "shift_k": _w((lambda *s: _rng.normal(s) * 0.05)(D, ks) * 0.5),
            "ssm_k": _w((lambda *s: _rng.normal(s) * 0.05)(D, S) * (1.0 / S ** 0.5)),
            "ssm_D": _w((lambda *s: _rng.normal(s) * 0.05)(D)),
        }
    _A_in = _A_setup()

    def _B_setup():
        B, H, Sq, Sk, D, M = 1, 16, 2048, 2048, 256, 448
        Dc = 4 * D
        return {
            "x": _w((lambda *s: _rng.normal(s) * 0.05)(B, Sq, M)),
            "c_kv": _w((lambda *s: _rng.normal(s) * 0.05)(B, Sk, Dc)),
            "w_q": _w((lambda *s: _rng.normal(s) * 0.05)(M, H, D) * (M ** -0.5)),
            "w_uk": _w((lambda *s: _rng.normal(s) * 0.05)(Dc, H, D) * (Dc ** -0.5)),
            "w_uv": _w((lambda *s: _rng.normal(s) * 0.05)(Dc, H, D) * (Dc ** -0.5)),
            "w_o": _w((lambda *s: _rng.normal(s) * 0.05)(H, D, M) * ((H * D) ** -0.5)),
        }
    _B_in = _B_setup()

    return {
        "A_q": _A_in["q"],
        "A_k": _A_in["k"],
        "A_v": _A_in["v"],
        "A_shift_k": _A_in["shift_k"],
        "A_ssm_k": _A_in["ssm_k"],
        "A_ssm_D": _A_in["ssm_D"],
        "B_x": _B_in["x"],
        "B_c_kv": _B_in["c_kv"],
        "B_w_q": _B_in["w_q"],
        "B_w_uk": _B_in["w_uk"],
        "B_w_uv": _B_in["w_uv"],
        "B_w_o": _B_in["w_o"],
    }

def reference(A_q, A_k, A_v, A_shift_k, A_ssm_k, A_ssm_D, B_x, B_c_kv, B_w_q, B_w_uk, B_w_uv, B_w_o):
    def _A_ref(q, k, v, shift_k, ssm_k, ssm_D):
        B, S, D = q.shape
        ks = shift_k.shape[-1]
        k_pad = jnp.pad(k, ((0, 0), (ks - 1, 0), (0, 0)))
        k_shift = jnp.zeros_like(k)
        for t in range(ks):
            k_shift = k_shift + k_pad[:, t:t + S, :] * shift_k[:, ks - 1 - t][None, None, :]
        kv = k_shift * v
        L = 2 * S
        kv_pad = jnp.pad(kv, ((0, 0), (0, S), (0, 0)))
        kf_pad = jnp.pad(ssm_k, ((0, 0), (0, S)))
        kv_f = (lambda x, axes=(-2,-1): jnp.fft.rfft2(x.astype(jnp.float32), axes=axes))(kv_pad[:, None, :, :], axes=(1, 2))
        kf_f = (lambda x, axes=(-2,-1): jnp.fft.rfft2(x.astype(jnp.float32), axes=axes))(kf_pad[:, None, :], axes=(1, 2))
        kf_f = (lambda x, *d: x.transpose(*d))(kf_f, 1, 2, 0)
        y_f = kv_f * kf_f[None, :, :, :]
        y = (lambda x, s, axes=(-2,-1): jnp.fft.irfft2(x, s=s, axes=axes).astype(jnp.bfloat16))(y_f, (1, L), axes=(1, 2))[:, 0, :S, :]
        y = y + kv * ssm_D[None, None, :]
        return q * y

    def _B_ref(x, c_kv, w_q, w_uk, w_uv, w_o):
        B, Sq, M = x.shape[0], x.shape[1], x.shape[2]
        Sk = c_kv.shape[1]
        H, D = w_q.shape[1], w_q.shape[2]
        q = jnp.einsum("bqm,mhd->bhqd", x, w_q)
        k = jnp.einsum("bkc,chd->bhkd", c_kv, w_uk)
        v = jnp.einsum("bkc,chd->bhkd", c_kv, w_uv)
        scores = jnp.einsum("bhqd,bhkd->bhqk", q, k) * (D ** -0.5)
        off = Sk - Sq
        qi = jnp.arange(Sq)[:, None]
        kj = jnp.arange(Sk)[None, :]
        cmask = kj <= (qi + off)
        scores = jnp.where(cmask[None, None], scores, -1e9)
        p = _softmax(scores, axis=-1)
        ctx = jnp.einsum("bhqk,bhkd->bhqd", p, v)
        return jnp.einsum("bhqd,hdm->bqm", ctx, w_o)

    a = _A_ref(A_q, A_k, A_v, A_shift_k, A_ssm_k, A_ssm_D)
    b = _B_ref(B_x, B_c_kv, B_w_q, B_w_uk, B_w_uv, B_w_o)
    return jnp.concatenate([a, b], axis=-1)
```

```python
import math

import jax
import jax.numpy as jnp
import numpy as np
import jax.experimental.pallas as pl
import jax.experimental.pallas.tpu as pltpu

F32 = jnp.float32
BF16 = jnp.bfloat16
U32 = jnp.uint32

S = 2048
DA = 448
H = 16
D = 256
DC = 1024
KS = 4
C = 128
NCH = S // C
TQ = 128
NQ = S // TQ
KC = 128
LOG2E = math.log2(math.e)
QSCALE = (D ** -0.5) * LOG2E
NEG = -1e9 * LOG2E


def _nn(a, b):
    return jnp.dot(a, b, preferred_element_type=F32)


def _nt(a, b):
    return jax.lax.dot_general(a, b, (((1,), (1,)), ((), ())), preferred_element_type=F32)


def _dft_mats():
    k = np.concatenate([np.arange(0, C, 2), np.arange(1, C, 2)]).astype(np.float64)
    n = np.arange(C, dtype=np.float64)
    th = 2.0 * np.pi * np.outer(n, k + 0.5) / (2 * C)
    fwd = np.concatenate([np.cos(th), np.sin(th)], axis=1)
    inv = fwd.T / C
    return fwd, inv


def _kernel(qT_hbm, kT_hbm, vT_hbm, shT_ref, ssm_hbm, dvec_ref, xT_hbm, ckv_hbm, wq_hbm, wuk_hbm, wuv_hbm,
            woT_hbm, fwd_ref, inv_ref,
            out_hbm,
            aq, ak, av, ssm, xT, xs, ckv, wq, wuk, wuv, woT, qs, ks, vTs, cs, acc, aT, xspec, hspec, kvb, outs, sems):
    def cp(src, dst, i):
        return pltpu.make_async_copy(src, dst, sems.at[i])

    wq_u, wuk_u, wuv_u = wq_hbm.bitcast(U32), wuk_hbm.bitcast(U32), wuv_hbm.bitcast(U32)
    c_x = cp(xT_hbm, xT, 0)
    c_wq = [cp(wq_u.at[:, pl.ds(128 * t, 128)], wq.at[t], 1 + t) for t in range(2)]
    c_ak, c_av, c_ssm, c_aq = cp(kT_hbm, ak, 3), cp(vT_hbm, av, 4), cp(ssm_hbm, ssm, 5), cp(qT_hbm, aq, 6)
    c_ckv = cp(ckv_hbm, ckv, 7)
    c_wuk = [cp(wuk_u.at[:, pl.ds(128 * t, 128)], wuk.at[t], 8 + t) for t in range(2)]
    c_wuv = [cp(wuv_u.at[:, pl.ds(128 * t, 128)], wuv.at[t], 10 + t) for t in range(2)]
    c_wo = cp(woT_hbm, woT, 12)
    for c in [c_x, *c_wq, c_ak, c_av, c_ssm, c_aq, c_ckv, *c_wuk, *c_wuv, c_wo]:
        c.start()

    acc[...] = jnp.zeros(acc.shape, F32)

    c_x.wait()
    xs[...] = xT[...].T
    for c in c_wq:
        c.wait()
    hi_mask = jnp.uint32(0xFFFF0000)
    for j in range(H // 2):
        words = [wq[t, pl.ds(j, DA, stride=8), :] for t in range(2)]
        lo = [pltpu.bitcast(w << 16, F32).astype(BF16) for w in words]
        hi = [pltpu.bitcast(w & hi_mask, F32).astype(BF16) for w in words]
        wpair = jnp.concatenate(lo + hi, axis=1)
        q2 = (_nn(xs[...], wpair) * QSCALE).astype(BF16)
        qs[2 * j] = q2[:, :D]
        qs[2 * j + 1] = q2[:, D:]

    c_ak.wait()
    c_av.wait()
    c_ssm.wait()
    c_aq.wait()
    coef = jnp.concatenate([shT_ref[...].astype(F32), dvec_ref[...].astype(F32)[None, :],
                            jnp.zeros((3, DA), F32)], axis=0).T
    fwd = fwd_ref[...]
    inv = inv_ref[...]
    G = 64
    lane = jax.lax.broadcasted_iota(jnp.int32, (G, S), 1)
    for g in range(DA // G):
        rows = slice(g * G, (g + 1) * G)
        kf = ak[rows, :].astype(F32)
        ksh = kf * coef[rows, 0:1]
        for j in range(1, KS):
            sh = jnp.where(lane >= j, pltpu.roll(kf, j, 1), 0.0)
            ksh = ksh + sh * coef[rows, j:j + 1]
        kv = (ksh * av[rows, :].astype(F32)).astype(BF16)
        kvb[...] = kv
        prev = None
        for c in range(NCH):
            cols = slice(c * C, (c + 1) * C)
            xh = _nn(kvb[:, cols], fwd)
            hspec[c] = _nn(ssm[rows, cols], fwd)
            if prev is None:
                xspec[c] = xh
            else:
                hc = C // 2
                sgn_im = jnp.concatenate([prev[:, 2 * hc:3 * hc], -prev[:, 3 * hc:]], axis=1)
                sgn_re = jnp.concatenate([-prev[:, :hc], prev[:, hc:2 * hc]], axis=1)
                xspec[c] = xh + jnp.concatenate([sgn_im, sgn_re], axis=1)
            prev = xh
        for a in range(NCH):
            zr = zi = None
            for c in range(a + 1):
                ur, ui = xspec[c, :, :C], xspec[c, :, C:]
                hr, hi_ = hspec[a - c, :, :C], hspec[a - c, :, C:]
                pr = ur * hr - ui * hi_
                pi = ur * hi_ + ui * hr
                zr = pr if zr is None else zr + pr
                zi = pi if zi is None else zi + pi
            w = jnp.concatenate([zr, zi], axis=1).astype(BF16)
            y = _nn(w, inv)
            cols = slice(a * C, (a + 1) * C)
            y = y + kvb[:, cols].astype(F32) * coef[rows, KS:KS + 1]
            aT[rows, cols] = aq[rows, cols].astype(F32) * y

    c_ckv.wait()
    for c in c_wuk + c_wuv:
        c.wait()
    c_wo.wait()

    krow = jax.lax.broadcasted_iota(jnp.int32, (TQ, TQ), 0)
    qcol = jax.lax.broadcasted_iota(jnp.int32, (TQ, TQ), 1)

    def head(h, carry):
        j = h >> 1
        sh = (16 - 16 * (h & 1)).astype(U32)

        def extract(ref, t):
            return pltpu.bitcast((ref[t, pl.ds(j, DC, stride=8), :] << sh) & hi_mask, F32)

        wk = jnp.concatenate([extract(wuk, 0).astype(BF16), extract(wuk, 1).astype(BF16)], axis=1)
        wvT = jnp.concatenate([extract(wuv, 0).T.astype(BF16), extract(wuv, 1).T.astype(BF16)], axis=0)
        wo = woT[h]
        causal = krow <= qcol

        def kproj(c):
            r = slice(c * KC, (c + 1) * KC)
            ks[r, :] = _nn(ckv[r, :], wk).astype(BF16)

        def vproj(c):
            r = slice(c * KC, (c + 1) * KC)
            vTs[:, r] = _nt(wvT, ckv[r, :]).astype(BF16)

        def qk(i):
            n = TQ * (i + 1)
            return _nt(ks[:n, :], qs[h, TQ * i:n, :])

        def pv(i, sT):
            n = TQ * (i + 1)
            sd = jnp.where(causal, sT[n - TQ:], NEG)
            m = jnp.max(sd, axis=0, keepdims=True)
            if i > 0:
                so = sT[:n - TQ]
                m = jnp.maximum(m, jnp.max(so, axis=0, keepdims=True))
                p = jnp.concatenate([jnp.exp2(so - m), jnp.exp2(sd - m)], axis=0)
            else:
                p = jnp.exp2(sd - m)
            l = jnp.sum(p, axis=0, keepdims=True)
            ctxT = _nn(vTs[:, :n], p.astype(BF16)) * (1.0 / l)
            cs[:, TQ * i:n] = ctxT.astype(BF16)

        def oproj(i0, i1):
            cols = slice(TQ * i0, TQ * i1)
            acc[:, cols] += _nn(wo, cs[:, cols])

        per = KC // TQ
        s_prev = None
        for i in range(NQ):
            if i % per == 0:
                kproj(i // per)
            s_cur = qk(i)
            if i % per == 0:
                vproj(i // per)
            if i > 0:
                pv(i - 1, s_prev)
            s_prev = s_cur
        oproj(0, NQ // 2)
        pv(NQ - 1, s_prev)
        oproj(NQ // 2, NQ - 1)
        oproj(NQ - 1, NQ)
        return carry

    jax.lax.fori_loop(0, H, head, 0)

    TO = 256
    outc = []
    for i in range(S // TO):
        cols = slice(i * TO, (i + 1) * TO)
        blk = jnp.concatenate([aT[:, cols], acc[:, cols]], axis=0)
        outs[cols, :] = blk.T.astype(BF16)
        c = cp(outs.at[cols, :], out_hbm.at[cols, :], 13 + i)
        c.start()
        outc.append(c)
    for c in outc:
        c.wait()


@jax.jit
def pallas_concat_heads__ssm_conv_h3__compressed_kv_cla__prompt_kernel(
    A_q: jax.Array,
    A_k: jax.Array,
    A_v: jax.Array,
    A_shift_k: jax.Array,
    A_ssm_k: jax.Array,
    A_ssm_D: jax.Array,
    B_x: jax.Array,
    B_c_kv: jax.Array,
    B_w_q: jax.Array,
    B_w_uk: jax.Array,
    B_w_uv: jax.Array,
    B_w_o: jax.Array,
):
    fwd, inv = _dft_mats()
    tr = lambda a: jnp.swapaxes(a, 1, 2).reshape(DA, S)
    any_spec = pl.BlockSpec(memory_space=pl.ANY)
    vmem_spec = pl.BlockSpec(memory_space=pltpu.VMEM)
    out = pl.pallas_call(
        _kernel,
        out_shape=jax.ShapeDtypeStruct((S, 2 * DA), BF16),
        in_specs=[any_spec, any_spec, any_spec, vmem_spec, any_spec, vmem_spec, any_spec, any_spec, any_spec,
                  any_spec, any_spec, any_spec, vmem_spec, vmem_spec],
        out_specs=any_spec,
        scratch_shapes=[
            pltpu.VMEM((DA, S), BF16),
            pltpu.VMEM((DA, S), BF16),
            pltpu.VMEM((DA, S), BF16),
            pltpu.VMEM((DA, S), BF16),
            pltpu.VMEM((DA, S), BF16),
            pltpu.VMEM((S, DA), BF16),
            pltpu.VMEM((S, DC), BF16),
            pltpu.VMEM((2, DA * H // 2, 128), U32),
            pltpu.VMEM((2, DC * H // 2, 128), U32),
            pltpu.VMEM((2, DC * H // 2, 128), U32),
            pltpu.VMEM((H, DA, D), BF16),
            pltpu.VMEM((H, S, D), BF16),
            pltpu.VMEM((S, D), BF16),
            pltpu.VMEM((D, S), BF16),
            pltpu.VMEM((D, S), BF16),
            pltpu.VMEM((DA, S), F32),
            pltpu.VMEM((DA, S), F32),
            pltpu.VMEM((NCH, 64, 2 * C), F32),
            pltpu.VMEM((NCH, 64, 2 * C), F32),
            pltpu.VMEM((64, S), BF16),
            pltpu.VMEM((S, 2 * DA), BF16),
            pltpu.SemaphoreType.DMA((13 + S // 256,)),
        ],
        compiler_params=pltpu.CompilerParams(vmem_limit_bytes=100 * 1024 * 1024),
    )(
        tr(A_q), tr(A_k), tr(A_v), A_shift_k.T, A_ssm_k, A_ssm_D, tr(B_x), B_c_kv.reshape(S, DC),
        B_w_q.reshape(DA * H, D), B_w_uk.reshape(DC * H, D), B_w_uv.reshape(DC * H, D),
        jnp.swapaxes(B_w_o, 1, 2), jnp.asarray(fwd, BF16), jnp.asarray(inv, BF16),
    )
    return out.reshape(1, S, 2 * DA)
```

```python
import math

import jax
import jax.numpy as jnp
import numpy as np
import jax.experimental.pallas as pl
import jax.experimental.pallas.tpu as pltpu

F32 = jnp.float32
BF16 = jnp.bfloat16
U32 = jnp.uint32

S = 2048
DA = 448
H = 16
D = 256
DC = 1024
KS = 4
C = 128
NCH = S // C
G = 64
TQ = 128
NQ = S // TQ
KC = 128
RW = 64
NT = (((1,), (1,)), ((), ()))
LOG2E = math.log2(math.e)
QSCALE = (D ** -0.5) * LOG2E
NEG = -1e9 * LOG2E


def _nn(a, b):
    return jnp.dot(a, b, preferred_element_type=F32)


def _nt(a, b):
    return jax.lax.dot_general(a, b, (((1,), (1,)), ((), ())), preferred_element_type=F32)


def _dft_mats():
    k = np.concatenate([np.arange(0, C, 2), np.arange(1, C, 2)]).astype(np.float64)
    n = np.arange(C, dtype=np.float64)
    th = 2.0 * np.pi * np.outer(n, k + 0.5) / (2 * C)
    fwd = np.concatenate([np.cos(th), np.sin(th)], axis=1)
    inv = fwd.T / C
    return fwd, inv


def _kernel(qT_hbm, kT_hbm, vT_hbm, shT_ref, ssm_hbm, dvec_ref, xT_hbm, ckv_hbm, wq_hbm, wuk_hbm, wuv_hbm,
            woT_hbm, fwd_ref, inv_ref,
            out_hbm,
            aq, ak, av, ssm, xT, xs, ckv, wq, wuk, wuv, woT, qs, ks, vTs, cs, acc, aT, xspec, hspec, kvb, outs, sems):
    def cp(src, dst, i):
        return pltpu.make_async_copy(src, dst, sems.at[i])

    wq_u, wuk_u, wuv_u = wq_hbm.bitcast(U32), wuk_hbm.bitcast(U32), wuv_hbm.bitcast(U32)
    c_x = cp(xT_hbm, xT, 0)
    c_wq = [cp(wq_u.at[:, pl.ds(128 * t, 128)], wq.at[t], 1 + t) for t in range(2)]
    c_ak, c_av, c_ssm, c_aq = cp(kT_hbm, ak, 3), cp(vT_hbm, av, 4), cp(ssm_hbm, ssm, 5), cp(qT_hbm, aq, 6)
    c_ckv = cp(ckv_hbm, ckv, 7)
    c_wuk = [cp(wuk_u.at[:, pl.ds(128 * t, 128)], wuk.at[t], 8 + t) for t in range(2)]
    c_wuv = [cp(wuv_u.at[:, pl.ds(128 * t, 128)], wuv.at[t], 10 + t) for t in range(2)]
    c_wo = cp(woT_hbm, woT, 12)
    for c in [c_x, *c_wq, c_ak, c_av, c_ssm, c_aq, c_ckv, *c_wuk, *c_wuv, c_wo]:
        c.start()

    acc[...] = jnp.zeros(acc.shape, F32)

    hi_mask = jnp.uint32(0xFFFF0000)

    def wq_pair(j):
        words = [wq[t, pl.ds(j, DA, stride=8), :] for t in range(2)]
        lo = [pltpu.bitcast(w << 16, F32).astype(BF16) for w in words]
        hi = [pltpu.bitcast(w & hi_mask, F32).astype(BF16) for w in words]
        return jnp.concatenate(lo + hi, axis=1)

    def qproj(j, wpair, r0, r1):
        q2 = (jnp.dot(xs[r0:r1, :], wpair, preferred_element_type=F32) * QSCALE).astype(BF16)
        qs[2 * j, r0:r1, :] = q2[:, :D]
        qs[2 * j + 1, r0:r1, :] = q2[:, D:]

    c_x.wait()
    xs[...] = xT[...].T
    for c in c_wq:
        c.wait()
    qproj(0, wq_pair(0), 0, S)

    c_ak.wait()
    c_av.wait()
    c_ssm.wait()
    c_aq.wait()
    coef = jnp.concatenate([shT_ref[...].astype(F32), dvec_ref[...].astype(F32)[None, :],
                            jnp.zeros((3, DA), F32)], axis=0).T
    lane = jax.lax.broadcasted_iota(jnp.int32, (G, S), 1)
    hc = C // 2

    def gate(g):
        rows = slice(g * G, (g + 1) * G)
        kf = ak[rows, :].astype(F32)
        ksh = kf * coef[rows, 0:1]
        for j in range(1, KS):
            sh = jnp.where(lane >= j, pltpu.roll(kf, j, 1), 0.0)
            ksh = ksh + sh * coef[rows, j:j + 1]
        kvb[rows, :] = (ksh * av[rows, :].astype(F32)).astype(BF16)

    def forward(g, c, prev):
        rows, cols = slice(g * G, (g + 1) * G), slice(c * C, (c + 1) * C)
        both = jnp.dot(jnp.concatenate([kvb[rows, cols], ssm[rows, cols]], axis=0), fwd_ref[...],
                       preferred_element_type=F32)
        xh, hh = both[:G], both[G:]
        if prev is None:
            u = xh
        else:
            u = xh + jnp.concatenate([prev[:, 2 * hc:3 * hc], -prev[:, 3 * hc:], -prev[:, :hc],
                                      prev[:, hc:2 * hc]], axis=1)
        xspec[g % 2, c] = u
        hspec[g % 2, c] = hh
        return xh

    def inverse(g, a):
        rows, cols = slice(g * G, (g + 1) * G), slice(a * C, (a + 1) * C)
        zr = zi = None
        for c in range(a + 1):
            ur, ui = xspec[g % 2, c, :, :C], xspec[g % 2, c, :, C:]
            hr, hi = hspec[g % 2, a - c, :, :C], hspec[g % 2, a - c, :, C:]
            pr = ur * hr - ui * hi
            pi = ur * hi + ui * hr
            zr = pr if zr is None else zr + pr
            zi = pi if zi is None else zi + pi
        w = jnp.concatenate([zr, zi], axis=1).astype(BF16)
        y = jnp.dot(w, inv_ref[...], preferred_element_type=F32)
        y = y + kvb[rows, cols].astype(F32) * coef[rows, KS:KS + 1]
        aT[rows, cols] = aq[rows, cols].astype(F32) * y

    NG = DA // G
    NP = NCH // 2
    gate(0)
    prev = None
    for c in range(NCH):
        prev = forward(0, c, prev)
    for g in range(NG):
        wpair = wq_pair(g + 1)
        if g + 1 < NG:
            gate(g + 1)
        prev = None
        for p in range(NP):
            qproj(g + 1, wpair, p * (S // NP), (p + 1) * (S // NP))
            inverse(g, NCH - 1 - p)
            inverse(g, p)
            if g + 1 < NG:
                prev = forward(g + 1, 2 * p, prev)
                prev = forward(g + 1, 2 * p + 1, prev)

    c_ckv.wait()
    for c in c_wuk + c_wuv:
        c.wait()
    c_wo.wait()

    krow = jax.lax.broadcasted_iota(jnp.int32, (TQ, TQ), 0)
    qcol = jax.lax.broadcasted_iota(jnp.int32, (TQ, TQ), 1)

    def head(h, carry):
        j = h >> 1
        sh = (16 - 16 * (h & 1)).astype(U32)

        def extract(ref, t):
            return pltpu.bitcast((ref[t, pl.ds(j, DC, stride=8), :] << sh) & hi_mask, F32)

        wk = jnp.concatenate([extract(wuk, 0).astype(BF16), extract(wuk, 1).astype(BF16)], axis=1)
        wvT = jnp.concatenate([extract(wuv, 0).T.astype(BF16), extract(wuv, 1).T.astype(BF16)], axis=0)
        wo = woT[h]
        causal = krow <= qcol

        def kproj(c):
            r = slice(c * KC, (c + 1) * KC)
            ks[r, :] = jnp.dot(ckv[r, :], wk, preferred_element_type=F32).astype(BF16)

        def vproj(c):
            r = slice(c * KC, (c + 1) * KC)
            vTs[:, r] = jax.lax.dot_general(wvT, ckv[r, :], NT, preferred_element_type=F32).astype(BF16)

        def qk(i):
            n = TQ * (i + 1)
            return jax.lax.dot_general(ks[:n, :], qs[h, TQ * i:n, :], NT, preferred_element_type=F32)

        def softmax(i, sT):
            n = TQ * (i + 1)
            sd = jnp.where(causal, sT[n - TQ:], NEG)
            s = sd if i == 0 else jnp.concatenate([sT[:n - TQ], sd], axis=0)
            m = jnp.max(jnp.max(s.reshape(n // RW, RW, TQ), axis=0), axis=0, keepdims=True)
            m8 = jnp.broadcast_to(m, (8, TQ))
            ls, ps = None, []
            for c0 in range(0, n, TQ):
                mm = m8 if ls is None else jnp.where(ls < 0.0, ls, m8)
                p = jnp.exp2(s[c0:c0 + TQ] - jnp.concatenate([mm] * (TQ // 8), axis=0))
                part = jnp.sum(p.reshape(TQ // 8, 8, TQ), axis=0)
                ls = part if ls is None else ls + part
                ps.append(p.astype(BF16))
            l = jnp.sum(ls, axis=0, keepdims=True)
            return jnp.concatenate(ps, axis=0), 1.0 / l

        def pv(i, p, rl):
            n = TQ * (i + 1)
            ctxT = jnp.dot(vTs[:, :n], p, preferred_element_type=F32) * rl
            cs[:, TQ * i:n] = ctxT.astype(BF16)

        def oproj(i0, i1):
            cols = slice(TQ * i0, TQ * i1)
            acc[:, cols] += jnp.dot(wo, cs[:, cols], preferred_element_type=F32)

        per = KC // TQ
        s_prev = None
        for i in range(NQ):
            if i % per == 0:
                kproj(i // per)
            if i > 0:
                sm = softmax(i - 1, s_prev)
            s_prev = qk(i)
            if i % per == 0:
                vproj(i // per)
            if i > 0:
                pv(i - 1, *sm)
        sm = softmax(NQ - 1, s_prev)
        oproj(0, NQ // 2)
        pv(NQ - 1, *sm)
        oproj(NQ // 2, NQ - 1)
        oproj(NQ - 1, NQ)
        return carry

    jax.lax.fori_loop(0, H, head, 0)

    TO = 256
    outc = []
    for i in range(S // TO):
        cols = slice(i * TO, (i + 1) * TO)
        blk = jnp.concatenate([aT[:, cols], acc[:, cols]], axis=0)
        outs[cols, :] = blk.T.astype(BF16)
        c = cp(outs.at[cols, :], out_hbm.at[cols, :], 13 + i)
        c.start()
        outc.append(c)
    for c in outc:
        c.wait()


@jax.jit
def pallas_concat_heads__ssm_conv_h3__compressed_kv_cla__prompt_kernel(
    A_q: jax.Array,
    A_k: jax.Array,
    A_v: jax.Array,
    A_shift_k: jax.Array,
    A_ssm_k: jax.Array,
    A_ssm_D: jax.Array,
    B_x: jax.Array,
    B_c_kv: jax.Array,
    B_w_q: jax.Array,
    B_w_uk: jax.Array,
    B_w_uv: jax.Array,
    B_w_o: jax.Array,
):
    fwd, inv = _dft_mats()
    tr = lambda a: jnp.swapaxes(a, 1, 2).reshape(DA, S)
    any_spec = pl.BlockSpec(memory_space=pl.ANY)
    vmem_spec = pl.BlockSpec(memory_space=pltpu.VMEM)
    out = pl.pallas_call(
        _kernel,
        out_shape=jax.ShapeDtypeStruct((S, 2 * DA), BF16),
        in_specs=[any_spec, any_spec, any_spec, vmem_spec, any_spec, vmem_spec, any_spec, any_spec, any_spec,
                  any_spec, any_spec, any_spec, vmem_spec, vmem_spec],
        out_specs=any_spec,
        scratch_shapes=[
            pltpu.VMEM((DA, S), BF16),
            pltpu.VMEM((DA, S), BF16),
            pltpu.VMEM((DA, S), BF16),
            pltpu.VMEM((DA, S), BF16),
            pltpu.VMEM((DA, S), BF16),
            pltpu.VMEM((S, DA), BF16),
            pltpu.VMEM((S, DC), BF16),
            pltpu.VMEM((2, DA * H // 2, 128), U32),
            pltpu.VMEM((2, DC * H // 2, 128), U32),
            pltpu.VMEM((2, DC * H // 2, 128), U32),
            pltpu.VMEM((H, DA, D), BF16),
            pltpu.VMEM((H, S, D), BF16),
            pltpu.VMEM((S, D), BF16),
            pltpu.VMEM((D, S), BF16),
            pltpu.VMEM((D, S), BF16),
            pltpu.VMEM((DA, S), F32),
            pltpu.VMEM((DA, S), F32),
            pltpu.VMEM((2, NCH, G, 2 * C), F32),
            pltpu.VMEM((2, NCH, G, 2 * C), F32),
            pltpu.VMEM((DA, S), BF16),
            pltpu.VMEM((S, 2 * DA), BF16),
            pltpu.SemaphoreType.DMA((13 + S // 256,)),
        ],
        compiler_params=pltpu.CompilerParams(vmem_limit_bytes=100 * 1024 * 1024),
    )(
        tr(A_q), tr(A_k), tr(A_v), A_shift_k.T, A_ssm_k, A_ssm_D, tr(B_x), B_c_kv.reshape(S, DC),
        B_w_q.reshape(DA * H, D), B_w_uk.reshape(DC * H, D), B_w_uv.reshape(DC * H, D),
        jnp.swapaxes(B_w_o, 1, 2), jnp.asarray(fwd, BF16), jnp.asarray(inv, BF16),
    )
    return out.reshape(1, S, 2 * DA)
```

```python
import functools
import math

import jax
import jax.numpy as jnp
import numpy as np
import jax.experimental.pallas as pl
import jax.experimental.pallas.tpu as pltpu

F32 = jnp.float32
BF16 = jnp.bfloat16
U32 = jnp.uint32

S = 2048
DA = 448
H = 16
D = 256
DC = 1024
KS = 4
C = 128
NCH = S // C
G = 32
NG = DA // G
TQ = 128
NQ = S // TQ
NT = (((1,), (1,)), ((), ()))
NSEM = 3 * (H // 2) + 7 + 8
LOG2E = math.log2(math.e)
QSCALE = (D ** -0.5) * LOG2E
NEG = -1e9 * LOG2E

NHEADS = H
CONV = 1
KSPL = 1
VSPL = 2
PSPL = 2
KAHEAD = 1
CSSA = 1
SLAB = 8
CHAIN = 1
TOK = 1
QN = 2048
FWD_AT = 2
INV_SCHED = {4: [0, 1, 2, 3], 5: [4, 5], 6: [6], 7: [7], 8: [8], 9: [9], 10: [10], 11: [11], 12: [12], 13: [13], 14: [14], 15: [15]}


def _dft_mats():
    k = np.concatenate([np.arange(0, C, 2), np.arange(1, C, 2)]).astype(np.float64)
    n = np.arange(C, dtype=np.float64)
    th = 2.0 * np.pi * np.outer(n, k + 0.5) / (2 * C)
    fwd = np.concatenate([np.cos(th), np.sin(th)], axis=1)
    inv = fwd.T / C
    return fwd, inv


def _b(x):
    return pltpu.bitcast(x, BF16)


def _w(x):
    return pltpu.bitcast(x, U32)


def _kernel(qT_hbm, kT_hbm, vT_hbm, shT_ref, ssm_hbm, dvec_ref, xT_hbm, ckv_hbm, wq_hbm, wuk_hbm, wuv_hbm,
            woT_hbm, fwd_ref, inv_ref,
            out_hbm,
            aq, ak, av, ssm, xT, ckv, wq, wuk, wuv, woT, wqs, qs, ks, vTs, cs, acc, aT, coef, wks, wvs,
            outs, sems):
    sem_ids = iter(range(NSEM))

    def cp(src, dst):
        return pltpu.make_async_copy(src, dst, sems.at[next(sem_ids)])

    wq_u, wuk_u, wuv_u = wq_hbm.bitcast(U32), wuk_hbm.bitcast(U32), wuv_hbm.bitcast(U32)
    c_wq = [cp(wq_u.at[:, j, :], wq.at[j]) for j in range(H // 2)]
    c_wuk = [cp(wuk_u.at[:, j, :], wuk.at[j]) for j in range(H // 2)]
    c_wuv = [cp(wuv_u.at[:, j, :], wuv.at[j]) for j in range(H // 2)]
    c_x = cp(xT_hbm.bitcast(U32), xT)
    c_ak, c_av = cp(kT_hbm.bitcast(U32), ak), cp(vT_hbm.bitcast(U32), av)
    c_ssm, c_aq = cp(ssm_hbm.bitcast(U32), ssm), cp(qT_hbm.bitcast(U32), aq)
    c_ckv = cp(ckv_hbm.bitcast(U32), ckv)
    c_wo = cp(woT_hbm.bitcast(U32), woT)
    early = [c_ckv, c_wuk[0], c_wuv[0], c_wo, c_ak, c_av, c_ssm, c_aq]
    late = [c for j in range(1, H // 2) for c in (c_wuk[j], c_wuv[j])]
    for c in [c_wq[0], c_x, *c_wq[1:], *early, *late]:
        c.start()

    hi_mask = jnp.uint32(0xFFFF0000)

    def prep_wq(j):
        w = wq[j]
        wqs[:D // 2, :] = _w(pltpu.bitcast(w << 16, F32).T.astype(BF16))
        wqs[D // 2:, :] = _w(pltpu.bitcast(w & hi_mask, F32).T.astype(BF16))

    def prep_wkv(h):
        j = h >> 1
        sh = jnp.asarray(16 - 16 * (h & 1), U32)
        wks[...] = _w(pltpu.bitcast((wuk[j] << sh) & hi_mask, F32).astype(BF16))
        wvs[...] = _w(pltpu.bitcast((wuv[j] << sh) & hi_mask, F32).T.astype(BF16))

    acc[...] = jnp.zeros(acc.shape, F32)
    cf = jnp.concatenate([shT_ref[...].astype(F32), dvec_ref[...].astype(F32)[None, :],
                          jnp.zeros((3, DA), F32)], axis=0).T
    for j in range(KS + 1):
        coef[j] = jnp.broadcast_to(cf[:, j:j + 1], (DA, 128))
    c_wq[0].wait()
    prep_wq(0)

    c_x.wait()

    def qpair(j, carry):
        @pl.when(j + 1 < H // 2)
        def _():
            pltpu.make_async_copy(wq_u.at[:, j + 1, :], wq.at[j + 1], sems.at[j + 1]).wait()

        for c0 in range(0, S, QN):
            q2 = (jnp.dot(_b(wqs[...]), _b(xT[:, c0:c0 + QN]), preferred_element_type=F32) * QSCALE).astype(BF16)
            qs[2 * j, :, c0:c0 + QN] = _w(q2[:D])
            qs[2 * j + 1, :, c0:c0 + QN] = _w(q2[D:])
        prep_wq(jnp.minimum(j + 1, H // 2 - 1))
        return carry

    jax.lax.fori_loop(0, H // 2, qpair, 0)

    for c in early:
        c.wait()
    prep_wkv(0)

    hc = C // 2

    def conv_ops(g):
        rows = pl.ds(pl.multiple_of(g * G, G), G)
        roww = pl.ds(pl.multiple_of(g * (G // 2), G // 2), G // 2)
        lane = jax.lax.broadcasted_iota(jnp.int32, (G, C), 1)
        st = {}

        def forward():
            kvs, kprev = [], None
            for c in range(NCH):
                cols = slice(c * C, (c + 1) * C)
                kf = _b(ak[roww, cols]).astype(F32)
                ksh = kf * coef[0, rows, :]
                rolled = []
                for j in range(1, KS):
                    r = pltpu.roll(kf, j, 1)
                    rolled.append(r)
                    ksh = ksh + jnp.where(lane >= j, r, 0.0 if kprev is None else kprev[j - 1]) * coef[j, rows, :]
                kvs.append((ksh * _b(av[roww, cols]).astype(F32)).astype(BF16))
                kprev = rolled
            st["kv"] = kvs
            lhs = jnp.concatenate(kvs + [_b(ssm[roww, c * C:(c + 1) * C]) for c in range(NCH)], axis=0)
            both = jnp.dot(lhs, fwd_ref[...], preferred_element_type=F32)
            xh = [both[c * G:(c + 1) * G] for c in range(NCH)]
            st["h"] = [both[(NCH + c) * G:(NCH + c + 1) * G] for c in range(NCH)]
            st["u"] = [xh[0]] + [
                xh[c] + jnp.concatenate([xh[c - 1][:, 2 * hc:3 * hc], -xh[c - 1][:, 3 * hc:], -xh[c - 1][:, :hc],
                                         xh[c - 1][:, hc:2 * hc]], axis=1) for c in range(1, NCH)]

        def inverse(todo):
            ws, tok = [], None
            for a in todo:
                slabs = []
                for r0 in range(0, G, SLAB):
                    rs = slice(r0, r0 + SLAB)
                    zr = zi = None
                    for c in range(a + 1):
                        ur, ui = st["u"][c][rs, :C], st["u"][c][rs, C:]
                        hr, hi = st["h"][a - c][rs, :C], st["h"][a - c][rs, C:]
                        if zr is None and tok is not None:
                            ur = jnp.where(jnp.abs(tok) < -1.0, tok, ur)
                        pr = ur * hr - ui * hi
                        pi = ur * hi + ui * hr
                        zr = pr if zr is None else zr + pr
                        zi = pi if zi is None else zi + pi
                    tok = zr if CHAIN else None
                    slabs.append(jnp.concatenate([zr, zi], axis=1))
                ws.append(jnp.concatenate(slabs, axis=0).astype(BF16))
            ys = jnp.dot(jnp.concatenate(ws, axis=0), inv_ref[...], preferred_element_type=F32)
            for t, a in enumerate(todo):
                cols = slice(a * C, (a + 1) * C)
                y = ys[t * G:(t + 1) * G] + st["kv"][a].astype(F32) * coef[KS, rows, :]
                aT[rows, cols] = _b(aq[roww, cols]).astype(F32) * y

        ops = {FWD_AT: forward}
        for step, todo in INV_SCHED.items():
            ops[step] = functools.partial(inverse, todo)
        return ops

    def head(h, carry):
        @pl.when(h == 1)
        def _():
            for c in late:
                c.wait()

        extra = conv_ops(jnp.minimum(h, NG - 1)) if CONV else {}
        wo = _b(woT[h])
        krow = jax.lax.broadcasted_iota(jnp.int32, (TQ, TQ), 0)
        qcol = jax.lax.broadcasted_iota(jnp.int32, (TQ, TQ), 1)
        causal = krow <= qcol

        def kproj(c):
            r = slice(c * TQ // 2, (c + 1) * TQ // 2)
            w = D // KSPL
            for t in range(KSPL):
                ks[r, t * w:(t + 1) * w] = _w(jnp.dot(_b(ckv[r, :]), _b(wks[:, t * w:(t + 1) * w]),
                                                      preferred_element_type=F32).astype(BF16))

        def vproj(c):
            r = slice(c * TQ // 2, (c + 1) * TQ // 2)
            w = D // VSPL // 2
            for t in range(VSPL):
                vTs[t * w:(t + 1) * w, c * TQ:(c + 1) * TQ] = _w(jax.lax.dot_general(
                    _b(wvs[t * w:(t + 1) * w, :]), _b(ckv[r, :]), NT, preferred_element_type=F32).astype(BF16))

        def qk(i):
            n = TQ * (i + 1)
            return jnp.dot(_b(ks[:n // 2, :]), _b(qs[h, :, TQ * i:n]), preferred_element_type=F32)

        def softmax(i, sT):
            n = TQ * (i + 1)
            blocks = [sT[c0:c0 + TQ] for c0 in range(0, n - TQ, TQ)] + [jnp.where(causal, sT[n - TQ:], NEG)]
            m8 = None
            for blk in blocks:
                bm = jnp.max(blk.reshape(TQ // 8, 8, TQ), axis=0)
                m8 = bm if m8 is None else jnp.where(bm > m8, bm, m8)
            m8 = jnp.broadcast_to(jnp.max(m8, axis=0, keepdims=True), (8, TQ))
            ls, p, ps = None, None, []
            for blk in blocks:
                if p is None:
                    mm = m8
                else:
                    tk = p[TQ - 8 * TOK:TQ - 8 * TOK + 8]
                    mm = jnp.where(tk < 0.0, tk, m8)
                p = jnp.exp2(blk - jnp.concatenate([mm] * (TQ // 8), axis=0))
                part = jnp.sum(p.reshape(TQ // 8, 8, TQ), axis=0)
                ls = part if ls is None else ls + part
                ps.append(p)
            l = jnp.sum(ls, axis=0, keepdims=True)
            return jnp.concatenate(ps, axis=0).astype(BF16), 1.0 / l

        ctx = {}

        def pv(i, p, rl):
            n = TQ * (i + 1)
            w = D // PSPL // 2
            parts = []
            for t in range(PSPL):
                ctxT = jnp.dot(_b(vTs[t * w:(t + 1) * w, :n]), p, preferred_element_type=F32) * rl
                if CSSA:
                    parts.append(ctxT)
                else:
                    cs[t * w:(t + 1) * w, TQ * i:n] = _w(ctxT.astype(BF16))
            if CSSA:
                ctx[i] = jnp.concatenate(parts, axis=0).astype(BF16)

        def oproj(i0, i1):
            if CSSA:
                for i in range(i0, i1):
                    acc[:, TQ * i:TQ * (i + 1)] += jnp.dot(wo, ctx[i], preferred_element_type=F32)
            else:
                cols = slice(TQ * i0, TQ * i1)
                acc[:, cols] += jnp.dot(wo, _b(cs[:, cols]), preferred_element_type=F32)

        s_prev = None
        if KAHEAD:
            kproj(0)
        for i in range(NQ):
            if not KAHEAD:
                kproj(i)
            elif i + 1 < NQ:
                kproj(i + 1)
            if i > 0:
                sm = softmax(i - 1, s_prev)
            s_prev = qk(i)
            vproj(i)
            if i in extra:
                extra[i]()
            if i > 0:
                pv(i - 1, *sm)
        prep_wkv(jnp.minimum(h + 1, H - 1))
        sm = softmax(NQ - 1, s_prev)
        oproj(0, NQ // 2)
        pv(NQ - 1, *sm)
        oproj(NQ // 2, NQ - 1)
        oproj(NQ - 1, NQ)
        return carry

    jax.lax.fori_loop(0, NHEADS, head, 0)

    TO = 256
    outc = []
    for i in range(S // TO):
        cols = slice(i * TO, (i + 1) * TO)
        blk = jnp.concatenate([aT[:, cols], acc[:, cols]], axis=0)
        outs[cols, :] = blk.T.astype(BF16)
        c = cp(outs.at[cols, :], out_hbm.at[cols, :])
        c.start()
        outc.append(c)
    for c in outc:
        c.wait()


@jax.jit
def pallas_concat_heads__ssm_conv_h3__compressed_kv_cla__prompt_kernel(
    A_q: jax.Array,
    A_k: jax.Array,
    A_v: jax.Array,
    A_shift_k: jax.Array,
    A_ssm_k: jax.Array,
    A_ssm_D: jax.Array,
    B_x: jax.Array,
    B_c_kv: jax.Array,
    B_w_q: jax.Array,
    B_w_uk: jax.Array,
    B_w_uv: jax.Array,
    B_w_o: jax.Array,
):
    fwd, inv = _dft_mats()
    tr = lambda a: jnp.swapaxes(a, 1, 2).reshape(DA, S)
    any_spec = pl.BlockSpec(memory_space=pl.ANY)
    vmem_spec = pl.BlockSpec(memory_space=pltpu.VMEM)
    out = pl.pallas_call(
        _kernel,
        out_shape=jax.ShapeDtypeStruct((S, 2 * DA), BF16),
        in_specs=[any_spec, any_spec, any_spec, vmem_spec, any_spec, vmem_spec, any_spec, any_spec, any_spec,
                  any_spec, any_spec, any_spec, vmem_spec, vmem_spec],
        out_specs=any_spec,
        scratch_shapes=[
            pltpu.VMEM((DA // 2, S), U32),
            pltpu.VMEM((DA // 2, S), U32),
            pltpu.VMEM((DA // 2, S), U32),
            pltpu.VMEM((DA // 2, S), U32),
            pltpu.VMEM((DA // 2, S), U32),
            pltpu.VMEM((S // 2, DC), U32),
            pltpu.VMEM((H // 2, DA, D), U32),
            pltpu.VMEM((H // 2, DC, D), U32),
            pltpu.VMEM((H // 2, DC, D), U32),
            pltpu.VMEM((H, DA // 2, D), U32),
            pltpu.VMEM((D, DA), U32),
            pltpu.VMEM((H, D // 2, S), U32),
            pltpu.VMEM((S // 2, D), U32),
            pltpu.VMEM((D // 2, S), U32),
            pltpu.VMEM((D // 2, S), U32),
            pltpu.VMEM((DA, S), F32),
            pltpu.VMEM((DA, S), F32),
            pltpu.VMEM((KS + 1, DA, 128), F32),
            pltpu.VMEM((DC // 2, D), U32),
            pltpu.VMEM((D // 2, DC), U32),
            pltpu.VMEM((S, 2 * DA), BF16),
            pltpu.SemaphoreType.DMA((NSEM,)),
        ],
        compiler_params=pltpu.CompilerParams(vmem_limit_bytes=100 * 1024 * 1024),
    )(
        tr(A_q), tr(A_k), tr(A_v), A_shift_k.T, A_ssm_k, A_ssm_D, tr(B_x), B_c_kv.reshape(S, DC),
        B_w_q, B_w_uk, B_w_uv,
        jnp.swapaxes(B_w_o, 1, 2), jnp.asarray(fwd, BF16), jnp.asarray(inv, BF16),
    )
    return out.reshape(1, S, 2 * DA)
```

```python
import functools
import math

import jax
import jax.numpy as jnp
import numpy as np
import jax.experimental.pallas as pl
import jax.experimental.pallas.tpu as pltpu

F32 = jnp.float32
BF16 = jnp.bfloat16
U32 = jnp.uint32

S = 2048
DA = 448
H = 16
D = 256
DC = 1024
KS = 4
C = 128
NCH = S // C
G = 32
NG = DA // G
TQ = 128
NQ = S // TQ
NT = (((1,), (1,)), ((), ()))
NSEM = 3 * (H // 2) + 7 + 12 + 16 + 8
LOG2E = math.log2(math.e)
QSCALE = (D ** -0.5) * LOG2E
NEG = -1e9 * LOG2E

NHEADS = H
CONV = 1
KSPL = 1
VSPL = 2
PSPL = 2
KAHEAD = 1
CSSA = 1
ATR_AT = 15
OSPLIT = 8
OUT_CHUNKS = [(0, 3), (3, 7), (7, 11), (11, 16)]
X_CHUNKS = [(0, 512), (512, 1024), (1024, 2048)]
SLAB = 8
CHAIN = 1
TOK = 1
FWD_AT = 2
INV_SCHED = {4: [0, 1, 2, 3], 5: [4, 5], 6: [6], 7: [7], 8: [8], 9: [9], 10: [10], 11: [11], 12: [12], 13: [13], 14: [14], 15: [15]}


def _dft_mats():
    k = np.concatenate([np.arange(0, C, 2), np.arange(1, C, 2)]).astype(np.float64)
    n = np.arange(C, dtype=np.float64)
    th = 2.0 * np.pi * np.outer(n, k + 0.5) / (2 * C)
    fwd = np.concatenate([np.cos(th), np.sin(th)], axis=1)
    inv = fwd.T / C
    return fwd, inv


def _b(x):
    return pltpu.bitcast(x, BF16)


def _w(x):
    return pltpu.bitcast(x, U32)


def _kernel(qT_hbm, kT_hbm, vT_hbm, shT_hbm, ssm_hbm, dvec_hbm, xT_hbm, ckv_hbm, wq_hbm, wuk_hbm, wuv_hbm,
            woT_hbm, fwd_hbm, inv_hbm,
            out_hbm,
            aq, ak, av, ssm, xT, ckv, wq, wuk, wuv, woT, wqs, qs, ks, vTs, cs, acc, aT, coef, wks, wvs,
            outs, shT_ref, dvec_ref, fwd_ref, inv_ref, sems):
    sem_ids = iter(range(NSEM))

    def cp(src, dst):
        return pltpu.make_async_copy(src, dst, sems.at[next(sem_ids)])

    wq_u, wuk_u, wuv_u = wq_hbm.bitcast(U32), wuk_hbm.bitcast(U32), wuv_hbm.bitcast(U32)
    c_wq = [cp(wq_u.at[:, j, :], wq.at[j]) for j in range(H // 2)]
    c_wuk = [cp(wuk_u.at[:, j, :], wuk.at[j]) for j in range(H // 2)]
    c_wuv = [cp(wuv_u.at[:, j, :], wuv.at[j]) for j in range(H // 2)]
    x_u = xT_hbm.bitcast(U32)
    c_x = [cp(x_u.at[:, c0:c1], xT.at[:, c0:c1]) for c0, c1 in X_CHUNKS]
    c_ak, c_av = cp(kT_hbm.bitcast(U32), ak), cp(vT_hbm.bitcast(U32), av)
    c_ssm, c_aq = cp(ssm_hbm.bitcast(U32), ssm), cp(qT_hbm.bitcast(U32), aq)
    c_ckv = cp(ckv_hbm.bitcast(U32), ckv)
    c_wo = cp(woT_hbm.bitcast(U32), woT)
    small = [cp(shT_hbm, shT_ref), cp(dvec_hbm, dvec_ref), cp(fwd_hbm.bitcast(U32), fwd_ref),
             cp(inv_hbm.bitcast(U32), inv_ref)]
    early = [*small, c_wuk[0], c_wuv[0], c_ckv, c_wo, c_ak, c_av, c_ssm, c_aq]
    late = [c for j in range(1, H // 2) for c in (c_wuk[j], c_wuv[j])]
    for c in [c_wq[0], *c_x, *c_wq[1:], *early, *late]:
        c.start()

    hi_mask = jnp.uint32(0xFFFF0000)

    def prep_wq(j):
        w = wq[j]
        wqs[:D // 2, :] = _w(pltpu.bitcast(w << 16, F32).T.astype(BF16))
        wqs[D // 2:, :] = _w(pltpu.bitcast(w & hi_mask, F32).T.astype(BF16))

    def prep_wkv(h):
        j = h >> 1
        sh = jnp.asarray(16 - 16 * (h & 1), U32)
        wks[...] = _w(pltpu.bitcast((wuk[j] << sh) & hi_mask, F32).astype(BF16))
        wvs[...] = _w(pltpu.bitcast((wuv[j] << sh) & hi_mask, F32).T.astype(BF16))

    def qproj(j, c0, c1):
        q2 = (jnp.dot(_b(wqs[...]), _b(xT[:, c0:c1]), preferred_element_type=F32) * QSCALE).astype(BF16)
        qs[2 * j, :, c0:c1] = _w(q2[:D])
        qs[2 * j + 1, :, c0:c1] = _w(q2[D:])

    acc[...] = jnp.zeros(acc.shape, F32)
    aT[:128, :] = jnp.zeros((128, S), F32)

    c_wq[0].wait()
    prep_wq(0)
    for t, (c0, c1) in enumerate(X_CHUNKS):
        c_x[t].wait()
        if t == len(X_CHUNKS) - 1:
            c_wq[1].wait()
        qproj(0, c0, c1)
    prep_wq(1)

    def qpair(j, carry):
        pltpu.make_async_copy(wq_u.at[:, j + 1, :], wq.at[j + 1], sems.at[j + 1]).wait()
        qproj(j, 0, S)
        prep_wq(j + 1)
        return carry

    jax.lax.fori_loop(1, H // 2 - 1, qpair, 0)

    for c in early:
        c.wait()
    qproj(H // 2 - 1, 0, S)
    prep_wkv(0)
    cf = jnp.concatenate([shT_ref[...].astype(F32), dvec_ref[...].astype(F32)[None, :],
                          jnp.zeros((3, DA), F32)], axis=0).T
    for j in range(KS + 1):
        coef[j] = jnp.broadcast_to(cf[:, j:j + 1], (DA, 128))

    out_u = out_hbm.bitcast(U32)
    NA = 3 * 128
    sem_a = next(sem_ids)
    for _ in range(11):
        next(sem_ids)

    def a_piece(p):
        r = pl.ds(pl.multiple_of((p & 3) * (S // 8), S // 8), S // 8)
        c = pl.ds(pl.multiple_of((p >> 2) * 128, 128), 128)
        return r, c

    def a_copy(p):
        r, c = a_piece(p)
        return pltpu.make_async_copy(outs.at[r, c], out_u.at[r, c], sems.at[sem_a + p])

    def a_transpose(p):
        blk = aT[pl.ds(pl.multiple_of((p >> 2) * 128, 128), 128), pl.ds(pl.multiple_of((p & 3) * (S // 4), S // 4), S // 4)]
        r, c = a_piece(p)
        outs[r, c] = _w(_b(_w(blk.astype(BF16))).T)

    hc = C // 2

    def conv_ops(g):
        rows = pl.ds(pl.multiple_of(g * G, G), G)
        roww = pl.ds(pl.multiple_of(g * (G // 2), G // 2), G // 2)
        lane = jax.lax.broadcasted_iota(jnp.int32, (G, C), 1)
        st = {}

        def forward():
            kvs, kprev = [], None
            for c in range(NCH):
                cols = slice(c * C, (c + 1) * C)
                kf = _b(ak[roww, cols]).astype(F32)
                ksh = kf * coef[0, rows, :]
                rolled = []
                for j in range(1, KS):
                    r = pltpu.roll(kf, j, 1)
                    rolled.append(r)
                    ksh = ksh + jnp.where(lane >= j, r, 0.0 if kprev is None else kprev[j - 1]) * coef[j, rows, :]
                kvs.append((ksh * _b(av[roww, cols]).astype(F32)).astype(BF16))
                kprev = rolled
            st["kv"] = kvs
            lhs = jnp.concatenate(kvs + [_b(ssm[roww, c * C:(c + 1) * C]) for c in range(NCH)], axis=0)
            both = jnp.dot(lhs, _b(fwd_ref[...]), preferred_element_type=F32)
            xh = [both[c * G:(c + 1) * G] for c in range(NCH)]
            st["h"] = [both[(NCH + c) * G:(NCH + c + 1) * G] for c in range(NCH)]
            st["u"] = [xh[0]] + [
                xh[c] + jnp.concatenate([xh[c - 1][:, 2 * hc:3 * hc], -xh[c - 1][:, 3 * hc:], -xh[c - 1][:, :hc],
                                         xh[c - 1][:, hc:2 * hc]], axis=1) for c in range(1, NCH)]

        def inverse(todo):
            ws, tok = [], None
            for a in todo:
                slabs = []
                for r0 in range(0, G, SLAB):
                    rs = slice(r0, r0 + SLAB)
                    zr = zi = None
                    for c in range(a + 1):
                        ur, ui = st["u"][c][rs, :C], st["u"][c][rs, C:]
                        hr, hi = st["h"][a - c][rs, :C], st["h"][a - c][rs, C:]
                        if zr is None and tok is not None:
                            ur = jnp.where(jnp.abs(tok) < -1.0, tok, ur)
                        pr = ur * hr - ui * hi
                        pi = ur * hi + ui * hr
                        zr = pr if zr is None else zr + pr
                        zi = pi if zi is None else zi + pi
                    tok = zr if CHAIN else None
                    slabs.append(jnp.concatenate([zr, zi], axis=1))
                ws.append(jnp.concatenate(slabs, axis=0).astype(BF16))
            ys = jnp.dot(jnp.concatenate(ws, axis=0), _b(inv_ref[...]), preferred_element_type=F32)
            for t, a in enumerate(todo):
                cols = slice(a * C, (a + 1) * C)
                y = ys[t * G:(t + 1) * G] + st["kv"][a].astype(F32) * coef[KS, rows, :]
                aT[rows, cols] = _b(aq[roww, cols]).astype(F32) * y

        ops = {FWD_AT: forward}
        for step, todo in INV_SCHED.items():
            ops[step] = functools.partial(inverse, todo)
        return ops

    def head(h, carry):
        @pl.when(h == 1)
        def _():
            for c in late:
                c.wait()

        @pl.when(h >= 5)
        def _():
            a_copy(h - 5).start()

        extra = conv_ops(jnp.minimum(h, NG - 1)) if CONV else {}
        wo = _b(woT[h])
        krow = jax.lax.broadcasted_iota(jnp.int32, (TQ, TQ), 0)
        qcol = jax.lax.broadcasted_iota(jnp.int32, (TQ, TQ), 1)
        causal = krow <= qcol

        def kproj(c):
            r = slice(c * TQ // 2, (c + 1) * TQ // 2)
            w = D // KSPL
            for t in range(KSPL):
                ks[r, t * w:(t + 1) * w] = _w(jnp.dot(_b(ckv[r, :]), _b(wks[:, t * w:(t + 1) * w]),
                                                      preferred_element_type=F32).astype(BF16))

        def vproj(c):
            r = slice(c * TQ // 2, (c + 1) * TQ // 2)
            w = D // VSPL // 2
            for t in range(VSPL):
                vTs[t * w:(t + 1) * w, c * TQ:(c + 1) * TQ] = _w(jax.lax.dot_general(
                    _b(wvs[t * w:(t + 1) * w, :]), _b(ckv[r, :]), NT, preferred_element_type=F32).astype(BF16))

        def qk(i):
            n = TQ * (i + 1)
            return jnp.dot(_b(ks[:n // 2, :]), _b(qs[h, :, TQ * i:n]), preferred_element_type=F32)

        def softmax(i, sT):
            n = TQ * (i + 1)
            blocks = [sT[c0:c0 + TQ] for c0 in range(0, n - TQ, TQ)] + [jnp.where(causal, sT[n - TQ:], NEG)]
            m8 = None
            for blk in blocks:
                bm = jnp.max(blk.reshape(TQ // 8, 8, TQ), axis=0)
                m8 = bm if m8 is None else jnp.where(bm > m8, bm, m8)
            m8 = jnp.broadcast_to(jnp.max(m8, axis=0, keepdims=True), (8, TQ))
            ls, p, ps = None, None, []
            for blk in blocks:
                if p is None:
                    mm = m8
                else:
                    tk = p[TQ - 8 * TOK:TQ - 8 * TOK + 8]
                    mm = jnp.where(tk < 0.0, tk, m8)
                p = jnp.exp2(blk - jnp.concatenate([mm] * (TQ // 8), axis=0))
                part = jnp.sum(p.reshape(TQ // 8, 8, TQ), axis=0)
                ls = part if ls is None else ls + part
                ps.append(p)
            l = jnp.sum(ls, axis=0, keepdims=True)
            return jnp.concatenate(ps, axis=0).astype(BF16), 1.0 / l

        ctx = {}

        def pv(i, p, rl):
            n = TQ * (i + 1)
            w = D // PSPL // 2
            parts = []
            for t in range(PSPL):
                ctxT = jnp.dot(_b(vTs[t * w:(t + 1) * w, :n]), p, preferred_element_type=F32) * rl
                if CSSA:
                    parts.append(ctxT)
                else:
                    cs[t * w:(t + 1) * w, TQ * i:n] = _w(ctxT.astype(BF16))
            if CSSA:
                ctx[i] = jnp.concatenate(parts, axis=0).astype(BF16)

        def oproj(i0, i1):
            if CSSA:
                for i in range(i0, i1):
                    acc[:, TQ * i:TQ * (i + 1)] += jnp.dot(wo, ctx[i], preferred_element_type=F32)
            else:
                cols = slice(TQ * i0, TQ * i1)
                acc[:, cols] += jnp.dot(wo, _b(cs[:, cols]), preferred_element_type=F32)

        s_prev = None
        if KAHEAD:
            kproj(0)
        for i in range(NQ):
            if not KAHEAD:
                kproj(i)
            elif i + 1 < NQ:
                kproj(i + 1)
            if i > 0:
                sm = softmax(i - 1, s_prev)
            s_prev = qk(i)
            vproj(i)
            if i in extra:
                extra[i]()
            if i > 0:
                pv(i - 1, *sm)
            if i == ATR_AT:
                a_transpose(jnp.maximum(h - 4, 0))
        prep_wkv(jnp.minimum(h + 1, H - 1))
        sm = softmax(NQ - 1, s_prev)
        oproj(0, OSPLIT)
        pv(NQ - 1, *sm)
        oproj(OSPLIT, NQ)
        return carry

    jax.lax.fori_loop(0, NHEADS, head, 0)
    if NHEADS < 2:
        for c in late:
            c.wait()

    a_copy(11).start()
    c_out = []
    for i0, i1 in OUT_CHUNKS:
        cols, r = slice(i0 * TQ, i1 * TQ), slice(i0 * TQ // 2, i1 * TQ // 2)
        blk = jnp.concatenate([aT[NA:, cols], acc[:, cols]], axis=0).astype(BF16)
        outs[r, NA:] = _w(_b(_w(blk)).T)
        c = cp(outs.at[r, NA:], out_u.at[r, NA:])
        c.start()
        c_out.append(c)
    for p in range(12):
        a_copy(p).wait()
    for c in c_out:
        c.wait()


@jax.jit
def pallas_concat_heads__ssm_conv_h3__compressed_kv_cla__prompt_kernel(
    A_q: jax.Array,
    A_k: jax.Array,
    A_v: jax.Array,
    A_shift_k: jax.Array,
    A_ssm_k: jax.Array,
    A_ssm_D: jax.Array,
    B_x: jax.Array,
    B_c_kv: jax.Array,
    B_w_q: jax.Array,
    B_w_uk: jax.Array,
    B_w_uv: jax.Array,
    B_w_o: jax.Array,
):
    fwd, inv = _dft_mats()
    tr = lambda a: jnp.swapaxes(a, 1, 2).reshape(DA, S)
    any_spec = pl.BlockSpec(memory_space=pl.ANY)
    out = pl.pallas_call(
        _kernel,
        out_shape=jax.ShapeDtypeStruct((S, 2 * DA), BF16),
        in_specs=[any_spec] * 14,
        out_specs=any_spec,
        scratch_shapes=[
            pltpu.VMEM((DA // 2, S), U32),
            pltpu.VMEM((DA // 2, S), U32),
            pltpu.VMEM((DA // 2, S), U32),
            pltpu.VMEM((DA // 2, S), U32),
            pltpu.VMEM((DA // 2, S), U32),
            pltpu.VMEM((S // 2, DC), U32),
            pltpu.VMEM((H // 2, DA, D), U32),
            pltpu.VMEM((H // 2, DC, D), U32),
            pltpu.VMEM((H // 2, DC, D), U32),
            pltpu.VMEM((H, DA // 2, D), U32),
            pltpu.VMEM((D, DA), U32),
            pltpu.VMEM((H, D // 2, S), U32),
            pltpu.VMEM((S // 2, D), U32),
            pltpu.VMEM((D // 2, S), U32),
            pltpu.VMEM((D // 2, S), U32),
            pltpu.VMEM((DA, S), F32),
            pltpu.VMEM((DA, S), F32),
            pltpu.VMEM((KS + 1, DA, 128), F32),
            pltpu.VMEM((DC // 2, D), U32),
            pltpu.VMEM((D // 2, DC), U32),
            pltpu.VMEM((S // 2, 2 * DA), U32),
            pltpu.VMEM((KS, DA), BF16),
            pltpu.VMEM((DA,), BF16),
            pltpu.VMEM((C // 2, 2 * C), U32),
            pltpu.VMEM((C, C), U32),
            pltpu.SemaphoreType.DMA((NSEM,)),
        ],
        compiler_params=pltpu.CompilerParams(vmem_limit_bytes=100 * 1024 * 1024),
    )(
        tr(A_q), tr(A_k), tr(A_v), A_shift_k.T, A_ssm_k, A_ssm_D, tr(B_x), B_c_kv.reshape(S, DC),
        B_w_q, B_w_uk, B_w_uv,
        jnp.swapaxes(B_w_o, 1, 2), jnp.asarray(fwd, BF16), jnp.asarray(inv, BF16),
    )
    return out.reshape(1, S, 2 * DA)
```

```python
import functools
import math

import jax
import jax.numpy as jnp
import numpy as np
import jax.experimental.pallas as pl
import jax.experimental.pallas.tpu as pltpu

F32 = jnp.float32
BF16 = jnp.bfloat16
U32 = jnp.uint32

S = 2048
DA = 448
H = 16
D = 256
DC = 1024
KS = 4
C = 128
NCH = S // C
G = 32
NG = DA // G
TQ = 128
NQ = S // TQ
NT = (((1,), (1,)), ((), ()))
NSEM = 3 * (H // 2) + 7 + 12 + 16 + 8
LOG2E = math.log2(math.e)
QSCALE = (D ** -0.5) * LOG2E
NEG = -1e9 * LOG2E

NHEADS = H
CONV = 1
KSPL = 1
VSPL = 1
PSPL = 2
KAHEAD = 1
CSSA = 1
ATR_AT = 15
OSPLIT = 12
OUT_CHUNKS = [(0, 3), (3, 7), (7, 11), (11, 16)]
X_CHUNKS = [(0, 384), (384, 1152), (1152, 2048)]
ALT = 1
OFILL = {14: (0, 4), 15: (4, 8)}
PMAX = 3
NEPI = 99
NOWAIT = 0
DEFER = 1
QREP = 0
STAGE = []
PREP_AT = 99
PFENCE = 99
ZLATE = 0
SLAB = 8
CHAIN = 1
TOK = 1
FWD_AT = 3
INV_SCHED = {4: [0, 1, 2, 3], 5: [4, 5], 6: [6], 7: [7], 8: [8], 9: [9], 10: [10], 11: [11], 12: [12], 13: [13], 14: [14], 15: [15]}


def _dft_mats():
    k = np.concatenate([np.arange(0, C, 2), np.arange(1, C, 2)]).astype(np.float64)
    n = np.arange(C, dtype=np.float64)
    th = 2.0 * np.pi * np.outer(n, k + 0.5) / (2 * C)
    fwd = np.concatenate([np.cos(th), np.sin(th)], axis=1)
    inv = fwd.T / C
    return fwd, inv


def _b(x):
    return pltpu.bitcast(x, BF16)


def _w(x):
    return pltpu.bitcast(x, U32)


def _kernel(qT_hbm, kT_hbm, vT_hbm, shT_hbm, ssm_hbm, dvec_hbm, xT_hbm, ckv_hbm, wq_hbm, wuk_hbm, wuv_hbm,
            woT_hbm, fwd_hbm, inv_hbm,
            out_hbm,
            aq, ak, av, ssm, xT, ckv, wq, wuk, wuv, woT, wqs, qs, ks, vTs, cs, acc, aT, coef, wks, wvs,
            outs, shT_ref, dvec_ref, fwd_ref, inv_ref, sems):
    sem_ids = iter(range(NSEM))

    def cp(src, dst):
        return pltpu.make_async_copy(src, dst, sems.at[next(sem_ids)])

    wq_u, wuk_u, wuv_u = wq_hbm.bitcast(U32), wuk_hbm.bitcast(U32), wuv_hbm.bitcast(U32)
    c_wq = [cp(wq_u.at[:, j, :], wq.at[j]) for j in range(H // 2)]
    c_wuk = [cp(wuk_u.at[:, j, :], wuk.at[j]) for j in range(H // 2)]
    c_wuv = [cp(wuv_u.at[:, j, :], wuv.at[j]) for j in range(H // 2)]
    x_u = xT_hbm.bitcast(U32)
    c_x = [cp(x_u.at[:, c0:c1], xT.at[:, c0:c1]) for c0, c1 in X_CHUNKS]
    c_ak, c_av = cp(kT_hbm.bitcast(U32), ak), cp(vT_hbm.bitcast(U32), av)
    c_ssm, c_aq = cp(ssm_hbm.bitcast(U32), ssm), cp(qT_hbm.bitcast(U32), aq)
    c_ckv = cp(ckv_hbm.bitcast(U32), ckv)
    c_wo = cp(woT_hbm.bitcast(U32), woT)
    small = [cp(shT_hbm, shT_ref), cp(dvec_hbm, dvec_ref), cp(fwd_hbm.bitcast(U32), fwd_ref),
             cp(inv_hbm.bitcast(U32), inv_ref)]
    early = [*small, c_wuk[0], c_wuv[0], c_ckv, c_wo, c_ak, c_av, c_ssm, c_aq]
    late = [c for j in range(1, H // 2) for c in (c_wuk[j], c_wuv[j])]
    order = [c_wq[0], *c_x, *c_wq[1:], *early] + (late if not DEFER else [])
    groups = [order[a:b] for a, b in zip([0] + STAGE, STAGE + [len(order)])]
    for c in groups[0]:
        c.start()

    hi_mask = jnp.uint32(0xFFFF0000)

    def prep_wq(j):
        w = wq[j]
        wqs[:D // 2, :] = _w(pltpu.bitcast(w << 16, F32).T.astype(BF16))
        wqs[D // 2:, :] = _w(pltpu.bitcast(w & hi_mask, F32).T.astype(BF16))

    def prep_wkv(h):
        j = h >> 1
        sh = jnp.asarray(16 - 16 * (h & 1), U32)
        wks[...] = _w(pltpu.bitcast((wuk[j] << sh) & hi_mask, F32).astype(BF16))
        wvs[...] = _w(pltpu.bitcast((wuv[j] << sh) & hi_mask, F32).T.astype(BF16))

    def qproj(j, c0, c1):
        q2 = (jnp.dot(_b(wqs[...]), _b(xT[:, c0:c1]), preferred_element_type=F32) * QSCALE).astype(BF16)
        qs[2 * j, :, c0:c1] = _w(q2[:D])
        qs[2 * j + 1, :, c0:c1] = _w(q2[D:])

    def zero_init():
        acc[...] = jnp.zeros(acc.shape, F32)
        aT[:128, :] = jnp.zeros((128, S), F32)

    if not ZLATE:
        zero_init()

    if not NOWAIT:
        c_wq[0].wait()
    prep_wq(0)
    for t, (c0, c1) in enumerate(X_CHUNKS):
        if not NOWAIT:
            c_x[t].wait()
            if t == len(X_CHUNKS) - 1:
                c_wq[1].wait()
        if t + 1 < len(groups):
            for c in groups[t + 1]:
                c.start()
        qproj(0, c0, c1)
    if ZLATE:
        zero_init()
    prep_wq(1)
    if NOWAIT:
        for c in [c_wq[0], c_wq[1], *c_x]:
            c.wait()

    def qpair(j, carry):
        if QREP:
            @pl.when(j < H // 2 - 1)
            def _():
                pltpu.make_async_copy(wq_u.at[:, j + 1, :], wq.at[j + 1], sems.at[j + 1]).wait()
            j = jnp.minimum(j, H // 2 - 2)
        else:
            pltpu.make_async_copy(wq_u.at[:, j + 1, :], wq.at[j + 1], sems.at[j + 1]).wait()
        qproj(j, 0, S)
        prep_wq(j + 1)
        return carry

    jax.lax.fori_loop(1, H // 2 - 1 + QREP, qpair, 0)

    for c in early:
        c.wait()
    if DEFER:
        for c in late:
            c.start()
    qproj(H // 2 - 1, 0, S)
    prep_wkv(0)
    cf = jnp.concatenate([shT_ref[...].astype(F32), dvec_ref[...].astype(F32)[None, :],
                          jnp.zeros((3, DA), F32)], axis=0).T
    for j in range(KS + 1):
        coef[j] = jnp.broadcast_to(cf[:, j:j + 1], (DA, 128))

    NA = 3 * 128
    sem_a = next(sem_ids)
    for _ in range(11):
        next(sem_ids)

    def a_piece(p):
        r = pl.ds(pl.multiple_of((p & 3) * (S // 4), S // 4), S // 4)
        c = pl.ds(pl.multiple_of((p >> 2) * 128, 128), 128)
        return r, c

    def a_copy(p):
        r, c = a_piece(p)
        return pltpu.make_async_copy(outs.at[r, c], out_hbm.at[r, c], sems.at[sem_a + p])

    def a_transpose(p):
        r, c = a_piece(p)
        outs[r, c] = _b(_w(aT[c, r].astype(BF16))).T

    hc = C // 2

    def conv_ops(g):
        rows = pl.ds(pl.multiple_of(g * G, G), G)
        roww = pl.ds(pl.multiple_of(g * (G // 2), G // 2), G // 2)
        lane = jax.lax.broadcasted_iota(jnp.int32, (G, C), 1)
        st = {}

        def forward():
            kvs, kprev = [], None
            for c in range(NCH):
                cols = slice(c * C, (c + 1) * C)
                kf = _b(ak[roww, cols]).astype(F32)
                ksh = kf * coef[0, rows, :]
                rolled = []
                for j in range(1, KS):
                    r = pltpu.roll(kf, j, 1)
                    rolled.append(r)
                    ksh = ksh + jnp.where(lane >= j, r, 0.0 if kprev is None else kprev[j - 1]) * coef[j, rows, :]
                kvs.append((ksh * _b(av[roww, cols]).astype(F32)).astype(BF16))
                kprev = rolled
            st["kv"] = kvs
            lhs = jnp.concatenate(kvs + [_b(ssm[roww, c * C:(c + 1) * C]) for c in range(NCH)], axis=0)
            both = jnp.dot(lhs, _b(fwd_ref[...]), preferred_element_type=F32)
            xh = [both[c * G:(c + 1) * G] for c in range(NCH)]
            st["h"] = [both[(NCH + c) * G:(NCH + c + 1) * G] for c in range(NCH)]
            st["u"] = [xh[0]] + [
                xh[c] + jnp.concatenate([xh[c - 1][:, 2 * hc:3 * hc], -xh[c - 1][:, 3 * hc:], -xh[c - 1][:, :hc],
                                         xh[c - 1][:, hc:2 * hc]], axis=1) for c in range(1, NCH)]

        def inverse(todo):
            ws, tok = [], None
            for a in todo:
                slabs = []
                for r0 in range(0, G, SLAB):
                    rs = slice(r0, r0 + SLAB)
                    zr = zi = None
                    for c in range(a + 1):
                        ur, ui = st["u"][c][rs, :C], st["u"][c][rs, C:]
                        hr, hi = st["h"][a - c][rs, :C], st["h"][a - c][rs, C:]
                        if zr is None and tok is not None:
                            ur = jnp.where(jnp.abs(tok) < -1.0, tok, ur)
                        pr = ur * hr - ui * hi
                        pi = ur * hi + ui * hr
                        zr = pr if zr is None else zr + pr
                        zi = pi if zi is None else zi + pi
                    tok = zr if CHAIN else None
                    slabs.append(jnp.concatenate([zr, zi], axis=1))
                ws.append(jnp.concatenate(slabs, axis=0).astype(BF16))
            ys = jnp.dot(jnp.concatenate(ws, axis=0), _b(inv_ref[...]), preferred_element_type=F32)
            for t, a in enumerate(todo):
                cols = slice(a * C, (a + 1) * C)
                y = ys[t * G:(t + 1) * G] + st["kv"][a].astype(F32) * coef[KS, rows, :]
                aT[rows, cols] = _b(aq[roww, cols]).astype(F32) * y

        ops = {FWD_AT: forward}
        for step, todo in INV_SCHED.items():
            ops[step] = functools.partial(inverse, todo)
        return ops

    def head(h, carry):
        @pl.when(h == 1)
        def _():
            for c in late:
                c.wait()

        @pl.when(h >= 5)
        def _():
            a_copy(h - 5).start()

        extra = conv_ops(jnp.minimum(h, NG - 1)) if CONV else {}
        wo = _b(woT[h])
        krow = jax.lax.broadcasted_iota(jnp.int32, (TQ, TQ), 0)
        qcol = jax.lax.broadcasted_iota(jnp.int32, (TQ, TQ), 1)
        causal = krow <= qcol

        def kproj(c, KC=TQ):
            r = slice(c * KC // 2, (c + 1) * KC // 2)
            w = D // KSPL
            for t in range(KSPL):
                ks[r, t * w:(t + 1) * w] = _w(jnp.dot(_b(ckv[r, :]), _b(wks[:, t * w:(t + 1) * w]),
                                                      preferred_element_type=F32).astype(BF16))

        def vproj(c, KC=TQ):
            r = slice(c * KC // 2, (c + 1) * KC // 2)
            w = D // VSPL // 2
            for t in range(VSPL):
                vTs[t * w:(t + 1) * w, c * KC:(c + 1) * KC] = _w(jax.lax.dot_general(
                    _b(wvs[t * w:(t + 1) * w, :]), _b(ckv[r, :]), NT, preferred_element_type=F32).astype(BF16))

        def qk(i):
            n = TQ * (i + 1)
            return jnp.dot(_b(ks[:n // 2, :]), _b(qs[h, :, TQ * i:n]), preferred_element_type=F32)

        def blockmax(i, sT):
            n = TQ * (i + 1)
            blocks = [sT[c0:c0 + TQ] for c0 in range(0, n - TQ, TQ)] + [jnp.where(causal, sT[n - TQ:], NEG)]
            m8, part = None, None
            for b, blk in enumerate(blocks):
                bm = jnp.max(blk.reshape(TQ // 8, 8, TQ), axis=0)
                m8 = bm if m8 is None else jnp.where(bm > m8, bm, m8)
                if b == i - PMAX:
                    part = m8[0:1]
            return blocks, m8, part

        def softmax(i, st):
            blocks, m8, _ = st
            m8 = jnp.broadcast_to(jnp.max(m8, axis=0, keepdims=True), (8, TQ))
            ls, p, ps = None, None, []
            for blk in blocks:
                if p is None:
                    mm = m8
                else:
                    tk = p[TQ - 8 * TOK:TQ - 8 * TOK + 8]
                    mm = jnp.where(tk < 0.0, tk, m8)
                p = jnp.exp2(blk - jnp.concatenate([mm] * (TQ // 8), axis=0))
                part = jnp.sum(p.reshape(TQ // 8, 8, TQ), axis=0)
                ls = part if ls is None else ls + part
                ps.append(p)
            l = jnp.sum(ls, axis=0, keepdims=True)
            return jnp.concatenate(ps, axis=0).astype(BF16), 1.0 / l

        ctx = {}

        def pv(i, p, rl):
            n = TQ * (i + 1)
            w = D // PSPL // 2
            parts = []
            for t in range(PSPL):
                ctxT = jnp.dot(_b(vTs[t * w:(t + 1) * w, :n]), p, preferred_element_type=F32) * rl
                if CSSA:
                    parts.append(ctxT)
                else:
                    cs[t * w:(t + 1) * w, TQ * i:n] = _w(ctxT.astype(BF16))
            if CSSA:
                ctx[i] = jnp.concatenate(parts, axis=0).astype(BF16)

        def oproj(i0, i1):
            if CSSA:
                for i in range(i0, i1):
                    acc[:, TQ * i:TQ * (i + 1)] += jnp.dot(wo, ctx[i], preferred_element_type=F32)
            else:
                cols = slice(TQ * i0, TQ * i1)
                acc[:, cols] += jnp.dot(wo, _b(cs[:, cols]), preferred_element_type=F32)

        s_prev = None
        if ALT == 1:
            kproj(0, 2 * TQ)
            vproj(0, 2 * TQ)
        elif ALT == 2:
            kproj(0, 2 * TQ)
        else:
            kproj(0)
        for i in range(NQ):
            if ALT == 1:
                if i + 2 < NQ:
                    (vproj if i & 1 else kproj)(i // 2 + 1, 2 * TQ)
                if i in OFILL:
                    oproj(*OFILL[i])
            elif ALT == 2:
                if i + 2 < NQ and i % 2 == 0:
                    kproj(i // 2 + 1, 2 * TQ)
            elif i + 1 < NQ:
                kproj(i + 1)
            if i > 0:
                sm = softmax(i - 1, s_prev)
            s_prev = blockmax(i, qk(i))
            if PMAX and i > 0 and s_prev[2] is not None:
                sm = (sm[0], jnp.where(jnp.abs(s_prev[2]) < -1.0, s_prev[2], sm[1]))
            if ALT != 1:
                vproj(i)
            if i in extra:
                extra[i]()
            if i == PREP_AT:
                prep_wkv(jnp.minimum(h + 1, H - 1))
            if i == PFENCE:
                r = pl.ds(pl.multiple_of(h * 8, 8), 8)
                c = pl.ds(pl.multiple_of((h & 1) * 128, 128), 128)
                tok = (wks[r, c] | wvs[r, c])[0:1] >> 31
                sm = (sm[0], jnp.where(tok > 1, 0.0, sm[1]))
            if i > 0:
                pv(i - 1, *sm)
            if i == ATR_AT:
                a_transpose(jnp.maximum(h - 4, 0))
        if PREP_AT >= NQ:
            prep_wkv(jnp.minimum(h + 1, H - 1))
        sm = softmax(NQ - 1, s_prev)
        oproj(max([0] + [e for _, e in OFILL.values()]), OSPLIT)
        pv(NQ - 1, *sm)
        oproj(OSPLIT, NQ)
        return carry

    jax.lax.fori_loop(0, NHEADS, head, 0)
    if NHEADS < 2:
        for c in late:
            c.wait()

    for p in range(max(NHEADS - 5, 0), 12):
        a_copy(p).start()
    c_out = []
    for i0, i1 in OUT_CHUNKS[:NEPI]:
        cols = slice(i0 * TQ, i1 * TQ)
        blk = jnp.concatenate([aT[NA:, cols], acc[:, cols]], axis=0).astype(BF16)
        outs[cols, NA:] = _b(_w(blk)).T
        c = cp(outs.at[cols, NA:], out_hbm.at[cols, NA:])
        c.start()
        c_out.append(c)
    for p in range(12):
        a_copy(p).wait()
    for c in c_out:
        c.wait()


@jax.jit
def pallas_concat_heads__ssm_conv_h3__compressed_kv_cla__prompt_kernel(
    A_q: jax.Array,
    A_k: jax.Array,
    A_v: jax.Array,
    A_shift_k: jax.Array,
    A_ssm_k: jax.Array,
    A_ssm_D: jax.Array,
    B_x: jax.Array,
    B_c_kv: jax.Array,
    B_w_q: jax.Array,
    B_w_uk: jax.Array,
    B_w_uv: jax.Array,
    B_w_o: jax.Array,
):
    fwd, inv = _dft_mats()
    tr = lambda a: jnp.swapaxes(a, 1, 2).reshape(DA, S)
    any_spec = pl.BlockSpec(memory_space=pl.ANY)
    out = pl.pallas_call(
        _kernel,
        out_shape=jax.ShapeDtypeStruct((S, 2 * DA), BF16),
        in_specs=[any_spec] * 14,
        out_specs=any_spec,
        scratch_shapes=[
            pltpu.VMEM((DA // 2, S), U32),
            pltpu.VMEM((DA // 2, S), U32),
            pltpu.VMEM((DA // 2, S), U32),
            pltpu.VMEM((DA // 2, S), U32),
            pltpu.VMEM((DA // 2, S), U32),
            pltpu.VMEM((S // 2, DC), U32),
            pltpu.VMEM((H // 2, DA, D), U32),
            pltpu.VMEM((H // 2, DC, D), U32),
            pltpu.VMEM((H // 2, DC, D), U32),
            pltpu.VMEM((H, DA // 2, D), U32),
            pltpu.VMEM((D, DA), U32),
            pltpu.VMEM((H, D // 2, S), U32),
            pltpu.VMEM((S // 2, D), U32),
            pltpu.VMEM((D // 2, S), U32),
            pltpu.VMEM((D // 2, S), U32),
            pltpu.VMEM((DA, S), F32),
            pltpu.VMEM((DA, S), F32),
            pltpu.VMEM((KS + 1, DA, 128), F32),
            pltpu.VMEM((DC // 2, D), U32),
            pltpu.VMEM((D // 2, DC), U32),
            pltpu.VMEM((S, 2 * DA), BF16),
            pltpu.VMEM((KS, DA), BF16),
            pltpu.VMEM((DA,), BF16),
            pltpu.VMEM((C // 2, 2 * C), U32),
            pltpu.VMEM((C, C), U32),
            pltpu.SemaphoreType.DMA((NSEM,)),
        ],
        compiler_params=pltpu.CompilerParams(vmem_limit_bytes=100 * 1024 * 1024),
    )(
        tr(A_q), tr(A_k), tr(A_v), A_shift_k.T, A_ssm_k, A_ssm_D, tr(B_x), B_c_kv.reshape(S, DC),
        B_w_q, B_w_uk, B_w_uv,
        jnp.swapaxes(B_w_o, 1, 2), jnp.asarray(fwd, BF16), jnp.asarray(inv, BF16),
    )
    return out.reshape(1, S, 2 * DA)
```

```python
import contextlib
import functools
import math

import jax
import jax.numpy as jnp
import numpy as np
import jax.experimental.pallas as pl
import jax.experimental.pallas.tpu as pltpu

F32 = jnp.float32
BF16 = jnp.bfloat16
U32 = jnp.uint32

S = 2048
DA = 448
H = 16
D = 256
DC = 1024
KS = 4
C = 128
NCH = S // C
G = 32
NG = DA // G
TQ = 128
NQ = S // TQ
KC = 256
NA = 384
NT = (((1,), (1,)), ((), ()))
LOG2E = math.log2(math.e)
QSCALE = (D ** -0.5) * LOG2E
NEG = -1e9 * LOG2E

X_CHUNKS = [(0, 384), (384, 1152), (1152, 2048)]
OUT_CHUNKS = [(0, 3), (3, 7), (7, 11), (11, 16)]
FWD_AT = 3
INV_AT = {4: [0, 1, 2, 3], 5: [4, 5], 6: [6], 7: [7], 8: [8], 9: [9], 10: [10], 11: [11], 12: [12], 13: [13], 14: [14], 15: [15]}
OFILL = {14: (0, 4), 15: (4, 8)}
OSPLIT = 12
PRE = 0
PMAX = 3
SCOPES = 0


def _scope(name):
    return jax.named_scope(name) if SCOPES else contextlib.nullcontext()


def _dft_mats():
    k = np.concatenate([np.arange(0, C, 2), np.arange(1, C, 2)]).astype(np.float64)
    n = np.arange(C, dtype=np.float64)
    th = 2.0 * np.pi * np.outer(n, k + 0.5) / (2 * C)
    fwd = np.concatenate([np.cos(th), np.sin(th)], axis=1)
    inv = fwd.T / C
    return fwd, inv


def _b(x):
    return pltpu.bitcast(x, BF16)


def _w(x):
    return pltpu.bitcast(x, U32)


def _dot(a, b):
    return jnp.dot(a, b, preferred_element_type=F32)


def _after(tok, x):
    return jnp.where(jnp.abs(tok) < -1.0, tok, x)


def _kernel(qT_hbm, kT_hbm, vT_hbm, shT_hbm, ssm_hbm, dvec_hbm, xT_hbm, ckv_hbm, wq_hbm, wuk_hbm, wuv_hbm,
            woT_hbm, fwd_hbm, inv_hbm,
            out_hbm,
            aq, ak, av, ssm, xT, ckv, wq, wkv, woT, wqs, qs, ks, vTs, acc, aT, coef, wks, wvs,
            outs, shT, dvec, fwd, inv, sems):
    def cp(src, dst, sem):
        return pltpu.make_async_copy(src, dst, sems.at[sem])

    s_wq0, s_x, s_wq, s_early, s_late, s_out = 0, 1, 4, 5, 6, 7
    wq_u, wuk_u, wuv_u, x_u = (r.bitcast(U32) for r in (wq_hbm, wuk_hbm, wuv_hbm, xT_hbm))
    c_wq0 = cp(wq_u.at[:, 0, :], wq.at[0], s_wq0)
    c_x = [[cp(x_u.at[:, c0:c1], xT.at[:, c0:c1], s_x + t)] for t, (c0, c1) in enumerate(X_CHUNKS)]
    c_x[-1] += [cp(wq_u.at[:, j, :], wq.at[j], s_x + 2) for j in (1, 2)]
    c_wq = [cp(wq_u.at[:, j, :], wq.at[j], s_wq) for j in range(3, H // 2)]
    early = [cp(src, dst, s_early) for src, dst in (
        (shT_hbm, shT), (dvec_hbm, dvec), (fwd_hbm.bitcast(U32), fwd), (inv_hbm.bitcast(U32), inv),
        (wuk_u.at[:, 0, :], wkv.at[0, 0]), (wuv_u.at[:, 0, :], wkv.at[0, 1]), (ckv_hbm.bitcast(U32), ckv),
        (woT_hbm.bitcast(U32), woT), (kT_hbm.bitcast(U32), ak), (vT_hbm.bitcast(U32), av),
        (ssm_hbm.bitcast(U32), ssm), (qT_hbm.bitcast(U32), aq))]
    late = [cp(src.at[:, j, :], wkv.at[j, t], s_late)
            for j in range(1, H // 2) for t, src in enumerate((wuk_u, wuv_u))]
    for c in [c_wq0, *c_x[0], *c_x[1], *c_x[2], *c_wq, *early, *late]:
        c.start()

    hi_mask = jnp.uint32(0xFFFF0000)

    def prep_wq(j):
        w = wq[j]
        wqs[:D // 2, :] = _w(pltpu.bitcast(w << 16, F32).T.astype(BF16))
        wqs[D // 2:, :] = _w(pltpu.bitcast(w & hi_mask, F32).T.astype(BF16))

    def prep_wkv(h):
        j = h >> 1
        sh = jnp.asarray(16 - 16 * (h & 1), U32)
        wks[...] = _w(pltpu.bitcast((wkv[j, 0] << sh) & hi_mask, F32).astype(BF16))
        wvs[...] = _w(pltpu.bitcast((wkv[j, 1] << sh) & hi_mask, F32).T.astype(BF16))

    def qproj(j, c0, c1):
        q2 = (_dot(_b(wqs[...]), _b(xT[:, c0:c1])) * QSCALE).astype(BF16)
        qs[2 * j, :, c0:c1] = _w(q2[:D])
        qs[2 * j + 1, :, c0:c1] = _w(q2[D:])

    acc[...] = jnp.zeros(acc.shape, F32)
    aT[:128, :] = jnp.zeros((128, S), F32)
    if PRE:
        aT[NA:, :] = jnp.zeros((DA - NA, S), F32)

    c_wq0.wait()
    prep_wq(0)
    for cs, (c0, c1) in zip(c_x, X_CHUNKS):
        for c in cs:
            c.wait()
        qproj(0, c0, c1)
    prep_wq(1)

    def qpair(j, carry):
        @pl.when(j == 2)
        def _():
            cp(wq.at[3:], wq.at[3:], s_wq).wait()

        qproj(j, 0, S)
        prep_wq(j + 1)
        return carry

    with _scope("qloop"):
        jax.lax.fori_loop(1, H // 2 - 1, qpair, 0)

    for c in early:
        c.wait()
    qproj(H // 2 - 1, 0, S)
    prep_wkv(0)
    cf = jnp.concatenate([shT[...].astype(F32), dvec[...].astype(F32)[None, :],
                          jnp.zeros((3, DA), F32)], axis=0).T
    for j in range(KS + 1):
        coef[j] = jnp.broadcast_to(cf[:, j:j + 1], (DA, 128))

    def a_piece(p):
        r = pl.ds(pl.multiple_of((p & 3) * (S // 4), S // 4), S // 4)
        c = pl.ds(pl.multiple_of((p >> 2) * 128, 128), 128)
        return r, c

    def a_copy(p):
        r, c = a_piece(p)
        return cp(outs.at[r, c], out_hbm.at[r, c], s_out)

    def a_transpose(p):
        r, c = a_piece(p)
        outs[r, c] = _b(_w(aT[c, r].astype(BF16))).T

    def b_transpose(i0, i1):
        cols = slice(i0 * TQ, i1 * TQ)
        blk = jnp.concatenate([aT[NA:, cols], acc[:, cols]], axis=0).astype(BF16)
        outs[cols, NA:] = _b(_w(blk)).T

    def conv_ops(g):
        rows = pl.ds(pl.multiple_of(g * G, G), G)
        roww = pl.ds(pl.multiple_of(g * (G // 2), G // 2), G // 2)
        lane = jax.lax.broadcasted_iota(jnp.int32, (G, C), 1)
        hc = C // 2
        st = {}

        def forward():
            kvs, kprev = [], None
            for c in range(NCH):
                cols = slice(c * C, (c + 1) * C)
                kf = _b(ak[roww, cols]).astype(F32)
                ksh = kf * coef[0, rows, :]
                rolled = []
                for j in range(1, KS):
                    r = pltpu.roll(kf, j, 1)
                    rolled.append(r)
                    ksh = ksh + jnp.where(lane >= j, r, 0.0 if kprev is None else kprev[j - 1]) * coef[j, rows, :]
                kvs.append((ksh * _b(av[roww, cols]).astype(F32)).astype(BF16))
                kprev = rolled
            st["kv"] = kvs
            lhs = jnp.concatenate(kvs + [_b(ssm[roww, c * C:(c + 1) * C]) for c in range(NCH)], axis=0)
            both = _dot(lhs, _b(fwd[...]))
            xh = [both[c * G:(c + 1) * G] for c in range(NCH)]
            st["h"] = [both[(NCH + c) * G:(NCH + c + 1) * G] for c in range(NCH)]
            st["u"] = [xh[0]] + [
                xh[c] + jnp.concatenate([xh[c - 1][:, 2 * hc:3 * hc], -xh[c - 1][:, 3 * hc:], -xh[c - 1][:, :hc],
                                         xh[c - 1][:, hc:2 * hc]], axis=1) for c in range(1, NCH)]

        def inverse(todo):
            ws, tok = [], None
            for a in todo:
                slabs = []
                for r0 in range(0, G, 8):
                    rs = slice(r0, r0 + 8)
                    zr = zi = None
                    for c in range(a + 1):
                        ur, ui = st["u"][c][rs, :C], st["u"][c][rs, C:]
                        hr, hi = st["h"][a - c][rs, :C], st["h"][a - c][rs, C:]
                        if zr is None and tok is not None:
                            ur = _after(tok, ur)
                        pr = ur * hr - ui * hi
                        pi = ur * hi + ui * hr
                        zr = pr if zr is None else zr + pr
                        zi = pi if zi is None else zi + pi
                    tok = zr
                    slabs.append(jnp.concatenate([zr, zi], axis=1))
                ws.append(jnp.concatenate(slabs, axis=0).astype(BF16))
            ys = _dot(jnp.concatenate(ws, axis=0), _b(inv[...]))
            for t, a in enumerate(todo):
                cols = slice(a * C, (a + 1) * C)
                y = ys[t * G:(t + 1) * G] + st["kv"][a].astype(F32) * coef[KS, rows, :]
                aT[rows, cols] = _b(aq[roww, cols]).astype(F32) * y

        ops = {FWD_AT: forward}
        for step, todo in INV_AT.items():
            ops[step] = functools.partial(inverse, todo)
        return ops

    def head(h, carry):
        @pl.when(h == 1)
        def _():
            cp(wkv.at[1:], wkv.at[1:], s_late).wait()

        @pl.when(h >= 5)
        def _():
            a_copy(h - 5).start()

        conv = conv_ops(jnp.minimum(h, NG - 1))
        wo = _b(woT[h])
        krow = jax.lax.broadcasted_iota(jnp.int32, (TQ, TQ), 0)
        qcol = jax.lax.broadcasted_iota(jnp.int32, (TQ, TQ), 1)
        causal = krow <= qcol
        ctx = {}

        def kproj(c):
            r = slice(c * KC // 2, (c + 1) * KC // 2)
            ks[r, :] = _w(_dot(_b(ckv[r, :]), _b(wks[...])).astype(BF16))

        def vproj(c):
            r = slice(c * KC // 2, (c + 1) * KC // 2)
            vTs[:, c * KC:(c + 1) * KC] = _w(jax.lax.dot_general(
                _b(wvs[...]), _b(ckv[r, :]), NT, preferred_element_type=F32).astype(BF16))

        def scores(i):
            n = TQ * (i + 1)
            sT = _dot(_b(ks[:n // 2, :]), _b(qs[h, :, TQ * i:n]))
            blocks = [sT[c0:c0 + TQ] for c0 in range(0, n - TQ, TQ)] + [jnp.where(causal, sT[n - TQ:], NEG)]
            m8, part = None, None
            for b, blk in enumerate(blocks):
                bm = jnp.max(blk.reshape(TQ // 8, 8, TQ), axis=0)
                m8 = bm if m8 is None else jnp.where(bm > m8, bm, m8)
                if b == i - PMAX:
                    part = m8[0:1]
            return blocks, m8, part

        def softmax(blocks, m8):
            m8 = jnp.broadcast_to(jnp.max(m8, axis=0, keepdims=True), (8, TQ))
            ls, p, ps = None, None, []
            for blk in blocks:
                mm = m8 if p is None else jnp.where(p[TQ - 8:] < 0.0, p[TQ - 8:], m8)
                p = jnp.exp2(blk - jnp.concatenate([mm] * (TQ // 8), axis=0))
                part = jnp.sum(p.reshape(TQ // 8, 8, TQ), axis=0)
                ls = part if ls is None else ls + part
                ps.append(p)
            return jnp.concatenate(ps, axis=0).astype(BF16), 1.0 / jnp.sum(ls, axis=0, keepdims=True)

        def pv(i, p, rl):
            n = TQ * (i + 1)
            halves = [_dot(_b(vTs[t * D // 4:(t + 1) * D // 4, :n]), p) * rl for t in range(2)]
            ctx[i] = jnp.concatenate(halves, axis=0).astype(BF16)

        def oproj(i0, i1):
            for i in range(i0, i1):
                acc[:, TQ * i:TQ * (i + 1)] += _dot(wo, ctx[i])

        kproj(0)
        vproj(0)
        st = None
        for i in range(NQ):
            if i + 2 < NQ:
                (vproj if i & 1 else kproj)(i // 2 + 1)
            if i in OFILL:
                oproj(*OFILL[i])
            if i > 0:
                p, rl = softmax(*st[:2])
            st = scores(i)
            if i > 0 and st[2] is not None:
                rl = _after(st[2], rl)
            if i in conv:
                conv[i]()
            if i > 0:
                pv(i - 1, p, rl)
        a_transpose(jnp.maximum(h - 4, 0))
        if PRE:
            b_transpose(*OUT_CHUNKS[0])
        prep_wkv(jnp.minimum(h + 1, H - 1))
        p, rl = softmax(*st[:2])
        oproj(max(e for _, e in OFILL.values()), OSPLIT)
        pv(NQ - 1, p, rl)
        oproj(OSPLIT, NQ)
        return carry

    def head_scoped(h, carry):
        with _scope("head"):
            return head(h, carry)

    jax.lax.fori_loop(0, H, head_scoped, 0)

    a_copy(11).start()
    c_out = [a_copy(p) for p in range(12)]
    for t, (i0, i1) in enumerate(OUT_CHUNKS):
        cols = slice(i0 * TQ, i1 * TQ)
        if t > 0 or not PRE:
            b_transpose(i0, i1)
        c = cp(outs.at[cols, NA:], out_hbm.at[cols, NA:], s_out)
        c.start()
        c_out.append(c)
    with _scope("wout"):
        for c in c_out:
            c.wait()


@jax.jit
def pallas_concat_heads__ssm_conv_h3__compressed_kv_cla__prompt_kernel(
    A_q: jax.Array,
    A_k: jax.Array,
    A_v: jax.Array,
    A_shift_k: jax.Array,
    A_ssm_k: jax.Array,
    A_ssm_D: jax.Array,
    B_x: jax.Array,
    B_c_kv: jax.Array,
    B_w_q: jax.Array,
    B_w_uk: jax.Array,
    B_w_uv: jax.Array,
    B_w_o: jax.Array,
):
    fwd, inv = _dft_mats()
    tr = lambda a: jnp.swapaxes(a, 1, 2).reshape(DA, S)
    any_spec = pl.BlockSpec(memory_space=pl.ANY)
    out = pl.pallas_call(
        _kernel,
        out_shape=jax.ShapeDtypeStruct((S, 2 * DA), BF16),
        in_specs=[any_spec] * 14,
        out_specs=any_spec,
        scratch_shapes=[
            pltpu.VMEM((DA // 2, S), U32),
            pltpu.VMEM((DA // 2, S), U32),
            pltpu.VMEM((DA // 2, S), U32),
            pltpu.VMEM((DA // 2, S), U32),
            pltpu.VMEM((DA // 2, S), U32),
            pltpu.VMEM((S // 2, DC), U32),
            pltpu.VMEM((H // 2, DA, D), U32),
            pltpu.VMEM((H // 2, 2, DC, D), U32),
            pltpu.VMEM((H, DA // 2, D), U32),
            pltpu.VMEM((D, DA), U32),
            pltpu.VMEM((H, D // 2, S), U32),
            pltpu.VMEM((S // 2, D), U32),
            pltpu.VMEM((D // 2, S), U32),
            pltpu.VMEM((DA, S), F32),
            pltpu.VMEM((DA, S), F32),
            pltpu.VMEM((KS + 1, DA, 128), F32),
            pltpu.VMEM((DC // 2, D), U32),
            pltpu.VMEM((D // 2, DC), U32),
            pltpu.VMEM((S, 2 * DA), BF16),
            pltpu.VMEM((KS, DA), BF16),
            pltpu.VMEM((DA,), BF16),
            pltpu.VMEM((C // 2, 2 * C), U32),
            pltpu.VMEM((C, C), U32),
            pltpu.SemaphoreType.DMA((8,)),
        ],
        compiler_params=pltpu.CompilerParams(vmem_limit_bytes=100 * 1024 * 1024),
    )(
        tr(A_q), tr(A_k), tr(A_v), A_shift_k.T, A_ssm_k, A_ssm_D, tr(B_x), B_c_kv.reshape(S, DC),
        B_w_q, B_w_uk, B_w_uv,
        jnp.swapaxes(B_w_o, 1, 2), jnp.asarray(fwd, BF16), jnp.asarray(inv, BF16),
    )
    return out.reshape(1, S, 2 * DA)
```

```python
import contextlib
import functools
import math

import jax
import jax.numpy as jnp
import numpy as np
import jax.experimental.pallas as pl
import jax.experimental.pallas.tpu as pltpu

F32 = jnp.float32
BF16 = jnp.bfloat16
U32 = jnp.uint32

S = 2048
DA = 448
H = 16
D = 256
DC = 1024
KS = 4
C = 128
NCH = S // C
G = 32
NG = DA // G
TQ = 128
NQ = S // TQ
KC = 256
NA = 384
NT = (((1,), (1,)), ((), ()))
LOG2E = math.log2(math.e)
QSCALE = (D ** -0.5) * LOG2E
NEG = -1e9 * LOG2E

X_CHUNKS = [(0, 384), (384, 1152), (1152, 2048)]
OUT_CHUNKS = [(0, 3), (3, 7), (7, 11), (11, 16)]
FWD_AT = 2
INV_AT = {4: [0, 1, 2, 3], 5: [4, 5], 6: [6], 7: [7], 8: [8], 9: [9], 10: [10], 11: [11], 12: [12], 13: [13], 14: [14], 15: [15]}
OFILL = {14: (0, 2), 15: (2, 4)}
OSPLIT = 12
PRE = 0
PAD = 0
PADMAX = 16
LSM = 0
NOTOK = 0
JIT0 = 3
JSTEP = 8
JOFF = 0
JONLY = 1
PSPL = 2
PSPL1 = 99
GPACE = 0
GSRC = [2, 3]
TP0 = 0
TP1 = 0
PMAX = 3
SCOPES = 0


def _scope(name):
    return jax.named_scope(name) if SCOPES else contextlib.nullcontext()


def _dft_mats():
    k = np.concatenate([np.arange(0, C, 2), np.arange(1, C, 2)]).astype(np.float64)
    n = np.arange(C, dtype=np.float64)
    th = 2.0 * np.pi * np.outer(n, k + 0.5) / (2 * C)
    fwd = np.concatenate([np.cos(th), np.sin(th)], axis=1)
    inv = fwd.T / C
    return fwd, inv


def _b(x):
    return pltpu.bitcast(x, BF16)


def _w(x):
    return pltpu.bitcast(x, U32)


def _dot(a, b):
    return jnp.dot(a, b, preferred_element_type=F32)


def _after(tok, x):
    return jnp.where(jnp.abs(tok) < -1.0, tok, x)


def _kernel(qT_hbm, kT_hbm, vT_hbm, shT_hbm, ssm_hbm, dvec_hbm, xT_hbm, ckv_hbm, wq_hbm, wuk_hbm, wuv_hbm,
            woT_hbm, fwd_hbm, inv_hbm,
            out_hbm,
            aq, ak, av, ssm, xT, ckv, wq, wkv, woT, wqs, qs, ks, vTs, acc, aT, coef, wks, wvs,
            outs, shT, dvec, fwd, inv, sems):
    def cp(src, dst, sem):
        return pltpu.make_async_copy(src, dst, sems.at[sem])

    s_wq0, s_x, s_wq, s_early, s_late, s_out = 0, 1, 4, 5, 6, 7
    wq_u, wuk_u, wuv_u, x_u = (r.bitcast(U32) for r in (wq_hbm, wuk_hbm, wuv_hbm, xT_hbm))
    c_wq0 = cp(wq_u.at[:, 0, :], wq.at[0], s_wq0)
    c_x = [[cp(x_u.at[:, c0:c1], xT.at[:, c0:c1], s_x + t)] for t, (c0, c1) in enumerate(X_CHUNKS)]
    c_x[-1] += [cp(wq_u.at[:, j, :], wq.at[j], s_x + 2) for j in (1, 2)]
    c_wq = [cp(wq_u.at[:, j, :], wq.at[j], s_wq) for j in range(3, H // 2)]
    early = [cp(src, dst, s_early) for src, dst in (
        (shT_hbm, shT), (dvec_hbm, dvec), (fwd_hbm.bitcast(U32), fwd), (inv_hbm.bitcast(U32), inv),
        (wuk_u.at[:, 0, :], wkv.at[0, 0]), (wuv_u.at[:, 0, :], wkv.at[0, 1]), (ckv_hbm.bitcast(U32), ckv),
        (woT_hbm.bitcast(U32), woT), (kT_hbm.bitcast(U32), ak), (vT_hbm.bitcast(U32), av),
        (ssm_hbm.bitcast(U32), ssm), (qT_hbm.bitcast(U32), aq))]
    late = [cp(src.at[:, j, :], wkv.at[j, t], s_late)
            for j in range(1, H // 2) for t, src in enumerate((wuk_u, wuv_u))]
    for c in [c_wq0, *c_x[0], *c_x[1], *c_x[2], *c_wq, *early, *late]:
        c.start()

    hi_mask = jnp.uint32(0xFFFF0000)

    def prep_wq(j):
        w = wq[j]
        wqs[:D // 2, :] = _w(pltpu.bitcast(w << 16, F32).T.astype(BF16))
        wqs[D // 2:, :] = _w(pltpu.bitcast(w & hi_mask, F32).T.astype(BF16))

    def prep_wkv(h):
        j = h >> 1
        sh = jnp.asarray(16 - 16 * (h & 1), U32)
        wks[...] = _w(pltpu.bitcast((wkv[j, 0] << sh) & hi_mask, F32).astype(BF16))
        wvs[...] = _w(pltpu.bitcast((wkv[j, 1] << sh) & hi_mask, F32).T.astype(BF16))

    def qproj(j, c0, c1):
        q2 = (_dot(_b(wqs[...]), _b(xT[:, c0:c1])) * QSCALE).astype(BF16)
        qs[2 * j, :, c0:c1] = _w(q2[:D])
        qs[2 * j + 1, :, c0:c1] = _w(q2[D:])

    acc[...] = jnp.zeros(acc.shape, F32)
    aT[:128, :] = jnp.zeros((128, S), F32)
    if PRE:
        aT[NA:, :] = jnp.zeros((DA - NA, S), F32)

    c_wq0.wait()
    prep_wq(0)
    for cs, (c0, c1) in zip(c_x, X_CHUNKS):
        for c in cs:
            c.wait()
        qproj(0, c0, c1)
    prep_wq(1)

    def qpair(j, carry):
        @pl.when(j == 2)
        def _():
            cp(wq.at[3:], wq.at[3:], s_wq).wait()

        qproj(j, 0, S)
        prep_wq(j + 1)
        return carry

    with _scope("qloop"):
        jax.lax.fori_loop(1, H // 2 - 1, qpair, 0)

    for c in early:
        c.wait()
    qproj(H // 2 - 1, 0, S)
    prep_wkv(0)
    cf = jnp.concatenate([shT[...].astype(F32), dvec[...].astype(F32)[None, :],
                          jnp.zeros((3, DA), F32)], axis=0).T
    for j in range(KS + 1):
        coef[j] = jnp.broadcast_to(cf[:, j:j + 1], (DA, 128))

    def a_piece(p):
        r = pl.ds(pl.multiple_of((p & 3) * (S // 4), S // 4), S // 4)
        c = pl.ds(pl.multiple_of((p >> 2) * 128, 128), 128)
        return r, c

    def a_copy(p):
        r, c = a_piece(p)
        return cp(outs.at[r, c], out_hbm.at[r, c], s_out)

    def a_transpose(p):
        r, c = a_piece(p)
        outs[r, c] = _b(_w(aT[c, r].astype(BF16))).T

    def b_transpose(i0, i1):
        cols = slice(i0 * TQ, i1 * TQ)
        blk = jnp.concatenate([aT[NA:, cols], acc[:, cols]], axis=0).astype(BF16)
        outs[cols, NA:] = _b(_w(blk)).T

    def conv_ops(g, toks):
        rows = pl.ds(pl.multiple_of(g * G, G), G)
        roww = pl.ds(pl.multiple_of(g * (G // 2), G // 2), G // 2)
        lane = jax.lax.broadcasted_iota(jnp.int32, (G, C), 1)
        hc = C // 2
        st = {}

        def forward():
            kvs, kprev = [], None
            for c in range(NCH):
                cols = slice(c * C, (c + 1) * C)
                kf = _b(ak[roww, cols]).astype(F32)
                if GPACE:
                    src = toks[GSRC[c * len(GSRC) // NCH]]
                    r0 = (c * len(GSRC) % NCH) * src.shape[0] // NCH // 8 * 8
                    kf = jnp.concatenate([_after(src[r0:r0 + 8, :C], kf[:8]), kf[8:]], axis=0) if GPACE == 1 else \
                        _after(jnp.concatenate([src[r0:r0 + 8, :C]] * (G // 8), axis=0), kf)
                ksh = kf * coef[0, rows, :]
                rolled = []
                for j in range(1, KS):
                    r = pltpu.roll(kf, j, 1)
                    rolled.append(r)
                    ksh = ksh + jnp.where(lane >= j, r, 0.0 if kprev is None else kprev[j - 1]) * coef[j, rows, :]
                kvs.append((ksh * _b(av[roww, cols]).astype(F32)).astype(BF16))
                kprev = rolled
            st["kv"] = kvs
            lhs = jnp.concatenate(kvs + [_b(ssm[roww, c * C:(c + 1) * C]) for c in range(NCH)], axis=0)
            both = _dot(lhs, _b(fwd[...]))
            xh = [both[c * G:(c + 1) * G] for c in range(NCH)]
            st["h"] = [both[(NCH + c) * G:(NCH + c + 1) * G] for c in range(NCH)]
            st["u"] = [xh[0]] + [
                xh[c] + jnp.concatenate([xh[c - 1][:, 2 * hc:3 * hc], -xh[c - 1][:, 3 * hc:], -xh[c - 1][:, :hc],
                                         xh[c - 1][:, hc:2 * hc]], axis=1) for c in range(1, NCH)]

        def inverse(todo):
            ws, tok = [], None
            for a in todo:
                slabs = []
                for r0 in range(0, G, 8):
                    rs = slice(r0, r0 + 8)
                    zr = zi = None
                    for c in range(a + 1):
                        ur, ui = st["u"][c][rs, :C], st["u"][c][rs, C:]
                        hr, hi = st["h"][a - c][rs, :C], st["h"][a - c][rs, C:]
                        if zr is None and tok is not None:
                            ur = _after(tok, ur)
                        pr = ur * hr - ui * hi
                        pi = ur * hi + ui * hr
                        zr = pr if zr is None else zr + pr
                        zi = pi if zi is None else zi + pi
                    tok = zr
                    slabs.append(jnp.concatenate([zr, zi], axis=1))
                ws.append(jnp.concatenate(slabs, axis=0).astype(BF16))
            ys = _dot(jnp.concatenate(ws, axis=0), _b(inv[...]))
            for t, a in enumerate(todo):
                cols = slice(a * C, (a + 1) * C)
                y = ys[t * G:(t + 1) * G] + st["kv"][a].astype(F32) * coef[KS, rows, :]
                aT[rows, cols] = _b(aq[roww, cols]).astype(F32) * y

        ops = {FWD_AT: forward}
        for step, todo in INV_AT.items():
            ops[step] = functools.partial(inverse, todo)
        return ops

    def head(h, carry):
        @pl.when(h == 1)
        def _():
            cp(wkv.at[1:], wkv.at[1:], s_late).wait()

        @pl.when(h >= 5)
        def _():
            a_copy(h - 5).start()

        toks = {}
        conv = conv_ops(jnp.minimum(h, NG - 1), toks)
        wo = _b(woT[h])
        krow = jax.lax.broadcasted_iota(jnp.int32, (TQ, TQ), 0)
        qcol = jax.lax.broadcasted_iota(jnp.int32, (TQ, TQ), 1)
        causal = krow <= qcol
        ctx = {}

        def kproj(c):
            r = slice(c * KC // 2, (c + 1) * KC // 2)
            toks[2 * c] = _dot(_b(ckv[r, :]), _b(wks[...]))
            ks[r, :] = _w(toks[2 * c].astype(BF16))

        def vproj(c):
            r = slice(c * KC // 2, (c + 1) * KC // 2)
            toks[2 * c + 1] = jax.lax.dot_general(_b(wvs[...]), _b(ckv[r, :]), NT, preferred_element_type=F32)
            vTs[:, c * KC:(c + 1) * KC] = _w(toks[2 * c + 1].astype(BF16))

        def scores(i):
            n = TQ * (i + 1)
            sT = _dot(_b(ks[:n // 2, :]), _b(qs[h, :, TQ * i:n]))
            blocks = [sT[c0:c0 + TQ] for c0 in range(0, n - TQ, TQ)] + [jnp.where(causal, sT[n - TQ:], NEG)]
            m8, part = None, None
            for b, blk in enumerate(blocks):
                bm = jnp.max(blk.reshape(TQ // 8, 8, TQ), axis=0)
                m8 = bm if m8 is None else jnp.where(bm > m8, bm, m8)
                if b == i - PMAX:
                    part = m8[0:1]
            return blocks, m8, part

        def softmax(blocks, m8, nxt=None, pace=None):
            m8 = jnp.broadcast_to(jnp.max(m8, axis=0, keepdims=True), (8, TQ))
            ls, p, ps = None, None, []
            for b, blk in enumerate(blocks):
                mm = m8 if p is None else jnp.where(p[TQ - 8:] < 0.0, p[TQ - 8:], m8)
                if nxt is not None and JIT0 and b >= JIT0:
                    v = JSTEP * (b - JIT0) + JOFF
                    tok = nxt[v // 16][v % 16 * 8:v % 16 * 8 + 8]
                    mm = _after(tok, m8 if JONLY else mm)
                if pace is not None:
                    mm = _after(pace[b], m8)
                p = jnp.exp2(blk - jnp.concatenate([mm] * (TQ // 8), axis=0))
                part = jnp.sum(p.reshape(TQ // 8, 8, TQ), axis=0)
                if LSM:
                    part = jnp.maximum(part, 0.0)
                ls = part if ls is None else ls + part
                ps.append(p)
            return jnp.concatenate(ps, axis=0).astype(BF16), 1.0 / jnp.sum(ls, axis=0, keepdims=True)

        def pv(i, p, rl):
            n = TQ * (i + 1)
            ns = PSPL if i < PSPL1 else 1
            w = D // 2 // ns
            halves = [_dot(_b(vTs[t * w:(t + 1) * w, :n]), p) * rl for t in range(ns)]
            ctx[i] = jnp.concatenate(halves, axis=0).astype(BF16)

        def oproj(i0, i1):
            for i in range(i0, i1):
                toks["o", i] = _dot(wo, ctx[i])
                acc[:, TQ * i:TQ * (i + 1)] += toks["o", i]

        kproj(0)
        vproj(0)
        st = None
        for i in range(NQ):
            if i + 2 < NQ:
                (vproj if i & 1 else kproj)(i // 2 + 1)
            if i in OFILL:
                oproj(*OFILL[i])
            prev, st = st, scores(i)
            if i > 0:
                p, rl = softmax(*prev[:2], st[0])
            if i > 0 and st[2] is not None:
                rl = _after(st[2], rl)
            if i in conv:
                conv[i]()
            if i > 0:
                pv(i - 1, p, rl)
        a_transpose(jnp.maximum(h - 4, 0))
        if PRE:
            b_transpose(*OUT_CHUNKS[0])
        prep_wkv(jnp.minimum(h + 1, H - 1))
        o0 = max(e for _, e in OFILL.values())
        oproj(o0, OSPLIT)
        pace = None
        if TP1:
            times = [TP0 + TP1 * b for b in range(NQ)]
            pace = [toks["o", o0 + 2 * (t // DA)][t % DA // 8 * 8:t % DA // 8 * 8 + 8] for t in times]
        p, rl = softmax(*st[:2], pace=pace)
        pv(NQ - 1, p, rl)
        oproj(OSPLIT, NQ)
        return carry

    def head_scoped(h, carry):
        with _scope("head"):
            return head(h, carry)

    jax.lax.fori_loop(0, H, head_scoped, 0)

    a_copy(11).start()
    c_out = [a_copy(p) for p in range(12)]
    for t, (i0, i1) in enumerate(OUT_CHUNKS):
        cols = slice(i0 * TQ, i1 * TQ)
        if t > 0 or not PRE:
            b_transpose(i0, i1)
        c = cp(outs.at[cols, NA:], out_hbm.at[cols, NA:], s_out)
        c.start()
        c_out.append(c)
    with _scope("wout"):
        for c in c_out:
            c.wait()


@jax.jit
def pallas_concat_heads__ssm_conv_h3__compressed_kv_cla__prompt_kernel(
    A_q: jax.Array,
    A_k: jax.Array,
    A_v: jax.Array,
    A_shift_k: jax.Array,
    A_ssm_k: jax.Array,
    A_ssm_D: jax.Array,
    B_x: jax.Array,
    B_c_kv: jax.Array,
    B_w_q: jax.Array,
    B_w_uk: jax.Array,
    B_w_uv: jax.Array,
    B_w_o: jax.Array,
):
    fwd, inv = _dft_mats()
    tr = lambda a: jnp.swapaxes(a, 1, 2).reshape(DA, S)
    any_spec = pl.BlockSpec(memory_space=pl.ANY)
    out = pl.pallas_call(
        _kernel,
        out_shape=jax.ShapeDtypeStruct((S, 2 * DA), BF16),
        in_specs=[any_spec] * 14,
        out_specs=any_spec,
        scratch_shapes=[
            pltpu.VMEM((DA // 2, S), U32),
            pltpu.VMEM((DA // 2, S), U32),
            pltpu.VMEM((DA // 2, S), U32),
            pltpu.VMEM((DA // 2, S), U32),
            pltpu.VMEM((DA // 2, S), U32),
            pltpu.VMEM((S // 2, DC), U32),
            pltpu.VMEM((H // 2, DA, D), U32),
            pltpu.VMEM((H // 2, 2, DC, D), U32),
            pltpu.VMEM((H, DA // 2, D), U32),
            pltpu.VMEM((D, DA), U32),
            pltpu.VMEM((H, D // 2, S), U32),
            pltpu.VMEM((S // 2, D), U32),
            pltpu.VMEM((D // 2, S), U32),
            pltpu.VMEM((DA, S), F32),
            pltpu.VMEM((DA, S), F32),
            pltpu.VMEM((KS + 1, DA, 128), F32),
            pltpu.VMEM((DC // 2, D), U32),
            pltpu.VMEM((D // 2, DC), U32),
            pltpu.VMEM((S, 2 * DA), BF16),
            pltpu.VMEM((KS, DA), BF16),
            pltpu.VMEM((DA,), BF16),
            pltpu.VMEM((C // 2, 2 * C), U32),
            pltpu.VMEM((C, C), U32),
            pltpu.SemaphoreType.DMA((8,)),
        ],
        compiler_params=pltpu.CompilerParams(vmem_limit_bytes=100 * 1024 * 1024),
    )(
        tr(A_q), tr(A_k), tr(A_v), A_shift_k.T, A_ssm_k, A_ssm_D, tr(B_x), B_c_kv.reshape(S, DC),
        B_w_q, B_w_uk, B_w_uv,
        jnp.swapaxes(B_w_o, 1, 2), jnp.asarray(fwd, BF16), jnp.asarray(inv, BF16),
    )
    return out.reshape(1, S, 2 * DA)
```

```python
import functools
import math

import jax
import jax.numpy as jnp
import numpy as np
import jax.experimental.pallas as pl
import jax.experimental.pallas.tpu as pltpu

F32 = jnp.float32
BF16 = jnp.bfloat16
U32 = jnp.uint32

S = 2048
DA = 448
H = 16
D = 256
DC = 1024
KS = 4
C = 128
NCH = S // C
G = 32
NG = DA // G
TQ = 128
NQ = S // TQ
KC = 256
NA = 384
NT = (((1,), (1,)), ((), ()))
LOG2E = math.log2(math.e)
QSCALE = (D ** -0.5) * LOG2E
NEG = -1e9 * LOG2E

X_CHUNKS = ((0, 384), (384, 1152), (1152, 2048))
OUT_CHUNKS = ((0, 3), (3, 7), (7, 11), (11, 16))
FWD_AT = 2
INV_AT = {4: (0, 1, 2, 3), 5: (4, 5), **{a: (a,) for a in range(6, NCH)}}
OFILL = {14: (0, 2), 15: (2, 4)}
OSPLIT = 12
PMAX = 3
JIT0 = 3


def _dft_mats():
    k = np.concatenate([np.arange(0, C, 2), np.arange(1, C, 2)]).astype(np.float64)
    n = np.arange(C, dtype=np.float64)
    th = 2.0 * np.pi * np.outer(n, k + 0.5) / (2 * C)
    fwd = np.concatenate([np.cos(th), np.sin(th)], axis=1)
    inv = fwd.T / C
    return fwd, inv


def _b(x):
    return pltpu.bitcast(x, BF16)


def _w(x):
    return pltpu.bitcast(x, U32)


def _dot(a, b):
    return jnp.dot(a, b, preferred_element_type=F32)


def _after(tok, x):
    return jnp.where(jnp.abs(tok) < -1.0, tok, x)


def _kernel(qT_hbm, kT_hbm, vT_hbm, shT_hbm, ssm_hbm, dvec_hbm, xT_hbm, ckv_hbm, wq_hbm, wuk_hbm, wuv_hbm,
            woT_hbm, fwd_hbm, inv_hbm,
            out_hbm,
            aq, ak, av, ssm, xT, ckv, wq, wkv, woT, wqs, qs, ks, vTs, acc, aT, coef, wks, wvs,
            outs, shT, dvec, fwd, inv, sems):
    def cp(src, dst, sem):
        return pltpu.make_async_copy(src, dst, sems.at[sem])

    s_wq0, s_x, s_wq, s_early, s_late, s_out = 0, 1, 4, 5, 6, 7
    wq_u, wuk_u, wuv_u, x_u = (r.bitcast(U32) for r in (wq_hbm, wuk_hbm, wuv_hbm, xT_hbm))
    c_wq0 = cp(wq_u.at[:, 0, :], wq.at[0], s_wq0)
    c_x = [[cp(x_u.at[:, c0:c1], xT.at[:, c0:c1], s_x + t)] for t, (c0, c1) in enumerate(X_CHUNKS)]
    c_x[-1] += [cp(wq_u.at[:, j, :], wq.at[j], s_x + 2) for j in (1, 2)]
    c_wq = [cp(wq_u.at[:, j, :], wq.at[j], s_wq) for j in range(3, H // 2)]
    early = [cp(src, dst, s_early) for src, dst in (
        (shT_hbm, shT), (dvec_hbm, dvec), (fwd_hbm.bitcast(U32), fwd), (inv_hbm.bitcast(U32), inv),
        (wuk_u.at[:, 0, :], wkv.at[0, 0]), (wuv_u.at[:, 0, :], wkv.at[0, 1]), (ckv_hbm.bitcast(U32), ckv),
        (woT_hbm.bitcast(U32), woT), (kT_hbm.bitcast(U32), ak), (vT_hbm.bitcast(U32), av),
        (ssm_hbm.bitcast(U32), ssm), (qT_hbm.bitcast(U32), aq))]
    late = [cp(src.at[:, j, :], wkv.at[j, t], s_late)
            for j in range(1, H // 2) for t, src in enumerate((wuk_u, wuv_u))]
    for c in [c_wq0, *c_x[0], *c_x[1], *c_x[2], *c_wq, *early, *late]:
        c.start()

    hi_mask = jnp.uint32(0xFFFF0000)

    def prep_wq(j):
        w = wq[j]
        wqs[:D // 2, :] = _w(pltpu.bitcast(w << 16, F32).T.astype(BF16))
        wqs[D // 2:, :] = _w(pltpu.bitcast(w & hi_mask, F32).T.astype(BF16))

    def prep_wkv(h):
        j = h >> 1
        sh = jnp.asarray(16 - 16 * (h & 1), U32)
        wks[...] = _w(pltpu.bitcast((wkv[j, 0] << sh) & hi_mask, F32).astype(BF16))
        wvs[...] = _w(pltpu.bitcast((wkv[j, 1] << sh) & hi_mask, F32).T.astype(BF16))

    def qproj(j, c0, c1):
        q2 = (_dot(_b(wqs[...]), _b(xT[:, c0:c1])) * QSCALE).astype(BF16)
        qs[2 * j, :, c0:c1] = _w(q2[:D])
        qs[2 * j + 1, :, c0:c1] = _w(q2[D:])

    acc[...] = jnp.zeros(acc.shape, F32)
    aT[:128, :] = jnp.zeros((128, S), F32)

    c_wq0.wait()
    prep_wq(0)
    for cs, (c0, c1) in zip(c_x, X_CHUNKS):
        for c in cs:
            c.wait()
        qproj(0, c0, c1)
    prep_wq(1)

    def qpair(j, carry):
        @pl.when(j == 2)
        def _():
            cp(wq.at[3:], wq.at[3:], s_wq).wait()

        qproj(j, 0, S)
        prep_wq(j + 1)
        return carry

    jax.lax.fori_loop(1, H // 2 - 1, qpair, 0)

    for c in early:
        c.wait()
    qproj(H // 2 - 1, 0, S)
    prep_wkv(0)
    taps = shT[...].astype(F32)
    for j in range(KS + 1):
        row = taps[j:j + 1] if j < KS else dvec[...].astype(F32)[None, :]
        coef[j] = jnp.broadcast_to(row, (128, DA)).T

    def a_piece(p):
        r = pl.ds(pl.multiple_of((p & 3) * (S // 4), S // 4), S // 4)
        c = pl.ds(pl.multiple_of((p >> 2) * 128, 128), 128)
        return r, c

    def a_copy(p):
        r, c = a_piece(p)
        return cp(outs.at[r, c], out_hbm.at[r, c], s_out)

    def a_transpose(p):
        r, c = a_piece(p)
        outs[r, c] = _b(_w(aT[c, r].astype(BF16))).T

    def conv_ops(g):
        rows = pl.ds(pl.multiple_of(g * G, G), G)
        roww = pl.ds(pl.multiple_of(g * (G // 2), G // 2), G // 2)
        lane = jax.lax.broadcasted_iota(jnp.int32, (G, C), 1)
        hc = C // 2
        st = {}

        def forward():
            kvs, kprev = [], None
            for c in range(NCH):
                cols = slice(c * C, (c + 1) * C)
                kf = _b(ak[roww, cols]).astype(F32)
                ksh = kf * coef[0, rows, :]
                rolled = []
                for j in range(1, KS):
                    r = pltpu.roll(kf, j, 1)
                    rolled.append(r)
                    ksh = ksh + jnp.where(lane >= j, r, 0.0 if kprev is None else kprev[j - 1]) * coef[j, rows, :]
                kvs.append((ksh * _b(av[roww, cols]).astype(F32)).astype(BF16))
                kprev = rolled
            st["kv"] = kvs
            lhs = jnp.concatenate(kvs + [_b(ssm[roww, c * C:(c + 1) * C]) for c in range(NCH)], axis=0)
            both = _dot(lhs, _b(fwd[...]))
            xh = [both[c * G:(c + 1) * G] for c in range(NCH)]
            st["h"] = [both[(NCH + c) * G:(NCH + c + 1) * G] for c in range(NCH)]
            st["u"] = [xh[0]] + [
                xh[c] + jnp.concatenate([xh[c - 1][:, 2 * hc:3 * hc], -xh[c - 1][:, 3 * hc:], -xh[c - 1][:, :hc],
                                         xh[c - 1][:, hc:2 * hc]], axis=1) for c in range(1, NCH)]

        def inverse(todo):
            ws, tok = [], None
            for a in todo:
                slabs = []
                for r0 in range(0, G, 8):
                    rs = slice(r0, r0 + 8)
                    zr = zi = None
                    for c in range(a + 1):
                        ur, ui = st["u"][c][rs, :C], st["u"][c][rs, C:]
                        hr, hi = st["h"][a - c][rs, :C], st["h"][a - c][rs, C:]
                        if zr is None and tok is not None:
                            ur = _after(tok, ur)
                        pr = ur * hr - ui * hi
                        pi = ur * hi + ui * hr
                        zr = pr if zr is None else zr + pr
                        zi = pi if zi is None else zi + pi
                    tok = zr
                    slabs.append(jnp.concatenate([zr, zi], axis=1))
                ws.append(jnp.concatenate(slabs, axis=0).astype(BF16))
            ys = _dot(jnp.concatenate(ws, axis=0), _b(inv[...]))
            for t, a in enumerate(todo):
                cols = slice(a * C, (a + 1) * C)
                y = ys[t * G:(t + 1) * G] + st["kv"][a].astype(F32) * coef[KS, rows, :]
                aT[rows, cols] = _b(aq[roww, cols]).astype(F32) * y

        ops = {FWD_AT: forward}
        for step, todo in INV_AT.items():
            ops[step] = functools.partial(inverse, todo)
        return ops

    def head(h, carry):
        @pl.when(h == 1)
        def _():
            cp(wkv.at[1:], wkv.at[1:], s_late).wait()

        @pl.when(h >= 5)
        def _():
            a_copy(h - 5).start()

        conv = conv_ops(jnp.minimum(h, NG - 1))
        wo = _b(woT[h])
        krow = jax.lax.broadcasted_iota(jnp.int32, (TQ, TQ), 0)
        qcol = jax.lax.broadcasted_iota(jnp.int32, (TQ, TQ), 1)
        causal = krow <= qcol
        ctx = {}

        def kproj(c):
            r = slice(c * KC // 2, (c + 1) * KC // 2)
            ks[r, :] = _w(_dot(_b(ckv[r, :]), _b(wks[...])).astype(BF16))

        def vproj(c):
            r = slice(c * KC // 2, (c + 1) * KC // 2)
            vT = jax.lax.dot_general(_b(wvs[...]), _b(ckv[r, :]), NT, preferred_element_type=F32)
            vTs[:, c * KC:(c + 1) * KC] = _w(vT.astype(BF16))

        def scores(i):
            n = TQ * (i + 1)
            sT = _dot(_b(ks[:n // 2, :]), _b(qs[h, :, TQ * i:n]))
            blocks = [sT[c0:c0 + TQ] for c0 in range(0, n - TQ, TQ)] + [jnp.where(causal, sT[n - TQ:], NEG)]
            m8, part = None, None
            for b, blk in enumerate(blocks):
                bm = jnp.max(blk.reshape(TQ // 8, 8, TQ), axis=0)
                m8 = bm if m8 is None else jnp.where(bm > m8, bm, m8)
                if b == i - PMAX:
                    part = m8[0:1]
            return blocks, m8, part

        def softmax(blocks, m8, nxt=None):
            m8 = jnp.broadcast_to(jnp.max(m8, axis=0, keepdims=True), (8, TQ))
            ls, p, ps = None, None, []
            for b, blk in enumerate(blocks):
                if nxt is not None and b >= JIT0:
                    v = 8 * (b - JIT0)
                    mm = _after(nxt[v // 16][v % 16 * 8:v % 16 * 8 + 8], m8)
                else:
                    mm = m8 if p is None else jnp.where(p[TQ - 8:] < 0.0, p[TQ - 8:], m8)
                p = jnp.exp2(blk - jnp.concatenate([mm] * (TQ // 8), axis=0))
                part = jnp.sum(p.reshape(TQ // 8, 8, TQ), axis=0)
                ls = part if ls is None else ls + part
                ps.append(p)
            return jnp.concatenate(ps, axis=0).astype(BF16), 1.0 / jnp.sum(ls, axis=0, keepdims=True)

        def pv(i, p, rl):
            n = TQ * (i + 1)
            halves = [_dot(_b(vTs[t * D // 4:(t + 1) * D // 4, :n]), p) * rl for t in range(2)]
            ctx[i] = jnp.concatenate(halves, axis=0).astype(BF16)

        def oproj(i0, i1):
            for i in range(i0, i1):
                acc[:, TQ * i:TQ * (i + 1)] += _dot(wo, ctx[i])

        kproj(0)
        vproj(0)
        st = None
        for i in range(NQ):
            if i + 2 < NQ:
                (vproj if i & 1 else kproj)(i // 2 + 1)
            if i in OFILL:
                oproj(*OFILL[i])
            prev, st = st, scores(i)
            if i > 0:
                p, rl = softmax(*prev[:2], st[0])
            if i > 0 and st[2] is not None:
                rl = _after(st[2], rl)
            if i in conv:
                conv[i]()
            if i > 0:
                pv(i - 1, p, rl)
        a_transpose(jnp.maximum(h - 4, 0))
        prep_wkv(jnp.minimum(h + 1, H - 1))
        oproj(OFILL[NQ - 1][1], OSPLIT)
        p, rl = softmax(*st[:2])
        pv(NQ - 1, p, rl)
        oproj(OSPLIT, NQ)
        return carry

    jax.lax.fori_loop(0, H, head, 0)

    a_copy(11).start()
    c_out = [a_copy(p) for p in range(12)]
    for i0, i1 in OUT_CHUNKS:
        cols = slice(i0 * TQ, i1 * TQ)
        blk = jnp.concatenate([aT[NA:, cols], acc[:, cols]], axis=0).astype(BF16)
        outs[cols, NA:] = _b(_w(blk)).T
        c = cp(outs.at[cols, NA:], out_hbm.at[cols, NA:], s_out)
        c.start()
        c_out.append(c)
    for c in c_out:
        c.wait()


@jax.jit
def pallas_concat_heads__ssm_conv_h3__compressed_kv_cla__prompt_kernel(
    A_q: jax.Array,
    A_k: jax.Array,
    A_v: jax.Array,
    A_shift_k: jax.Array,
    A_ssm_k: jax.Array,
    A_ssm_D: jax.Array,
    B_x: jax.Array,
    B_c_kv: jax.Array,
    B_w_q: jax.Array,
    B_w_uk: jax.Array,
    B_w_uv: jax.Array,
    B_w_o: jax.Array,
):
    fwd, inv = _dft_mats()
    tr = lambda a: jnp.swapaxes(a, 1, 2).reshape(DA, S)
    any_spec = pl.BlockSpec(memory_space=pl.ANY)
    out = pl.pallas_call(
        _kernel,
        out_shape=jax.ShapeDtypeStruct((S, 2 * DA), BF16),
        in_specs=[any_spec] * 14,
        out_specs=any_spec,
        scratch_shapes=[
            pltpu.VMEM((DA // 2, S), U32),
            pltpu.VMEM((DA // 2, S), U32),
            pltpu.VMEM((DA // 2, S), U32),
            pltpu.VMEM((DA // 2, S), U32),
            pltpu.VMEM((DA // 2, S), U32),
            pltpu.VMEM((S // 2, DC), U32),
            pltpu.VMEM((H // 2, DA, D), U32),
            pltpu.VMEM((H // 2, 2, DC, D), U32),
            pltpu.VMEM((H, DA // 2, D), U32),
            pltpu.VMEM((D, DA), U32),
            pltpu.VMEM((H, D // 2, S), U32),
            pltpu.VMEM((S // 2, D), U32),
            pltpu.VMEM((D // 2, S), U32),
            pltpu.VMEM((DA, S), F32),
            pltpu.VMEM((DA, S), F32),
            pltpu.VMEM((KS + 1, DA, 128), F32),
            pltpu.VMEM((DC // 2, D), U32),
            pltpu.VMEM((D // 2, DC), U32),
            pltpu.VMEM((S, 2 * DA), BF16),
            pltpu.VMEM((KS, DA), BF16),
            pltpu.VMEM((DA,), BF16),
            pltpu.VMEM((C // 2, 2 * C), U32),
            pltpu.VMEM((C, C), U32),
            pltpu.SemaphoreType.DMA((8,)),
        ],
        compiler_params=pltpu.CompilerParams(vmem_limit_bytes=100 * 1024 * 1024),
    )(
        tr(A_q), tr(A_k), tr(A_v), A_shift_k.T, A_ssm_k, A_ssm_D, tr(B_x), B_c_kv.reshape(S, DC),
        B_w_q, B_w_uk, B_w_uv,
        jnp.swapaxes(B_w_o, 1, 2), jnp.asarray(fwd, BF16), jnp.asarray(inv, BF16),
    )
    return out.reshape(1, S, 2 * DA)
```

```python
import functools
import math

import jax
import jax.numpy as jnp
import numpy as np
import jax.experimental.pallas as pl
import jax.experimental.pallas.tpu as pltpu

F32 = jnp.float32
BF16 = jnp.bfloat16
U32 = jnp.uint32

S = 2048
DA = 448
H = 16
D = 256
DC = 1024
KS = 4
C = 128
NCH = S // C
G = 32
NG = DA // G
TQ = 128
NQ = S // TQ
KC = 256
NA = 384
NT = (((1,), (1,)), ((), ()))
LOG2E = math.log2(math.e)
QSCALE = (D ** -0.5) * LOG2E
NEG = -1e9 * LOG2E

X_CHUNKS = ((0, 384), (384, 1152), (1152, 2048))
OUT_CHUNKS = ((0, 1), (1, 4), (4, 8), (8, 12), (12, 16))
FWD_AT = 2
INV_AT = {4: (0, 1, 2, 3, 4), 5: (5, 6), **{a - 1: (a,) for a in range(7, 15)}, 15: (15,)}
OFILL = {14: (0, 2), 15: (2, 4)}
OSPLIT = 12
PMAX = 3
JIT0 = 3
GATE_PACE = (1, 2, 3)
TAIL_PACE = 32


def _dft_mats():
    k = np.concatenate([np.arange(0, C, 2), np.arange(1, C, 2)]).astype(np.float64)
    n = np.arange(C, dtype=np.float64)
    th = 2.0 * np.pi * np.outer(n, k + 0.5) / (2 * C)
    fwd = np.concatenate([np.cos(th), np.sin(th)], axis=1)
    inv = fwd.T / C
    return fwd, inv


def _b(x):
    return pltpu.bitcast(x, BF16)


def _w(x):
    return pltpu.bitcast(x, U32)


def _dot(a, b):
    return jnp.dot(a, b, preferred_element_type=F32)


def _after(tok, x):
    return jnp.where(jnp.abs(tok) < -1.0, tok, x)


def _kernel(qT_hbm, kT_hbm, vT_hbm, shT_hbm, ssm_hbm, dvec_hbm, xT_hbm, ckv_hbm, wq_hbm, wuk_hbm, wuv_hbm,
            woT_hbm, fwd_hbm, inv_hbm,
            out_hbm,
            aq, ak, av, ssm, xT, ckv, wq, wkv, woT, wqs, qs, ks, vTs, acc, aT, coef, wks, wvs,
            outs, shT, dvec, fwd, inv, sems):
    def cp(src, dst, sem):
        return pltpu.make_async_copy(src, dst, sems.at[sem])

    s_wq0, s_x, s_wq, s_early, s_late, s_out = 0, 1, 4, 5, 6, 7
    wq_u, wuk_u, wuv_u, x_u = (r.bitcast(U32) for r in (wq_hbm, wuk_hbm, wuv_hbm, xT_hbm))
    c_wq0 = cp(wq_u.at[:, 0, :], wq.at[0], s_wq0)
    c_x = [[cp(x_u.at[:, c0:c1], xT.at[:, c0:c1], s_x + t)] for t, (c0, c1) in enumerate(X_CHUNKS)]
    c_x[-1] += [cp(wq_u.at[:, j, :], wq.at[j], s_x + 2) for j in (1, 2)]
    c_wq = [cp(wq_u.at[:, j, :], wq.at[j], s_wq) for j in range(3, H // 2)]
    early = [cp(src, dst, s_early) for src, dst in (
        (shT_hbm, shT), (dvec_hbm, dvec), (fwd_hbm.bitcast(U32), fwd), (inv_hbm.bitcast(U32), inv),
        (wuk_u.at[:, 0, :], wkv.at[0, 0]), (wuv_u.at[:, 0, :], wkv.at[0, 1]), (ckv_hbm.bitcast(U32), ckv),
        (woT_hbm.bitcast(U32), woT), (kT_hbm.bitcast(U32), ak), (vT_hbm.bitcast(U32), av),
        (ssm_hbm.bitcast(U32), ssm), (qT_hbm.bitcast(U32), aq))]
    late = [cp(src.at[:, j, :], wkv.at[j, t], s_late)
            for j in range(1, H // 2) for t, src in enumerate((wuk_u, wuv_u))]
    for c in [c_wq0, *c_x[0], *c_x[1], *c_x[2], *c_wq, *early, *late]:
        c.start()

    hi_mask = jnp.uint32(0xFFFF0000)

    def prep_wq(j):
        w = wq[j]
        wqs[:D // 2, :] = _w(pltpu.bitcast(w << 16, F32).T.astype(BF16))
        wqs[D // 2:, :] = _w(pltpu.bitcast(w & hi_mask, F32).T.astype(BF16))

    def prep_wkv(h):
        j = h >> 1
        sh = jnp.asarray(16 - 16 * (h & 1), U32)
        wks[...] = _w(pltpu.bitcast((wkv[j, 0] << sh) & hi_mask, F32).astype(BF16))
        wvs[...] = _w(pltpu.bitcast((wkv[j, 1] << sh) & hi_mask, F32).T.astype(BF16))

    def qproj(j, c0, c1):
        q2 = (_dot(_b(wqs[...]), _b(xT[:, c0:c1])) * QSCALE).astype(BF16)
        qs[2 * j, :, c0:c1] = _w(q2[:D])
        qs[2 * j + 1, :, c0:c1] = _w(q2[D:])

    acc[...] = jnp.zeros(acc.shape, F32)
    aT[:128, :] = jnp.zeros((128, S), F32)

    c_wq0.wait()
    prep_wq(0)
    for cs, (c0, c1) in zip(c_x, X_CHUNKS):
        for c in cs:
            c.wait()
        qproj(0, c0, c1)
    prep_wq(1)

    def qpair(j, carry):
        @pl.when(j == 2)
        def _():
            cp(wq.at[3:], wq.at[3:], s_wq).wait()

        qproj(j, 0, S)
        prep_wq(j + 1)
        return carry

    jax.lax.fori_loop(1, H // 2 - 1, qpair, 0)

    for c in early:
        c.wait()
    qproj(H // 2 - 1, 0, S)
    prep_wkv(0)
    taps = shT[...].astype(F32)
    for j in range(KS + 1):
        row = taps[j:j + 1] if j < KS else dvec[...].astype(F32)[None, :]
        coef[j] = jnp.broadcast_to(row, (128, DA)).T

    def a_piece(p):
        r = pl.ds(pl.multiple_of((p & 3) * (S // 4), S // 4), S // 4)
        c = pl.ds(pl.multiple_of((p >> 2) * 128, 128), 128)
        return r, c

    def a_copy(p):
        r, c = a_piece(p)
        return cp(outs.at[r, c], out_hbm.at[r, c], s_out)

    def a_transpose(p):
        r, c = a_piece(p)
        outs[r, c] = _b(_w(aT[c, r].astype(BF16))).T

    def conv_ops(g, proj):
        rows = pl.ds(pl.multiple_of(g * G, G), G)
        roww = pl.ds(pl.multiple_of(g * (G // 2), G // 2), G // 2)
        lane = jax.lax.broadcasted_iota(jnp.int32, (G, C), 1)
        hc = C // 2
        st = {}

        def forward():
            kvs, kprev = [], None
            for c in range(NCH):
                cols = slice(c * C, (c + 1) * C)
                kf = _b(ak[roww, cols]).astype(F32)
                src = proj[GATE_PACE[c * len(GATE_PACE) // NCH]]
                r0 = (c * len(GATE_PACE) % NCH) * src.shape[0] // NCH // 8 * 8
                kf = jnp.concatenate([_after(src[r0:r0 + 8, :C], kf[:8]), kf[8:]], axis=0)
                ksh = kf * coef[0, rows, :]
                rolled = []
                for j in range(1, KS):
                    r = pltpu.roll(kf, j, 1)
                    rolled.append(r)
                    ksh = ksh + jnp.where(lane >= j, r, 0.0 if kprev is None else kprev[j - 1]) * coef[j, rows, :]
                kvs.append((ksh * _b(av[roww, cols]).astype(F32)).astype(BF16))
                kprev = rolled
            st["kv"] = kvs
            lhs = jnp.concatenate(kvs + [_b(ssm[roww, c * C:(c + 1) * C]) for c in range(NCH)], axis=0)
            both = _dot(lhs, _b(fwd[...]))
            xh = [both[c * G:(c + 1) * G] for c in range(NCH)]
            st["h"] = [both[(NCH + c) * G:(NCH + c + 1) * G] for c in range(NCH)]
            st["u"] = [xh[0]] + [
                xh[c] + jnp.concatenate([xh[c - 1][:, 2 * hc:3 * hc], -xh[c - 1][:, 3 * hc:], -xh[c - 1][:, :hc],
                                         xh[c - 1][:, hc:2 * hc]], axis=1) for c in range(1, NCH)]

        def inverse(todo):
            ws, tok = [], None
            for a in todo:
                slabs = []
                for r0 in range(0, G, 8):
                    rs = slice(r0, r0 + 8)
                    zr = zi = None
                    for c in range(a + 1):
                        ur, ui = st["u"][c][rs, :C], st["u"][c][rs, C:]
                        hr, hi = st["h"][a - c][rs, :C], st["h"][a - c][rs, C:]
                        if zr is None and tok is not None:
                            ur = _after(tok, ur)
                        pr = ur * hr - ui * hi
                        pi = ur * hi + ui * hr
                        zr = pr if zr is None else zr + pr
                        zi = pi if zi is None else zi + pi
                    tok = zr
                    slabs.append(jnp.concatenate([zr, zi], axis=1))
                ws.append(jnp.concatenate(slabs, axis=0).astype(BF16))
            ys = _dot(jnp.concatenate(ws, axis=0), _b(inv[...]))
            for t, a in enumerate(todo):
                cols = slice(a * C, (a + 1) * C)
                y = ys[t * G:(t + 1) * G] + st["kv"][a].astype(F32) * coef[KS, rows, :]
                aT[rows, cols] = _b(aq[roww, cols]).astype(F32) * y

        ops = {FWD_AT: forward}
        for step, todo in INV_AT.items():
            ops[step] = functools.partial(inverse, todo)
        return ops

    def head(h, carry):
        @pl.when(h == 1)
        def _():
            cp(wkv.at[1:], wkv.at[1:], s_late).wait()

        @pl.when(h >= 5)
        def _():
            a_copy(h - 5).start()

        proj, oacc = {}, {}
        conv = conv_ops(jnp.minimum(h, NG - 1), proj)
        wo = _b(woT[h])
        krow = jax.lax.broadcasted_iota(jnp.int32, (TQ, TQ), 0)
        qcol = jax.lax.broadcasted_iota(jnp.int32, (TQ, TQ), 1)
        causal = krow <= qcol
        ctx = {}

        def kproj(c):
            r = slice(c * KC // 2, (c + 1) * KC // 2)
            proj[2 * c] = _dot(_b(ckv[r, :]), _b(wks[...]))
            ks[r, :] = _w(proj[2 * c].astype(BF16))

        def vproj(c):
            r = slice(c * KC // 2, (c + 1) * KC // 2)
            proj[2 * c + 1] = jax.lax.dot_general(_b(wvs[...]), _b(ckv[r, :]), NT, preferred_element_type=F32)
            vTs[:, c * KC:(c + 1) * KC] = _w(proj[2 * c + 1].astype(BF16))

        def scores(i):
            n = TQ * (i + 1)
            sT = _dot(_b(ks[:n // 2, :]), _b(qs[h, :, TQ * i:n]))
            blocks = [sT[c0:c0 + TQ] for c0 in range(0, n - TQ, TQ)] + [jnp.where(causal, sT[n - TQ:], NEG)]
            m8, part = None, None
            for b, blk in enumerate(blocks):
                bm = jnp.max(blk.reshape(TQ // 8, 8, TQ), axis=0)
                m8 = bm if m8 is None else jnp.where(bm > m8, bm, m8)
                if b == i - PMAX:
                    part = m8[0:1]
            return blocks, m8, part

        def softmax(blocks, m8, pace):
            m8 = jnp.broadcast_to(jnp.max(m8, axis=0, keepdims=True), (8, TQ))
            ls, p, ps = None, None, []
            for b, blk in enumerate(blocks):
                if pace(b) is not None:
                    mm = _after(pace(b), m8)
                else:
                    mm = m8 if p is None else jnp.where(p[TQ - 8:] < 0.0, p[TQ - 8:], m8)
                p = jnp.exp2(blk - jnp.concatenate([mm] * (TQ // 8), axis=0))
                part = jnp.sum(p.reshape(TQ // 8, 8, TQ), axis=0)
                ls = part if ls is None else ls + part
                ps.append(p)
            return jnp.concatenate(ps, axis=0).astype(BF16), 1.0 / jnp.sum(ls, axis=0, keepdims=True)

        def pv(i, p, rl):
            n = TQ * (i + 1)
            halves = [_dot(_b(vTs[t * D // 4:(t + 1) * D // 4, :n]), p) * rl for t in range(2)]
            ctx[i] = jnp.concatenate(halves, axis=0).astype(BF16)

        def oproj(i0, i1):
            for i in range(i0, i1):
                oacc[i] = _dot(wo, ctx[i])
                acc[:, TQ * i:TQ * (i + 1)] += oacc[i]

        def by_scores(blocks):
            return lambda b: blocks[(b - JIT0) // 2][(b - JIT0) % 2 * 64:][:8] if b >= JIT0 else None

        def by_oproj(i0):
            return lambda b: oacc[i0 + 2 * (TAIL_PACE * b // DA)][TAIL_PACE * b % DA // 8 * 8:][:8]

        kproj(0)
        vproj(0)
        st = None
        for i in range(NQ):
            if i + 2 < NQ:
                (vproj if i & 1 else kproj)(i // 2 + 1)
            if i in OFILL:
                oproj(*OFILL[i])
            prev, st = st, scores(i)
            if i > 0:
                p, rl = softmax(*prev[:2], by_scores(st[0]))
            if i > 0 and st[2] is not None:
                rl = _after(st[2], rl)
            if i in conv:
                conv[i]()
            if i > 0:
                pv(i - 1, p, rl)
        a_transpose(jnp.maximum(h - 4, 0))
        prep_wkv(jnp.minimum(h + 1, H - 1))
        oproj(OFILL[NQ - 1][1], OSPLIT)
        p, rl = softmax(*st[:2], by_oproj(OFILL[NQ - 1][1]))
        pv(NQ - 1, p, rl)
        oproj(OSPLIT, NQ)
        return carry

    jax.lax.fori_loop(0, H, head, 0)

    a_copy(11).start()
    c_out = [a_copy(p) for p in range(12)]
    for i0, i1 in OUT_CHUNKS:
        cols = slice(i0 * TQ, i1 * TQ)
        blk = jnp.concatenate([aT[NA:, cols], acc[:, cols]], axis=0).astype(BF16)
        outs[cols, NA:] = _b(_w(blk)).T
        c = cp(outs.at[cols, NA:], out_hbm.at[cols, NA:], s_out)
        c.start()
        c_out.append(c)
    for c in c_out:
        c.wait()


@jax.jit
def pallas_concat_heads__ssm_conv_h3__compressed_kv_cla__prompt_kernel(
    A_q: jax.Array,
    A_k: jax.Array,
    A_v: jax.Array,
    A_shift_k: jax.Array,
    A_ssm_k: jax.Array,
    A_ssm_D: jax.Array,
    B_x: jax.Array,
    B_c_kv: jax.Array,
    B_w_q: jax.Array,
    B_w_uk: jax.Array,
    B_w_uv: jax.Array,
    B_w_o: jax.Array,
):
    fwd, inv = _dft_mats()
    tr = lambda a: jnp.swapaxes(a, 1, 2).reshape(DA, S)
    any_spec = pl.BlockSpec(memory_space=pl.ANY)
    out = pl.pallas_call(
        _kernel,
        out_shape=jax.ShapeDtypeStruct((S, 2 * DA), BF16),
        in_specs=[any_spec] * 14,
        out_specs=any_spec,
        scratch_shapes=[
            pltpu.VMEM((DA // 2, S), U32),
            pltpu.VMEM((DA // 2, S), U32),
            pltpu.VMEM((DA // 2, S), U32),
            pltpu.VMEM((DA // 2, S), U32),
            pltpu.VMEM((DA // 2, S), U32),
            pltpu.VMEM((S // 2, DC), U32),
            pltpu.VMEM((H // 2, DA, D), U32),
            pltpu.VMEM((H // 2, 2, DC, D), U32),
            pltpu.VMEM((H, DA // 2, D), U32),
            pltpu.VMEM((D, DA), U32),
            pltpu.VMEM((H, D // 2, S), U32),
            pltpu.VMEM((S // 2, D), U32),
            pltpu.VMEM((D // 2, S), U32),
            pltpu.VMEM((DA, S), F32),
            pltpu.VMEM((DA, S), F32),
            pltpu.VMEM((KS + 1, DA, 128), F32),
            pltpu.VMEM((DC // 2, D), U32),
            pltpu.VMEM((D // 2, DC), U32),
            pltpu.VMEM((S, 2 * DA), BF16),
            pltpu.VMEM((KS, DA), BF16),
            pltpu.VMEM((DA,), BF16),
            pltpu.VMEM((C // 2, 2 * C), U32),
            pltpu.VMEM((C, C), U32),
            pltpu.SemaphoreType.DMA((8,)),
        ],
        compiler_params=pltpu.CompilerParams(vmem_limit_bytes=100 * 1024 * 1024),
    )(
        tr(A_q), tr(A_k), tr(A_v), A_shift_k.T, A_ssm_k, A_ssm_D, tr(B_x), B_c_kv.reshape(S, DC),
        B_w_q, B_w_uk, B_w_uv,
        jnp.swapaxes(B_w_o, 1, 2), jnp.asarray(fwd, BF16), jnp.asarray(inv, BF16),
    )
    return out.reshape(1, S, 2 * DA)
```

```python
import functools
import math

import jax
import jax.numpy as jnp
import numpy as np
import jax.experimental.pallas as pl
import jax.experimental.pallas.tpu as pltpu

F32 = jnp.float32
BF16 = jnp.bfloat16
U32 = jnp.uint32

S = 2048
DA = 448
H = 16
D = 256
DC = 1024
KS = 4
C = 128
NCH = S // C
G = 32
NG = DA // G
TQ = 128
NQ = S // TQ
KC = 256
NA = 384
NT = (((1,), (1,)), ((), ()))
LOG2E = math.log2(math.e)
QSCALE = (D ** -0.5) * LOG2E
NEG = -1e9 * LOG2E

X_CHUNKS = ((0, 384), (384, 1152), (1152, 2048))
T0 = 2
HB = 4
NB = 5
FWD_AT = 2
INV_AT = {4: (0, 1, 2, 3, 4), 5: (5, 6), **{a - 1: (a,) for a in range(7, 15)}, 15: (15,)}
OFILL = {15: (2, 4)}
OSPLIT = 12
PMAX = 3
JIT0 = 3
GATE_PACE = (1, 2, 3)
TAIL_PACE = 24
OUT_PACE = 200


def _dft_mats():
    k = np.concatenate([np.arange(0, C, 2), np.arange(1, C, 2)]).astype(np.float64)
    n = np.arange(C, dtype=np.float64)
    th = 2.0 * np.pi * np.outer(n, k + 0.5) / (2 * C)
    fwd = np.concatenate([np.cos(th), np.sin(th)], axis=1)
    inv = fwd.T / C
    return fwd, inv


def _b(x):
    return pltpu.bitcast(x, BF16)


def _w(x):
    return pltpu.bitcast(x, U32)


def _dot(a, b):
    return jnp.dot(a, b, preferred_element_type=F32)


def _after(tok, x):
    return jnp.where(jnp.abs(tok) < -1.0, tok, x)


def _kernel(qT_hbm, kT_hbm, vT_hbm, shT_hbm, ssm_hbm, dvec_hbm, xT_hbm, ckv_hbm, wq_hbm, wuk_hbm, wuv_hbm,
            woT_hbm, fwd_hbm, inv_hbm,
            out_hbm,
            aq, ak, av, ssm, xT, ckv, wq, wkv, woT, wqs, qs, ks, vTs, k0s, v0s, acc, aT, coef, wks, wvs,
            outs, shT, dvec, fwd, inv, sems):
    def cp(src, dst, sem):
        return pltpu.make_async_copy(src, dst, sems.at[sem])

    s_wq0, s_x, s_wq, s_early, s_late, s_out = 0, 1, 4, 5, 6, 7
    wq_u, wuk_u, wuv_u, x_u = (r.bitcast(U32) for r in (wq_hbm, wuk_hbm, wuv_hbm, xT_hbm))
    c_wq0 = cp(wq_u.at[:, 0, :], wq.at[0], s_wq0)
    c_x = [[cp(x_u.at[:, c0:c1], xT.at[:, c0:c1], s_x + t)] for t, (c0, c1) in enumerate(X_CHUNKS)]
    c_x[-1] += [cp(wq_u.at[:, j, :], wq.at[j], s_x + 2) for j in (1, 2)]
    c_wq = [cp(wq_u.at[:, j, :], wq.at[j], s_wq) for j in range(3, H // 2)]
    early = [cp(src, dst, s_early) for src, dst in (
        (shT_hbm, shT), (dvec_hbm, dvec), (fwd_hbm.bitcast(U32), fwd), (inv_hbm.bitcast(U32), inv),
        (wuk_u.at[:, 0, :], wkv.at[0, 0]), (wuv_u.at[:, 0, :], wkv.at[0, 1]), (ckv_hbm.bitcast(U32), ckv),
        (woT_hbm.bitcast(U32), woT), (kT_hbm.bitcast(U32), ak), (vT_hbm.bitcast(U32), av),
        (ssm_hbm.bitcast(U32), ssm), (qT_hbm.bitcast(U32), aq))]
    late = [cp(src.at[:, j, :], wkv.at[j, t], s_late)
            for j in range(1, H // 2) for t, src in enumerate((wuk_u, wuv_u))]
    for c in [c_wq0, *c_x[0], *c_x[1], *c_x[2], *c_wq, *early, *late]:
        c.start()

    hi_mask = jnp.uint32(0xFFFF0000)

    def prep_wq(j):
        w = wq[j]
        wqs[:D // 2, :] = _w(pltpu.bitcast(w << 16, F32).T.astype(BF16))
        wqs[D // 2:, :] = _w(pltpu.bitcast(w & hi_mask, F32).T.astype(BF16))

    def prep_wkv(h):
        j = h >> 1
        sh = jnp.asarray(16 - 16 * (h & 1), U32)
        wks[...] = _w(pltpu.bitcast((wkv[j, 0] << sh) & hi_mask, F32).astype(BF16))
        wvs[...] = _w(pltpu.bitcast((wkv[j, 1] << sh) & hi_mask, F32).T.astype(BF16))

    def qproj(j, c0, c1):
        q2 = (_dot(_b(wqs[...]), _b(xT[:, c0:c1])) * QSCALE).astype(BF16)
        qs[2 * j, :, c0:c1] = _w(q2[:D])
        qs[2 * j + 1, :, c0:c1] = _w(q2[D:])

    acc[...] = jnp.zeros(acc.shape, F32)
    aT[:128, :] = jnp.zeros((128, S), F32)

    c_wq0.wait()
    prep_wq(0)
    for cs, (c0, c1) in zip(c_x, X_CHUNKS):
        for c in cs:
            c.wait()
        qproj(0, c0, c1)
    prep_wq(1)

    def qpair(j, carry):
        @pl.when(j == 2)
        def _():
            cp(wq.at[3:], wq.at[3:], s_wq).wait()

        qproj(j, 0, S)
        prep_wq(j + 1)
        return carry

    jax.lax.fori_loop(1, H // 2 - 1, qpair, 0)

    for c in early:
        c.wait()
    qproj(H // 2 - 1, 0, S)
    prep_wkv(0)
    taps = shT[...].astype(F32)
    for j in range(KS + 1):
        row = taps[j:j + 1] if j < KS else dvec[...].astype(F32)[None, :]
        coef[j] = jnp.broadcast_to(row, (128, DA)).T

    def a_piece(p):
        r = pl.ds(pl.multiple_of((p & 3) * (S // 4), S // 4), S // 4)
        c = pl.ds(pl.multiple_of((p >> 2) * 128, 128), 128)
        return r, c

    def a_copy(p):
        r, c = a_piece(p)
        return cp(outs.at[r, c], out_hbm.at[r, c], s_out)

    def a_transpose(p):
        r, c = a_piece(p)
        outs[r, c] = _b(_w(aT[c, r].astype(BF16))).T

    def conv_ops(g, proj):
        rows = pl.ds(pl.multiple_of(g * G, G), G)
        roww = pl.ds(pl.multiple_of(g * (G // 2), G // 2), G // 2)
        lane = jax.lax.broadcasted_iota(jnp.int32, (G, C), 1)
        hc = C // 2
        st = {}

        def forward():
            kvs, kprev = [], None
            for c in range(NCH):
                cols = slice(c * C, (c + 1) * C)
                kf = _b(ak[roww, cols]).astype(F32)
                src = proj[GATE_PACE[c * len(GATE_PACE) // NCH]]
                r0 = (c * len(GATE_PACE) % NCH) * src.shape[0] // NCH // 8 * 8
                kf = jnp.concatenate([_after(src[r0:r0 + 8, :C], kf[:8]), kf[8:]], axis=0)
                ksh = kf * coef[0, rows, :]
                rolled = []
                for j in range(1, KS):
                    r = pltpu.roll(kf, j, 1)
                    rolled.append(r)
                    ksh = ksh + jnp.where(lane >= j, r, 0.0 if kprev is None else kprev[j - 1]) * coef[j, rows, :]
                kvs.append((ksh * _b(av[roww, cols]).astype(F32)).astype(BF16))
                kprev = rolled
            st["kv"] = kvs
            lhs = jnp.concatenate(kvs + [_b(ssm[roww, c * C:(c + 1) * C]) for c in range(NCH)], axis=0)
            both = _dot(lhs, _b(fwd[...]))
            xh = [both[c * G:(c + 1) * G] for c in range(NCH)]
            st["h"] = [both[(NCH + c) * G:(NCH + c + 1) * G] for c in range(NCH)]
            st["u"] = [xh[0]] + [
                xh[c] + jnp.concatenate([xh[c - 1][:, 2 * hc:3 * hc], -xh[c - 1][:, 3 * hc:], -xh[c - 1][:, :hc],
                                         xh[c - 1][:, hc:2 * hc]], axis=1) for c in range(1, NCH)]

        def inverse(todo):
            ws, tok = [], None
            for a in todo:
                slabs = []
                for r0 in range(0, G, 8):
                    rs = slice(r0, r0 + 8)
                    zr = zi = None
                    for c in range(a + 1):
                        ur, ui = st["u"][c][rs, :C], st["u"][c][rs, C:]
                        hr, hi = st["h"][a - c][rs, :C], st["h"][a - c][rs, C:]
                        if zr is None and tok is not None:
                            ur = _after(tok, ur)
                        pr = ur * hr - ui * hi
                        pi = ur * hi + ui * hr
                        zr = pr if zr is None else zr + pr
                        zi = pi if zi is None else zi + pi
                    tok = zr
                    slabs.append(jnp.concatenate([zr, zi], axis=1))
                ws.append(jnp.concatenate(slabs, axis=0).astype(BF16))
            ys = _dot(jnp.concatenate(ws, axis=0), _b(inv[...]))
            for t, a in enumerate(todo):
                cols = slice(a * C, (a + 1) * C)
                y = ys[t * G:(t + 1) * G] + st["kv"][a].astype(F32) * coef[KS, rows, :]
                aT[rows, cols] = _b(aq[roww, cols]).astype(F32) * y

        ops = {FWD_AT: forward}
        for step, todo in INV_AT.items():
            ops[step] = functools.partial(inverse, todo)
        return ops

    def causal_mask():
        krow = jax.lax.broadcasted_iota(jnp.int32, (TQ, TQ), 0)
        qcol = jax.lax.broadcasted_iota(jnp.int32, (TQ, TQ), 1)
        return krow <= qcol

    def scores(i, k, q, causal):
        n = TQ * (i + 1)
        sT = _dot(k, q)
        blocks = [sT[c0:c0 + TQ] for c0 in range(0, n - TQ, TQ)] + [jnp.where(causal, sT[n - TQ:], NEG)]
        m8, part = None, None
        for b, blk in enumerate(blocks):
            bm = jnp.max(blk.reshape(TQ // 8, 8, TQ), axis=0)
            m8 = bm if m8 is None else jnp.where(bm > m8, bm, m8)
            if b == i - PMAX:
                part = m8[0:1]
        return blocks, m8, part

    def softmax(blocks, m8, pace):
        m8 = jnp.broadcast_to(jnp.max(m8, axis=0, keepdims=True), (8, TQ))
        ls, p, ps = None, None, []
        for b, blk in enumerate(blocks):
            if pace(b) is not None:
                mm = _after(pace(b), m8)
            else:
                mm = m8 if p is None else jnp.where(p[TQ - 8:] < 0.0, p[TQ - 8:], m8)
            p = jnp.exp2(blk - jnp.concatenate([mm] * (TQ // 8), axis=0))
            part = jnp.sum(p.reshape(TQ // 8, 8, TQ), axis=0)
            ls = part if ls is None else ls + part
            ps.append(p)
        return jnp.concatenate(ps, axis=0).astype(BF16), 1.0 / jnp.sum(ls, axis=0, keepdims=True)

    def context(vT, p, rl):
        halves = [_dot(_b(vT(t * D // 4, (t + 1) * D // 4)), p) * rl for t in range(2)]
        return jnp.concatenate(halves, axis=0).astype(BF16)

    def head(h, carry):
        @pl.when(h == 1)
        def _():
            cp(wkv.at[1:], wkv.at[1:], s_late).wait()

        @pl.when(h >= 5)
        def _():
            a_copy(h - 5).start()

        proj, oacc, ctx = {}, {}, {}
        conv = conv_ops(jnp.minimum(h, NG - 1), proj)
        wo = _b(woT[h])
        causal = causal_mask()

        def project(n):
            c = n // 2
            r = slice(c * KC // 2, (c + 1) * KC // 2)
            if n % 2 == 0:
                proj[n] = _dot(_b(ckv[r, :]), _b(wks[...]))
                ks[r, :] = _w(proj[n].astype(BF16))
                if c == 0:
                    k0s[h] = ks[r, :]
            else:
                proj[n] = jax.lax.dot_general(_b(wvs[...]), _b(ckv[r, :]), NT, preferred_element_type=F32)
                vTs[:, c * KC:(c + 1) * KC] = _w(proj[n].astype(BF16))
                if c == 0:
                    v0s[h] = vTs[:, :KC]

        def pv(i, p, rl):
            ctx[i] = context(lambda r0, r1: vTs[r0:r1, :TQ * (i + 1)], p, rl)

        def oproj(i0, i1):
            for i in range(i0, i1):
                oacc[i] = _dot(wo, ctx[i])
                acc[:, TQ * i:TQ * (i + 1)] += oacc[i]

        def by_scores(blocks):
            return lambda b: blocks[(b - JIT0) // 2][(b - JIT0) % 2 * 64:][:8] if b >= JIT0 else None

        def by_oproj(i0):
            return lambda b: oacc[i0 + 2 * (TAIL_PACE * b // DA)][TAIL_PACE * b % DA // 8 * 8:][:8]

        for n in range(T0 + 1):
            project(n)
        st = None
        for i in range(T0, NQ):
            if i + 1 < NQ:
                project(i + 1)
            if i in OFILL:
                oproj(*OFILL[i])
            prev, st = st, scores(i, _b(ks[:TQ * (i + 1) // 2, :]), _b(qs[h, :, TQ * i:TQ * (i + 1)]), causal)
            if i > T0:
                p, rl = softmax(*prev[:2], by_scores(st[0]))
                if st[2] is not None:
                    rl = _after(st[2], rl)
            if i in conv:
                conv[i]()
            if i > T0:
                pv(i - 1, p, rl)
        a_transpose(jnp.maximum(h - 4, 0))
        prep_wkv(jnp.minimum(h + 1, H - 1))
        oproj(OFILL[NQ - 1][1], OSPLIT)
        p, rl = softmax(*st[:2], by_oproj(OFILL[NQ - 1][1]))
        pv(NQ - 1, p, rl)
        oproj(OSPLIT, NQ)
        return carry

    jax.lax.fori_loop(0, H, head, 0)

    def b_transpose(src, dst, tok=None):
        blk = jnp.concatenate([aT[NA:, src], acc[:, src]], axis=0)
        if tok is not None:
            blk = jnp.concatenate([x for r in range(0, 2 * DA - NA, 128)
                                   for x in (_after(tok, blk[r:r + 8]), blk[r + 8:r + 128])], axis=0)
        blk = blk.astype(BF16)
        outs[dst, NA:] = _b(_w(blk)).T

    def b_copy(i0, i1):
        return cp(outs.at[i0 * TQ:i1 * TQ, NA:], out_hbm.at[i0 * TQ:i1 * TQ, NA:], s_out)

    nsteps = H // HB
    c_b = [b_copy(T0 + NB * t, min(T0 + NB * (t + 1), NQ)) for t in range(nsteps - 1)]
    a_copy(11).start()

    def first_tiles(t, carry):
        for u in range(nsteps - 1):
            pl.when(t == u + 1)(c_b[u].start)
        causal = causal_mask()
        items = [(HB * t + u, i) for u in range(HB) for i in range(T0)]
        sts = [scores(i, _b(k0s[h, :TQ * (i + 1) // 2, :]), _b(qs[h, :, TQ * i:TQ * (i + 1)]), causal)
               for h, i in items]
        ctxs = [context(lambda r0, r1: v0s[h, r0:r1, :TQ * (i + 1)], *softmax(*st[:2], lambda b: None))
                for (h, i), st in zip(items, sts)]
        o, ds = {}, []
        for (h, i), c in zip(items, ctxs):
            ds.append(_dot(_b(woT[h]), c))
            o[i] = ds[-1] if i not in o else o[i] + ds[-1]
        for k in range(NB):
            cb = T0 + NB * t + k
            tok = ds[2 * (OUT_PACE * k // DA)][OUT_PACE * k % DA // 8 * 8:][:8]
            b_transpose(pl.ds(pl.multiple_of(jnp.minimum(cb, NQ - 1) * TQ, TQ), TQ),
                        pl.ds(pl.multiple_of(cb * TQ, TQ), TQ), tok)
        for i in range(T0):
            acc[:, TQ * i:TQ * (i + 1)] += o[i]
        return carry

    jax.lax.fori_loop(0, nsteps, first_tiles, 0)

    c_last = []
    for i in range(T0):
        b_transpose(slice(i * TQ, (i + 1) * TQ), slice(i * TQ, (i + 1) * TQ))
        c_last.append(b_copy(i, i + 1))
        c_last[-1].start()
    for c in [a_copy(p) for p in range(12)] + c_b + c_last:
        c.wait()


@jax.jit
def pallas_concat_heads__ssm_conv_h3__compressed_kv_cla__prompt_kernel(
    A_q: jax.Array,
    A_k: jax.Array,
    A_v: jax.Array,
    A_shift_k: jax.Array,
    A_ssm_k: jax.Array,
    A_ssm_D: jax.Array,
    B_x: jax.Array,
    B_c_kv: jax.Array,
    B_w_q: jax.Array,
    B_w_uk: jax.Array,
    B_w_uv: jax.Array,
    B_w_o: jax.Array,
):
    fwd, inv = _dft_mats()
    tr = lambda a: jnp.swapaxes(a, 1, 2).reshape(DA, S)
    any_spec = pl.BlockSpec(memory_space=pl.ANY)
    out = pl.pallas_call(
        _kernel,
        out_shape=jax.ShapeDtypeStruct((S, 2 * DA), BF16),
        in_specs=[any_spec] * 14,
        out_specs=any_spec,
        scratch_shapes=[
            pltpu.VMEM((DA // 2, S), U32),
            pltpu.VMEM((DA // 2, S), U32),
            pltpu.VMEM((DA // 2, S), U32),
            pltpu.VMEM((DA // 2, S), U32),
            pltpu.VMEM((DA // 2, S), U32),
            pltpu.VMEM((S // 2, DC), U32),
            pltpu.VMEM((H // 2, DA, D), U32),
            pltpu.VMEM((H // 2, 2, DC, D), U32),
            pltpu.VMEM((H, DA // 2, D), U32),
            pltpu.VMEM((D, DA), U32),
            pltpu.VMEM((H, D // 2, S), U32),
            pltpu.VMEM((S // 2, D), U32),
            pltpu.VMEM((D // 2, S), U32),
            pltpu.VMEM((H, KC // 2, D), U32),
            pltpu.VMEM((H, D // 2, KC), U32),
            pltpu.VMEM((DA, S), F32),
            pltpu.VMEM((DA, S), F32),
            pltpu.VMEM((KS + 1, DA, 128), F32),
            pltpu.VMEM((DC // 2, D), U32),
            pltpu.VMEM((D // 2, DC), U32),
            pltpu.VMEM(((T0 + NB * H // HB) * TQ, 2 * DA), BF16),
            pltpu.VMEM((KS, DA), BF16),
            pltpu.VMEM((DA,), BF16),
            pltpu.VMEM((C // 2, 2 * C), U32),
            pltpu.VMEM((C, C), U32),
            pltpu.SemaphoreType.DMA((8,)),
        ],
        compiler_params=pltpu.CompilerParams(vmem_limit_bytes=100 * 1024 * 1024),
    )(
        tr(A_q), tr(A_k), tr(A_v), A_shift_k.T, A_ssm_k, A_ssm_D, tr(B_x), B_c_kv.reshape(S, DC),
        B_w_q, B_w_uk, B_w_uv,
        jnp.swapaxes(B_w_o, 1, 2), jnp.asarray(fwd, BF16), jnp.asarray(inv, BF16),
    )
    return out.reshape(1, S, 2 * DA)
```

```python
import functools
import math

import jax
import jax.numpy as jnp
import numpy as np
import jax.experimental.pallas as pl
import jax.experimental.pallas.tpu as pltpu

F32 = jnp.float32
BF16 = jnp.bfloat16
U32 = jnp.uint32

S = 2048
DA = 448
H = 16
D = 256
DC = 1024
KS = 4
C = 128
NCH = S // C
GQ = 32
GH = 16
RQ = GQ * (H // 2 - 2)
TQ = 128
NQ = S // TQ
KC = 256
NA = 384
NT = (((1,), (1,)), ((), ()))
LOG2E = math.log2(math.e)
QSCALE = (D ** -0.5) * LOG2E
NEG = -1e9 * LOG2E

X_CHUNKS = ((0, 384), (384, 1152), (1152, 2048))
Q_FWD_AT = 2
Q_INV_AT = {6: (0, 1, 2, 3, 4, 5), 7: (6, 7), 8: (8, 9), **{a - 1: (a,) for a in range(10, NCH)}}
Q_GATE_PACE = (0, 1)
T0 = 2
HB = 4
NB = 5
FWD_AT = 3
INV_AT = {6: (0, 1, 2, 3), 7: (4, 5, 6), 8: (7, 8), **{a: (a,) for a in range(9, NCH)}}
OFILL = {15: (2, 4)}
OSPLIT = 12
PMAX = 3
JIT0 = 4
TAIL_PACE = 32
OUT_PACE = 200


def _dft_mats():
    k = np.concatenate([np.arange(0, C, 2), np.arange(1, C, 2)]).astype(np.float64)
    n = np.arange(C, dtype=np.float64)
    th = 2.0 * np.pi * np.outer(n, k + 0.5) / (2 * C)
    fwd = np.concatenate([np.cos(th), np.sin(th)], axis=1)
    inv = fwd.T / C
    return fwd, inv


def _b(x):
    return pltpu.bitcast(x, BF16)


def _w(x):
    return pltpu.bitcast(x, U32)


def _dot(a, b):
    return jnp.dot(a, b, preferred_element_type=F32)


def _after(tok, x):
    return jnp.where(jnp.abs(tok) < -1.0, tok, x)


def _kernel(qT_hbm, kT_hbm, vT_hbm, shT_hbm, ssm_hbm, dvec_hbm, xT_hbm, ckv_hbm, wq_hbm, wuk_hbm, wuv_hbm,
            woT_hbm, fwd_hbm, inv_hbm,
            out_hbm,
            aq, ak, av, ssm, xT, ckv, wq, wkv, woT, wqs, qs, ks, vTs, k0s, v0s, acc, aT, coef, wks, wvs,
            outs, shT, dvec, fwd, inv, sems):
    def cp(src, dst, sem):
        return pltpu.make_async_copy(src, dst, sems.at[sem])

    s_wq0, s_x, s_a0, s_wq, s_early, s_late, s_out = 0, 1, 4, 5, 6, 7, 8
    wq_u, wuk_u, wuv_u, x_u = (r.bitcast(U32) for r in (wq_hbm, wuk_hbm, wuv_hbm, xT_hbm))
    a_in = [(r.bitcast(U32), d) for r, d in ((kT_hbm, ak), (vT_hbm, av), (ssm_hbm, ssm), (qT_hbm, aq))]

    def a_rows(r0, r1, sem):
        return [cp(src.at[r0 // 2:r1 // 2], dst.at[r0 // 2:r1 // 2], sem) for src, dst in a_in]

    c_wq0 = cp(wq_u.at[:, 0, :], wq.at[0], s_wq0)
    c_x = [[cp(x_u.at[:, c0:c1], xT.at[:, c0:c1], s_x + t)] for t, (c0, c1) in enumerate(X_CHUNKS)]
    c_x[-1] += [cp(wq_u.at[:, j, :], wq.at[j], s_x + 2) for j in (1, 2)]
    c_x[-1] += [cp(shT_hbm, shT, s_x + 2), cp(dvec_hbm, dvec, s_x + 2)]
    c_a0 = [cp(fwd_hbm.bitcast(U32), fwd, s_a0), cp(inv_hbm.bitcast(U32), inv, s_a0)] + a_rows(0, GQ, s_a0)
    c_wq = a_rows(GQ, RQ, s_wq) + [cp(wq_u.at[:, j, :], wq.at[j], s_wq) for j in range(3, H // 2)]
    early = [cp(src, dst, s_early) for src, dst in (
        (wuk_u.at[:, 0, :], wkv.at[0, 0]), (wuv_u.at[:, 0, :], wkv.at[0, 1]), (ckv_hbm.bitcast(U32), ckv),
        (woT_hbm.bitcast(U32), woT))] + a_rows(RQ, DA, s_early)
    late = [cp(src.at[:, j, :], wkv.at[j, t], s_late)
            for j in range(1, H // 2) for t, src in enumerate((wuk_u, wuv_u))]
    for c in [c_wq0, *c_x[0], *c_x[1], *c_x[2], *c_a0, *c_wq, *early, *late]:
        c.start()

    hi_mask = jnp.uint32(0xFFFF0000)

    def prep_wq(j):
        w = wq[j]
        wqs[:D // 2, :] = _w(pltpu.bitcast(w << 16, F32).T.astype(BF16))
        wqs[D // 2:, :] = _w(pltpu.bitcast(w & hi_mask, F32).T.astype(BF16))

    def prep_wkv(h):
        j = h >> 1
        sh = jnp.asarray(16 - 16 * (h & 1), U32)
        wks[...] = _w(pltpu.bitcast((wkv[j, 0] << sh) & hi_mask, F32).astype(BF16))
        wvs[...] = _w(pltpu.bitcast((wkv[j, 1] << sh) & hi_mask, F32).T.astype(BF16))

    def qproj(j, c0, c1):
        q = _dot(_b(wqs[...]), _b(xT[:, c0:c1]))
        q2 = (q * QSCALE).astype(BF16)
        qs[2 * j, :, c0:c1] = _w(q2[:D])
        qs[2 * j + 1, :, c0:c1] = _w(q2[D:])
        return q

    def zero(i, carry):
        acc[pl.ds(pl.multiple_of(i * 32, 32), 32), :] = jnp.zeros((32, S), F32)
        return carry

    jax.lax.fori_loop(0, DA // 32, zero, 0)

    def conv_ops(row0, G, proj, pace, fwd_at, inv_at):
        rows = pl.ds(pl.multiple_of(row0, 16), G)
        roww = pl.ds(pl.multiple_of(row0 >> 1, 8), G // 2)
        lane = jax.lax.broadcasted_iota(jnp.int32, (G, C), 1)
        hc = C // 2
        st = {}

        def forward():
            kvs, kprev = [], None
            for c in range(NCH):
                cols = slice(c * C, (c + 1) * C)
                kf = _b(ak[roww, cols]).astype(F32)
                if pace:
                    src = proj[pace[c * len(pace) // NCH]]
                    r0 = (c * len(pace) % NCH) * src.shape[0] // NCH // 8 * 8
                    kf = jnp.concatenate([_after(src[r0:r0 + 8, :C], kf[:8]), kf[8:]], axis=0)
                ksh = kf * coef[0, rows, :]
                rolled = []
                for j in range(1, KS):
                    r = pltpu.roll(kf, j, 1)
                    rolled.append(r)
                    ksh = ksh + jnp.where(lane >= j, r, 0.0 if kprev is None else kprev[j - 1]) * coef[j, rows, :]
                kvs.append((ksh * _b(av[roww, cols]).astype(F32)).astype(BF16))
                kprev = rolled
            st["kv"] = kvs
            lhs = jnp.concatenate(kvs + [_b(ssm[roww, c * C:(c + 1) * C]) for c in range(NCH)], axis=0)
            both = _dot(lhs, _b(fwd[...]))
            xh = [both[c * G:(c + 1) * G] for c in range(NCH)]
            st["h"] = [both[(NCH + c) * G:(NCH + c + 1) * G] for c in range(NCH)]
            st["u"] = [xh[0]] + [
                xh[c] + jnp.concatenate([xh[c - 1][:, 2 * hc:3 * hc], -xh[c - 1][:, 3 * hc:], -xh[c - 1][:, :hc],
                                         xh[c - 1][:, hc:2 * hc]], axis=1) for c in range(1, NCH)]

        def inverse(todo):
            ws, tok = [], None
            for a in todo:
                slabs = []
                for r0 in range(0, G, 8):
                    rs = slice(r0, r0 + 8)
                    zr = zi = None
                    for c in range(a + 1):
                        ur, ui = st["u"][c][rs, :C], st["u"][c][rs, C:]
                        hr, hi = st["h"][a - c][rs, :C], st["h"][a - c][rs, C:]
                        if zr is None and tok is not None:
                            ur = _after(tok, ur)
                        pr = ur * hr - ui * hi
                        pi = ur * hi + ui * hr
                        zr = pr if zr is None else zr + pr
                        zi = pi if zi is None else zi + pi
                    tok = zr
                    slabs.append(jnp.concatenate([zr, zi], axis=1))
                ws.append(jnp.concatenate(slabs, axis=0).astype(BF16))
            ys = _dot(jnp.concatenate(ws, axis=0), _b(inv[...]))
            for t, a in enumerate(todo):
                cols = slice(a * C, (a + 1) * C)
                y = ys[t * G:(t + 1) * G] + st["kv"][a].astype(F32) * coef[KS, rows, :]
                aT[rows, cols] = _b(aq[roww, cols]).astype(F32) * y

        ops = {fwd_at: forward}
        for step, todo in inv_at.items():
            ops[step] = functools.partial(inverse, todo)
        return ops

    c_wq0.wait()
    prep_wq(0)
    for cs, (c0, c1) in zip(c_x, X_CHUNKS):
        for c in cs:
            c.wait()
        qproj(0, c0, c1)
    prep_wq(1)
    taps = shT[...].astype(F32)
    for j in range(KS + 1):
        row = taps[j:j + 1] if j < KS else dvec[...].astype(F32)[None, :]
        coef[j] = jnp.broadcast_to(row, (128, DA)).T
    for c in c_a0:
        c.wait()

    def qpair(j, carry):
        @pl.when(j == 2)
        def _():
            for c in c_wq:
                c.wait()

        qv = {}
        conv = conv_ops((j - 1) * GQ, GQ, qv, Q_GATE_PACE, Q_FWD_AT, Q_INV_AT)
        for p in range(NQ):
            qv[p] = qproj(j, p * TQ, (p + 1) * TQ)
            if p in conv:
                conv[p]()
        prep_wq(j + 1)
        return carry

    jax.lax.fori_loop(1, H // 2 - 1, qpair, 0)

    for c in early:
        c.wait()
    qproj(H // 2 - 1, 0, S)
    prep_wkv(0)

    def a_piece(p):
        r = pl.ds(pl.multiple_of((p & 3) * (S // 4), S // 4), S // 4)
        c = pl.ds(pl.multiple_of((p >> 2) * 128, 128), 128)
        return r, c

    def a_copy(p):
        r, c = a_piece(p)
        return cp(outs.at[r, c], out_hbm.at[r, c], s_out)

    def a_transpose(p):
        r, c = a_piece(p)
        outs[r, c] = _b(_w(aT[c, r].astype(BF16))).T

    def causal_mask():
        krow = jax.lax.broadcasted_iota(jnp.int32, (TQ, TQ), 0)
        qcol = jax.lax.broadcasted_iota(jnp.int32, (TQ, TQ), 1)
        return krow <= qcol

    def scores(i, k, q, causal):
        n = TQ * (i + 1)
        sT = _dot(k, q)
        blocks = [sT[c0:c0 + TQ] for c0 in range(0, n - TQ, TQ)] + [jnp.where(causal, sT[n - TQ:], NEG)]
        m8, part = None, None
        for b, blk in enumerate(blocks):
            bm = jnp.max(blk.reshape(TQ // 8, 8, TQ), axis=0)
            m8 = bm if m8 is None else jnp.where(bm > m8, bm, m8)
            if b == i - PMAX:
                part = m8[0:1]
        return blocks, m8, part

    def softmax(blocks, m8, pace):
        m8 = jnp.broadcast_to(jnp.max(m8, axis=0, keepdims=True), (8, TQ))
        ls, p, ps = None, None, []
        for b, blk in enumerate(blocks):
            if pace(b) is not None:
                mm = _after(pace(b), m8)
            else:
                mm = m8 if p is None else jnp.where(p[TQ - 8:] < 0.0, p[TQ - 8:], m8)
            p = jnp.exp2(blk - jnp.concatenate([mm] * (TQ // 8), axis=0))
            part = jnp.sum(p.reshape(TQ // 8, 8, TQ), axis=0)
            ls = part if ls is None else ls + part
            ps.append(p)
        return jnp.concatenate(ps, axis=0).astype(BF16), 1.0 / jnp.sum(ls, axis=0, keepdims=True)

    def context(vT, p, rl):
        halves = [_dot(_b(vT(t * D // 4, (t + 1) * D // 4)), p) * rl for t in range(2)]
        return jnp.concatenate(halves, axis=0).astype(BF16)

    def head(h, carry):
        @pl.when(h == 1)
        def _():
            cp(wkv.at[1:], wkv.at[1:], s_late).wait()

        @pl.when(h >= 5)
        def _():
            a_copy(h - 5).start()

        oacc, ctx = {}, {}
        conv = conv_ops(RQ + h * GH, GH, None, (), FWD_AT, INV_AT)
        wo = _b(woT[h])
        causal = causal_mask()

        def project(n):
            c = n // 2
            r = slice(c * KC // 2, (c + 1) * KC // 2)
            if n % 2 == 0:
                ks[r, :] = _w(_dot(_b(ckv[r, :]), _b(wks[...])).astype(BF16))
                if c == 0:
                    k0s[h] = ks[r, :]
            else:
                vT = jax.lax.dot_general(_b(wvs[...]), _b(ckv[r, :]), NT, preferred_element_type=F32)
                vTs[:, c * KC:(c + 1) * KC] = _w(vT.astype(BF16))
                if c == 0:
                    v0s[h] = vTs[:, :KC]

        def pv(i, p, rl):
            ctx[i] = context(lambda r0, r1: vTs[r0:r1, :TQ * (i + 1)], p, rl)

        def oproj(i0, i1):
            for i in range(i0, i1):
                oacc[i] = _dot(wo, ctx[i])
                acc[:, TQ * i:TQ * (i + 1)] += oacc[i]

        def by_scores(blocks):
            return lambda b: blocks[(b - JIT0) // 2][(b - JIT0) % 2 * 64:][:8] if b >= JIT0 else None

        def by_oproj(i0):
            return lambda b: oacc[i0 + 2 * (TAIL_PACE * b // DA)][TAIL_PACE * b % DA // 8 * 8:][:8]

        for n in range(T0 + 1):
            project(n)
        st = None
        for i in range(T0, NQ):
            if i + 1 < NQ:
                project(i + 1)
            if i in OFILL:
                oproj(*OFILL[i])
            prev, st = st, scores(i, _b(ks[:TQ * (i + 1) // 2, :]), _b(qs[h, :, TQ * i:TQ * (i + 1)]), causal)
            if i > T0:
                p, rl = softmax(*prev[:2], by_scores(st[0]))
                if st[2] is not None:
                    rl = _after(st[2], rl)
            if i in conv:
                conv[i]()
            if i > T0:
                pv(i - 1, p, rl)
        a_transpose(jnp.maximum(h - 4, 0))
        prep_wkv(jnp.minimum(h + 1, H - 1))
        oproj(OFILL[NQ - 1][1], OSPLIT)
        p, rl = softmax(*st[:2], by_oproj(OFILL[NQ - 1][1]))
        pv(NQ - 1, p, rl)
        oproj(OSPLIT, NQ)
        return carry

    jax.lax.fori_loop(0, H, head, 0)

    def b_transpose(src, dst, tok=None):
        blk = jnp.concatenate([aT[NA:, src], acc[:, src]], axis=0)
        if tok is not None:
            blk = jnp.concatenate([x for r in range(0, 2 * DA - NA, 128)
                                   for x in (_after(tok, blk[r:r + 8]), blk[r + 8:r + 128])], axis=0)
        blk = blk.astype(BF16)
        outs[dst, NA:] = _b(_w(blk)).T

    def b_copy(i0, i1):
        return cp(outs.at[i0 * TQ:i1 * TQ, NA:], out_hbm.at[i0 * TQ:i1 * TQ, NA:], s_out)

    nsteps = H // HB
    c_b = [b_copy(T0 + NB * t, min(T0 + NB * (t + 1), NQ)) for t in range(nsteps - 1)]
    a_copy(11).start()

    def first_tiles(t, carry):
        for u in range(nsteps - 1):
            pl.when(t == u + 1)(c_b[u].start)
        causal = causal_mask()
        items = [(HB * t + u, i) for u in range(HB) for i in range(T0)]
        sts = [scores(i, _b(k0s[h, :TQ * (i + 1) // 2, :]), _b(qs[h, :, TQ * i:TQ * (i + 1)]), causal)
               for h, i in items]
        ctxs = [context(lambda r0, r1: v0s[h, r0:r1, :TQ * (i + 1)], *softmax(*st[:2], lambda b: None))
                for (h, i), st in zip(items, sts)]
        o, ds = {}, []
        for (h, i), c in zip(items, ctxs):
            ds.append(_dot(_b(woT[h]), c))
            o[i] = ds[-1] if i not in o else o[i] + ds[-1]
        for k in range(NB):
            cb = T0 + NB * t + k
            tok = ds[2 * (OUT_PACE * k // DA)][OUT_PACE * k % DA // 8 * 8:][:8]
            b_transpose(pl.ds(pl.multiple_of(jnp.minimum(cb, NQ - 1) * TQ, TQ), TQ),
                        pl.ds(pl.multiple_of(cb * TQ, TQ), TQ), tok)
        for i in range(T0):
            acc[:, TQ * i:TQ * (i + 1)] += o[i]
        return carry

    jax.lax.fori_loop(0, nsteps, first_tiles, 0)

    c_last = []
    for i in range(T0):
        b_transpose(slice(i * TQ, (i + 1) * TQ), slice(i * TQ, (i + 1) * TQ))
        c_last.append(b_copy(i, i + 1))
        c_last[-1].start()
    for c in [a_copy(p) for p in range(12)] + c_b + c_last:
        c.wait()


@jax.jit
def pallas_concat_heads__ssm_conv_h3__compressed_kv_cla__prompt_kernel(
    A_q: jax.Array,
    A_k: jax.Array,
    A_v: jax.Array,
    A_shift_k: jax.Array,
    A_ssm_k: jax.Array,
    A_ssm_D: jax.Array,
    B_x: jax.Array,
    B_c_kv: jax.Array,
    B_w_q: jax.Array,
    B_w_uk: jax.Array,
    B_w_uv: jax.Array,
    B_w_o: jax.Array,
):
    fwd, inv = _dft_mats()
    tr = lambda a: jnp.swapaxes(a, 1, 2).reshape(DA, S)
    any_spec = pl.BlockSpec(memory_space=pl.ANY)
    out = pl.pallas_call(
        _kernel,
        out_shape=jax.ShapeDtypeStruct((S, 2 * DA), BF16),
        in_specs=[any_spec] * 14,
        out_specs=any_spec,
        scratch_shapes=[
            pltpu.VMEM((DA // 2, S), U32),
            pltpu.VMEM((DA // 2, S), U32),
            pltpu.VMEM((DA // 2, S), U32),
            pltpu.VMEM((DA // 2, S), U32),
            pltpu.VMEM((DA // 2, S), U32),
            pltpu.VMEM((S // 2, DC), U32),
            pltpu.VMEM((H // 2, DA, D), U32),
            pltpu.VMEM((H // 2, 2, DC, D), U32),
            pltpu.VMEM((H, DA // 2, D), U32),
            pltpu.VMEM((D, DA), U32),
            pltpu.VMEM((H, D // 2, S), U32),
            pltpu.VMEM((S // 2, D), U32),
            pltpu.VMEM((D // 2, S), U32),
            pltpu.VMEM((H, KC // 2, D), U32),
            pltpu.VMEM((H, D // 2, KC), U32),
            pltpu.VMEM((DA, S), F32),
            pltpu.VMEM((DA, S), F32),
            pltpu.VMEM((KS + 1, DA, 128), F32),
            pltpu.VMEM((DC // 2, D), U32),
            pltpu.VMEM((D // 2, DC), U32),
            pltpu.VMEM(((T0 + NB * H // HB) * TQ, 2 * DA), BF16),
            pltpu.VMEM((KS, DA), BF16),
            pltpu.VMEM((DA,), BF16),
            pltpu.VMEM((C // 2, 2 * C), U32),
            pltpu.VMEM((C, C), U32),
            pltpu.SemaphoreType.DMA((9,)),
        ],
        compiler_params=pltpu.CompilerParams(vmem_limit_bytes=100 * 1024 * 1024),
    )(
        tr(A_q), tr(A_k), tr(A_v), A_shift_k.T, A_ssm_k, A_ssm_D, tr(B_x), B_c_kv.reshape(S, DC),
        B_w_q, B_w_uk, B_w_uv,
        jnp.swapaxes(B_w_o, 1, 2), jnp.asarray(fwd, BF16), jnp.asarray(inv, BF16),
    )
    return out.reshape(1, S, 2 * DA)
```

```python
import functools
import math

import jax
import jax.numpy as jnp
import numpy as np
import jax.experimental.pallas as pl
import jax.experimental.pallas.tpu as pltpu

F32 = jnp.float32
BF16 = jnp.bfloat16
U32 = jnp.uint32

S = 2048
DA = 448
H = 16
D = 256
DC = 1024
KS = 4
C = 128
NCH = S // C
GQ = 32
GH = 16
RQ = GQ * (H // 2 - 2)
TQ = 128
NQ = S // TQ
KC = 256
NA = 384
NT = (((1,), (1,)), ((), ()))
LOG2E = math.log2(math.e)
QSCALE = (D ** -0.5) * LOG2E
NEG = -1e9 * LOG2E

X_CHUNKS = ((0, 384), (384, 1152), (1152, 2048))
Q_FWD_AT = 2
Q_INV_AT = {6: (0, 1, 2, 3, 4, 5), 7: (6, 7), 8: (8, 9), **{a - 1: (a,) for a in range(10, NCH)}}
Q_GATE_PACE = (0, 1)
T0 = 2
HB = 4
NB = 5
FWD_AT = 3
INV_AT = {6: (0, 1, 2, 3), 7: (4, 5, 6), 8: (7, 8), **{a: (a,) for a in range(9, NCH)}}
OFILL = {15: (2, 4)}
OSPLIT = 12
PMAX = 3
JIT0 = 4
TAIL_PACE = 32
OUT_PACE = 150


def _dft_mats():
    k = np.concatenate([np.arange(0, C, 2), np.arange(1, C, 2)]).astype(np.float64)
    n = np.arange(C, dtype=np.float64)
    th = 2.0 * np.pi * np.outer(n, k + 0.5) / (2 * C)
    fwd = np.concatenate([np.cos(th), np.sin(th)], axis=1)
    inv = fwd.T / C
    return fwd, inv


def _b(x):
    return pltpu.bitcast(x, BF16)


def _w(x):
    return pltpu.bitcast(x, U32)


def _dot(a, b):
    return jnp.dot(a, b, preferred_element_type=F32)


def _after(tok, x):
    return jnp.where(jnp.abs(tok) < -1.0, tok, x)


def _kernel(qT_hbm, kT_hbm, vT_hbm, shT_hbm, ssm_hbm, dvec_hbm, xT_hbm, ckv_hbm, wq_hbm, wuk_hbm, wuv_hbm,
            woT_hbm, fwd_hbm, inv_hbm,
            out_hbm,
            aq, ak, av, ssm, xT, ckv, wq, wkv, woT, wqs, qs, ks, vTs, k0s, v0s, acc, aT, coef, wks, wvs,
            outs, shT, dvec, fwd, inv, sems):
    def cp(src, dst, sem):
        return pltpu.make_async_copy(src, dst, sems.at[sem])

    s_wq0, s_x, s_a0, s_wq, s_early, s_late, s_out = 0, 1, 4, 5, 6, 7, 8
    wq_u, wuk_u, wuv_u, x_u = (r.bitcast(U32) for r in (wq_hbm, wuk_hbm, wuv_hbm, xT_hbm))
    a_in = [(r.bitcast(U32), d) for r, d in ((kT_hbm, ak), (vT_hbm, av), (ssm_hbm, ssm), (qT_hbm, aq))]

    def a_rows(r0, r1, sem):
        return [cp(src.at[r0 // 2:r1 // 2], dst.at[r0 // 2:r1 // 2], sem) for src, dst in a_in]

    c_wq0 = cp(wq_u.at[:, 0, :], wq.at[0], s_wq0)
    c_x = [[cp(x_u.at[:, c0:c1], xT.at[:, c0:c1], s_x + t)] for t, (c0, c1) in enumerate(X_CHUNKS)]
    c_x[-1] += [cp(wq_u.at[:, j, :], wq.at[j], s_x + 2) for j in (1, 2)]
    c_x[-1] += [cp(shT_hbm, shT, s_x + 2), cp(dvec_hbm, dvec, s_x + 2)]
    c_a0 = [cp(fwd_hbm.bitcast(U32), fwd, s_a0), cp(inv_hbm.bitcast(U32), inv, s_a0)] + a_rows(0, GQ, s_a0)
    c_wq = a_rows(GQ, RQ, s_wq) + [cp(wq_u.at[:, j, :], wq.at[j], s_wq) for j in range(3, H // 2)]
    early = [cp(src, dst, s_early) for src, dst in (
        (wuk_u.at[:, 0, :], wkv.at[0, 0]), (wuv_u.at[:, 0, :], wkv.at[0, 1]), (ckv_hbm.bitcast(U32), ckv),
        (woT_hbm.bitcast(U32), woT))] + a_rows(RQ, DA, s_early)
    late = [cp(src.at[:, j, :], wkv.at[j, t], s_late)
            for j in range(1, H // 2) for t, src in enumerate((wuk_u, wuv_u))]
    for c in [c_wq0, *c_x[0], *c_x[1], *c_x[2], *c_a0, *c_wq, *early, *late]:
        c.start()

    hi_mask = jnp.uint32(0xFFFF0000)

    def prep_wq(j):
        w = wq[j]
        wqs[:D // 2, :] = _w(pltpu.bitcast(w << 16, F32).T.astype(BF16))
        wqs[D // 2:, :] = _w(pltpu.bitcast(w & hi_mask, F32).T.astype(BF16))

    def prep_wkv(h):
        j = h >> 1
        sh = jnp.asarray(16 - 16 * (h & 1), U32)
        wks[...] = _w(pltpu.bitcast((wkv[j, 0] << sh) & hi_mask, F32).astype(BF16))
        wvs[...] = _w(pltpu.bitcast((wkv[j, 1] << sh) & hi_mask, F32).T.astype(BF16))

    def qproj(j, c0, c1):
        q = _dot(_b(wqs[...]), _b(xT[:, c0:c1]))
        q2 = (q * QSCALE).astype(BF16)
        qs[2 * j, :, c0:c1] = _w(q2[:D])
        qs[2 * j + 1, :, c0:c1] = _w(q2[D:])
        return q

    def zero(i, carry):
        acc[pl.ds(pl.multiple_of(i * 32, 32), 32), :] = jnp.zeros((32, S), F32)
        return carry

    jax.lax.fori_loop(0, DA // 32, zero, 0)

    def conv_ops(row0, G, proj, pace, fwd_at, inv_at):
        rows = pl.ds(pl.multiple_of(row0, 16), G)
        roww = pl.ds(pl.multiple_of(row0 >> 1, 8), G // 2)
        lane = jax.lax.broadcasted_iota(jnp.int32, (G, C), 1)
        hc = C // 2
        st = {}

        def forward():
            kvs, kprev = [], None
            for c in range(NCH):
                cols = slice(c * C, (c + 1) * C)
                kf = _b(ak[roww, cols]).astype(F32)
                if pace:
                    src = proj[pace[c * len(pace) // NCH]]
                    r0 = (c * len(pace) % NCH) * src.shape[0] // NCH // 8 * 8
                    kf = jnp.concatenate([_after(src[r0:r0 + 8, :C], kf[:8]), kf[8:]], axis=0)
                ksh = kf * coef[0, rows, :]
                rolled = []
                for j in range(1, KS):
                    r = pltpu.roll(kf, j, 1)
                    rolled.append(r)
                    ksh = ksh + jnp.where(lane >= j, r, 0.0 if kprev is None else kprev[j - 1]) * coef[j, rows, :]
                kvs.append((ksh * _b(av[roww, cols]).astype(F32)).astype(BF16))
                kprev = rolled
            st["kv"] = kvs
            lhs = jnp.concatenate(kvs + [_b(ssm[roww, c * C:(c + 1) * C]) for c in range(NCH)], axis=0)
            both = _dot(lhs, _b(fwd[...]))
            xh = [both[c * G:(c + 1) * G] for c in range(NCH)]
            st["h"] = [both[(NCH + c) * G:(NCH + c + 1) * G] for c in range(NCH)]
            st["u"] = [xh[0]] + [
                xh[c] + jnp.concatenate([xh[c - 1][:, 2 * hc:3 * hc], -xh[c - 1][:, 3 * hc:], -xh[c - 1][:, :hc],
                                         xh[c - 1][:, hc:2 * hc]], axis=1) for c in range(1, NCH)]

        def inverse(todo):
            ws, tok = [], None
            for a in todo:
                slabs = []
                for r0 in range(0, G, 8):
                    rs = slice(r0, r0 + 8)
                    zr = zi = None
                    for c in range(a + 1):
                        ur, ui = st["u"][c][rs, :C], st["u"][c][rs, C:]
                        hr, hi = st["h"][a - c][rs, :C], st["h"][a - c][rs, C:]
                        if zr is None and tok is not None:
                            ur = _after(tok, ur)
                        pr = ur * hr - ui * hi
                        pi = ur * hi + ui * hr
                        zr = pr if zr is None else zr + pr
                        zi = pi if zi is None else zi + pi
                    tok = zr
                    slabs.append(jnp.concatenate([zr, zi], axis=1))
                ws.append(jnp.concatenate(slabs, axis=0).astype(BF16))
            ys = _dot(jnp.concatenate(ws, axis=0), _b(inv[...]))
            for t, a in enumerate(todo):
                cols = slice(a * C, (a + 1) * C)
                y = ys[t * G:(t + 1) * G] + st["kv"][a].astype(F32) * coef[KS, rows, :]
                aT[rows, cols] = _b(aq[roww, cols]).astype(F32) * y

        ops = {fwd_at: forward}
        for step, todo in inv_at.items():
            ops[step] = functools.partial(inverse, todo)
        return ops

    c_wq0.wait()
    prep_wq(0)
    for cs, (c0, c1) in zip(c_x, X_CHUNKS):
        for c in cs:
            c.wait()
        qproj(0, c0, c1)
    prep_wq(1)
    taps = shT[...].astype(F32)
    for j in range(KS + 1):
        row = taps[j:j + 1] if j < KS else dvec[...].astype(F32)[None, :]
        coef[j] = jnp.broadcast_to(row, (128, DA)).T
    for c in c_a0:
        c.wait()

    def qpair(j, carry):
        @pl.when(j == 2)
        def _():
            for c in c_wq:
                c.wait()

        qv = {}
        conv = conv_ops((j - 1) * GQ, GQ, qv, Q_GATE_PACE, Q_FWD_AT, Q_INV_AT)
        for p in range(NQ):
            qv[p] = qproj(j, p * TQ, (p + 1) * TQ)
            if p in conv:
                conv[p]()
        prep_wq(j + 1)
        return carry

    jax.lax.fori_loop(1, H // 2 - 1, qpair, 0)

    for c in early:
        c.wait()
    qproj(H // 2 - 1, 0, S)
    prep_wkv(0)

    def a_piece(p):
        r = pl.ds(pl.multiple_of((p & 3) * (S // 4), S // 4), S // 4)
        c = pl.ds(pl.multiple_of((p >> 2) * 128, 128), 128)
        return r, c

    def a_copy(p):
        r, c = a_piece(p)
        return cp(outs.at[r, c], out_hbm.at[r, c], s_out)

    def a_transpose(p):
        r, c = a_piece(p)
        outs[r, c] = _b(_w(aT[c, r].astype(BF16))).T

    def causal_mask():
        krow = jax.lax.broadcasted_iota(jnp.int32, (TQ, TQ), 0)
        qcol = jax.lax.broadcasted_iota(jnp.int32, (TQ, TQ), 1)
        return krow <= qcol

    def scores(i, k, q, causal):
        n = TQ * (i + 1)
        sT = _dot(k, q)
        blocks = [sT[c0:c0 + TQ] for c0 in range(0, n - TQ, TQ)] + [jnp.where(causal, sT[n - TQ:], NEG)]
        m8, part = None, None
        for b, blk in enumerate(blocks):
            bm = jnp.max(blk.reshape(TQ // 8, 8, TQ), axis=0)
            m8 = bm if m8 is None else jnp.where(bm > m8, bm, m8)
            if b == i - PMAX:
                part = m8[0:1]
        return blocks, m8, part

    def softmax(blocks, m8, pace):
        m8 = jnp.broadcast_to(jnp.max(m8, axis=0, keepdims=True), (8, TQ))
        ls, p, ps = None, None, []
        for b, blk in enumerate(blocks):
            if pace(b) is not None:
                mm = _after(pace(b), m8)
            else:
                mm = m8 if p is None else jnp.where(p[TQ - 8:] < 0.0, p[TQ - 8:], m8)
            p = jnp.exp2(blk - jnp.concatenate([mm] * (TQ // 8), axis=0))
            part = jnp.sum(p.reshape(TQ // 8, 8, TQ), axis=0)
            ls = part if ls is None else ls + part
            ps.append(p)
        return jnp.concatenate(ps, axis=0).astype(BF16), 1.0 / jnp.sum(ls, axis=0, keepdims=True)

    def context(vT, p, rl):
        halves = [_dot(_b(vT(t * D // 4, (t + 1) * D // 4)), p) * rl for t in range(2)]
        return jnp.concatenate(halves, axis=0).astype(BF16)

    def head(h, carry):
        @pl.when(h == 1)
        def _():
            cp(wkv.at[1:], wkv.at[1:], s_late).wait()

        @pl.when(h >= 5)
        def _():
            a_copy(h - 5).start()

        oacc, ctx = {}, {}
        conv = conv_ops(RQ + h * GH, GH, None, (), FWD_AT, INV_AT)
        wo = _b(woT[h])
        causal = causal_mask()

        def project(n):
            c = n // 2
            r = slice(c * KC // 2, (c + 1) * KC // 2)
            if n % 2 == 0:
                ks[r, :] = _w(_dot(_b(ckv[r, :]), _b(wks[...])).astype(BF16))
                if c == 0:
                    k0s[h] = ks[r, :]
            else:
                vT = jax.lax.dot_general(_b(wvs[...]), _b(ckv[r, :]), NT, preferred_element_type=F32)
                vTs[:, c * KC:(c + 1) * KC] = _w(vT.astype(BF16))
                if c == 0:
                    v0s[h] = vTs[:, :KC]

        def pv(i, p, rl):
            ctx[i] = context(lambda r0, r1: vTs[r0:r1, :TQ * (i + 1)], p, rl)

        def oproj(i0, i1):
            for i in range(i0, i1):
                oacc[i] = _dot(wo, ctx[i])
                acc[:, TQ * i:TQ * (i + 1)] += oacc[i]

        def by_scores(blocks):
            return lambda b: blocks[(b - JIT0) // 2][(b - JIT0) % 2 * 64:][:8] if b >= JIT0 else None

        def by_oproj(i0):
            return lambda b: oacc[i0 + 2 * (TAIL_PACE * b // DA)][TAIL_PACE * b % DA // 8 * 8:][:8]

        for n in range(T0 + 1):
            project(n)
        st = None
        for i in range(T0, NQ):
            if i + 1 < NQ:
                project(i + 1)
            if i in OFILL:
                oproj(*OFILL[i])
            prev, st = st, scores(i, _b(ks[:TQ * (i + 1) // 2, :]), _b(qs[h, :, TQ * i:TQ * (i + 1)]), causal)
            if i > T0:
                p, rl = softmax(*prev[:2], by_scores(st[0]))
                if st[2] is not None:
                    rl = _after(st[2], rl)
            if i in conv:
                conv[i]()
            if i > T0:
                pv(i - 1, p, rl)
        a_transpose(jnp.maximum(h - 4, 0))
        prep_wkv(jnp.minimum(h + 1, H - 1))
        oproj(OFILL[NQ - 1][1], OSPLIT)
        p, rl = softmax(*st[:2], by_oproj(OFILL[NQ - 1][1]))
        pv(NQ - 1, p, rl)
        oproj(OSPLIT, NQ)
        return carry

    jax.lax.fori_loop(0, H, head, 0)

    def b_transpose(src, dst, tok=None):
        blk = jnp.concatenate([aT[NA:, src], acc[:, src]], axis=0)
        if tok is not None:
            blk = jnp.concatenate([x for r in range(0, 2 * DA - NA, 128)
                                   for x in (_after(tok, blk[r:r + 8]), blk[r + 8:r + 128])], axis=0)
        blk = blk.astype(BF16)
        outs[dst, NA:] = _b(_w(blk)).T

    def b_copy(i0, i1):
        return cp(outs.at[i0 * TQ:i1 * TQ, NA:], out_hbm.at[i0 * TQ:i1 * TQ, NA:], s_out)

    nsteps = H // HB
    c_b = [b_copy(T0 + NB * t, min(T0 + NB * (t + 1), NQ)) for t in range(nsteps - 1)]
    a_copy(11).start()

    def first_tiles(t, carry):
        for u in range(nsteps - 1):
            pl.when(t == u + 1)(c_b[u].start)
        causal = causal_mask()
        items = [(HB * t + u, i) for i in range(T0) for u in range(HB)]
        sts = [scores(i, _b(k0s[h, :TQ * (i + 1) // 2, :]), _b(qs[h, :, TQ * i:TQ * (i + 1)]), causal)
               for h, i in items]
        ctxs = [context(lambda r0, r1: v0s[h, r0:r1, :TQ * (i + 1)], *softmax(*st[:2], lambda b: None))
                for (h, i), st in zip(items, sts)]
        o, ds = {}, []
        for (h, i), c in zip(items, ctxs):
            ds.append(_dot(_b(woT[h]), c))
            o[i] = ds[-1] if i not in o else o[i] + ds[-1]
        for k in range(NB):
            cb = T0 + NB * t + k
            tok = ds[2 * (OUT_PACE * k // DA)][OUT_PACE * k % DA // 8 * 8:][:8]
            b_transpose(pl.ds(pl.multiple_of(jnp.minimum(cb, NQ - 1) * TQ, TQ), TQ),
                        pl.ds(pl.multiple_of(cb * TQ, TQ), TQ), tok)
        for i in range(T0):
            acc[:, TQ * i:TQ * (i + 1)] += o[i]
            if i == 0:
                b_transpose(slice(0, TQ), slice(0, TQ))
        return carry

    jax.lax.fori_loop(0, nsteps, first_tiles, 0)

    c_last = []
    for i in range(T0):
        if i > 0:
            b_transpose(slice(i * TQ, (i + 1) * TQ), slice(i * TQ, (i + 1) * TQ))
        c_last.append(b_copy(i, i + 1))
        c_last[-1].start()
    for c in [a_copy(p) for p in range(12)] + c_b + c_last:
        c.wait()


@jax.jit
def pallas_concat_heads__ssm_conv_h3__compressed_kv_cla__prompt_kernel(
    A_q: jax.Array,
    A_k: jax.Array,
    A_v: jax.Array,
    A_shift_k: jax.Array,
    A_ssm_k: jax.Array,
    A_ssm_D: jax.Array,
    B_x: jax.Array,
    B_c_kv: jax.Array,
    B_w_q: jax.Array,
    B_w_uk: jax.Array,
    B_w_uv: jax.Array,
    B_w_o: jax.Array,
):
    fwd, inv = _dft_mats()
    tr = lambda a: jnp.swapaxes(a, 1, 2).reshape(DA, S)
    any_spec = pl.BlockSpec(memory_space=pl.ANY)
    out = pl.pallas_call(
        _kernel,
        out_shape=jax.ShapeDtypeStruct((S, 2 * DA), BF16),
        in_specs=[any_spec] * 14,
        out_specs=any_spec,
        scratch_shapes=[
            pltpu.VMEM((DA // 2, S), U32),
            pltpu.VMEM((DA // 2, S), U32),
            pltpu.VMEM((DA // 2, S), U32),
            pltpu.VMEM((DA // 2, S), U32),
            pltpu.VMEM((DA // 2, S), U32),
            pltpu.VMEM((S // 2, DC), U32),
            pltpu.VMEM((H // 2, DA, D), U32),
            pltpu.VMEM((H // 2, 2, DC, D), U32),
            pltpu.VMEM((H, DA // 2, D), U32),
            pltpu.VMEM((D, DA), U32),
            pltpu.VMEM((H, D // 2, S), U32),
            pltpu.VMEM((S // 2, D), U32),
            pltpu.VMEM((D // 2, S), U32),
            pltpu.VMEM((H, KC // 2, D), U32),
            pltpu.VMEM((H, D // 2, KC), U32),
            pltpu.VMEM((DA, S), F32),
            pltpu.VMEM((DA, S), F32),
            pltpu.VMEM((KS + 1, DA, 128), F32),
            pltpu.VMEM((DC // 2, D), U32),
            pltpu.VMEM((D // 2, DC), U32),
            pltpu.VMEM(((T0 + NB * H // HB) * TQ, 2 * DA), BF16),
            pltpu.VMEM((KS, DA), BF16),
            pltpu.VMEM((DA,), BF16),
            pltpu.VMEM((C // 2, 2 * C), U32),
            pltpu.VMEM((C, C), U32),
            pltpu.SemaphoreType.DMA((9,)),
        ],
        compiler_params=pltpu.CompilerParams(vmem_limit_bytes=100 * 1024 * 1024),
    )(
        tr(A_q), tr(A_k), tr(A_v), A_shift_k.T, A_ssm_k, A_ssm_D, tr(B_x), B_c_kv.reshape(S, DC),
        B_w_q, B_w_uk, B_w_uv,
        jnp.swapaxes(B_w_o, 1, 2), jnp.asarray(fwd, BF16), jnp.asarray(inv, BF16),
    )
    return out.reshape(1, S, 2 * DA)
```
